```python
import jax
import jax.numpy as jnp

def _softmax(x, axis=-1):
    return jax.nn.softmax(x, axis=axis)

def _gelu(x):
    return jax.nn.gelu(x, approximate=True)

def _silu(x):
    return jax.nn.silu(x)

def _sigmoid(x):
    return jax.nn.sigmoid(x)

def _layernorm(x, axis=-1, eps=1e-05):
    m = jnp.mean(x, axis=axis, keepdims=True)
    v = jnp.var(x, axis=axis, keepdims=True)
    return (x - m) / jnp.sqrt(v + eps)

def _scatter_add(tgt, idx, src, axis=0):
    return tgt.at[idx].add(src)

def _segment_sum(src, seg, n):
    return jax.ops.segment_sum(src, seg, n)

class _Rng:

    def __init__(self, key):
        self._k = key

    def _next(self):
        self._k, sub = jax.random.split(self._k)
        return sub

    def normal(self, shape):
        return jax.random.normal(self._next(), shape, dtype=jnp.bfloat16)

    def randint(self, lo, hi, shape):
        return jax.random.randint(self._next(), shape, lo, hi, dtype=jnp.int32)

    def uniform(self, shape, lo=0.0, hi=1.0):
        return jax.random.uniform(self._next(), shape, jnp.bfloat16, lo, hi)

    def permutation(self, n):
        return jax.random.permutation(self._next(), n)
kernel_name = 'interleave_layers__linear_kernel_hedgehog__memory_aug_recurrent_mem_tr__prompt'

def setup_inputs():
    _rng = _Rng(jax.random.key(int.from_bytes(__import__("os").urandom(4), "little")))
    _w = lambda a: (lambda t: t.astype(jnp.bfloat16) if jnp.issubdtype(t.dtype, jnp.floating) else t)(jnp.asarray(a))

    def _A_setup():
        B, S, D, H = (1, 2048, 640, 32)
        Dh = D // H
        return {'x': _w((lambda *s: _rng.normal(s) * 0.05)(B, S, D)), 'wqkv': _w((lambda *s: _rng.normal(s) * 0.05)(D, 3 * D)), 'w_phi': _w((lambda *s: _rng.normal(s) * 0.05)(H, Dh, Dh) * Dh ** (-0.5)), 'wo': _w((lambda *s: _rng.normal(s) * 0.05)(D, D))}
    _A_in = _A_setup()

    def _B_setup():
        B, S, Dm = (1, 2048, 640)
        H, Dh = (32, 192)
        M, seg = (8, 32)
        seg = min(seg, S)
        S = S // seg * seg
        return {'x': _w((lambda *s: _rng.normal(s) * 0.05)(B, S, Dm)), 'mem0': _w((lambda *s: _rng.normal(s) * 0.05)(B, M, Dm)), 'Wq': _w((lambda *s: _rng.normal(s) * 0.05)(Dm, H, Dh) * Dm ** (-0.5)), 'Wk': _w((lambda *s: _rng.normal(s) * 0.05)(Dm, H, Dh) * Dm ** (-0.5)), 'Wv': _w((lambda *s: _rng.normal(s) * 0.05)(Dm, H, Dh) * Dm ** (-0.5)), 'Wo': _w((lambda *s: _rng.normal(s) * 0.05)(H, Dh, Dm) * (H * Dh) ** (-0.5)), 'seg_len': seg}
    _B_in = _B_setup()
    return {'A_x': _A_in['x'], 'A_wqkv': _A_in['wqkv'], 'A_w_phi': _A_in['w_phi'], 'A_wo': _A_in['wo'], 'B_x': _B_in['x'], 'B_mem0': _B_in['mem0'], 'B_Wq': _B_in['Wq'], 'B_Wk': _B_in['Wk'], 'B_Wv': _B_in['Wv'], 'B_Wo': _B_in['Wo'], 'B_seg_len': _B_in['seg_len']}

def reference(A_x, A_wqkv, A_w_phi, A_wo, B_x, B_mem0, B_Wq, B_Wk, B_Wv, B_Wo, B_seg_len):

    def _A_ref(x, wqkv, w_phi, wo):
        B, S, D = x.shape
        H = 32
        Dh = D // H
        qkv = (lambda x, *d: x.transpose(*d))((x @ wqkv).reshape(B, S, 3, H, Dh), 2, 0, 3, 1, 4)
        q, k, v = (qkv[0], qkv[1], qkv[2])
        pq = jnp.einsum('bhsd,hdf->bhsf', q, w_phi)
        pk = jnp.einsum('bhsd,hdf->bhsf', k, w_phi)
        phi_q = jnp.concatenate([_softmax(pq, axis=-1), _softmax(-pq, axis=-1)], axis=-1)
        phi_k = jnp.concatenate([_softmax(pk, axis=-1), _softmax(-pk, axis=-1)], axis=-1)
        kv = jnp.einsum('bhsf,bhsd->bhfd', phi_k, v)
        z = jnp.einsum('bhsf->bhf', phi_k)
        num = jnp.einsum('bhqf,bhfd->bhqd', phi_q, kv)
        den = jnp.einsum('bhqf,bhf->bhq', phi_q, z)[..., None] + 1e-06
        o = num / den
        return (lambda x, *d: x.transpose(*d))(o, 0, 2, 1, 3).reshape(B, S, D) @ wo

    def _B_ref(x, mem0, Wq, Wk, Wv, Wo, seg_len):
        B, S, Dm = x.shape
        H, Dh = (Wq.shape[1], Wq.shape[2])
        M = mem0.shape[1]
        scale = Dh ** (-0.5)
        n_seg = S // seg_len
        L = M + seg_len
        idx = jnp.arange(L)
        mask = (idx[:, None] < M) | (idx[:, None] >= idx[None, :])
        mem = mem0
        outs = []
        for s in range(n_seg):
            xs = x[:, s * seg_len:(s + 1) * seg_len, :].copy()
            h = jnp.concatenate([mem, xs], axis=1)
            q = jnp.einsum('btd,dhe->bhte', h, Wq)
            k = jnp.einsum('btd,dhe->bhte', h, Wk)
            v = jnp.einsum('btd,dhe->bhte', h, Wv)
            scores = jnp.einsum('bhqe,bhke->bhqk', q, k) * scale
            scores = jnp.where(mask[None, None], scores, -1000000000.0)
            p = _softmax(scores, axis=-1)
            o = jnp.einsum('bhqk,bhke->bhqe', p, v)
            o = jnp.einsum('bhte,hed->btd', o, Wo)
            mem = o[:, :M, :].copy()
            outs.append(o[:, M:, :])
        return jnp.concatenate(outs, axis=1)
    x = A_x
    x = x + _A_ref(_layernorm(x, axis=-1), A_wqkv, A_w_phi, A_wo)
    x = x + _B_ref(_layernorm(x, axis=-1), B_mem0, B_Wq, B_Wk, B_Wv, B_Wo, B_seg_len)
    x = x + _A_ref(_layernorm(x, axis=-1), A_wqkv, A_w_phi, A_wo)
    x = x + _B_ref(_layernorm(x, axis=-1), B_mem0, B_Wq, B_Wk, B_Wv, B_Wo, B_seg_len)
    return x
```

```python
import functools

import jax
import jax.numpy as jnp
from jax import lax
import jax.experimental.pallas as pl
import jax.experimental.pallas.tpu as pltpu

bf16 = jnp.bfloat16
f32 = jnp.float32
u32 = jnp.uint32
i32 = jnp.int32

S = 2048
D = 640
AH = 32
AD = 20
G = 8
NG = AH // G
GR = AD * G
TA = 256
BH = 32
BE = 192
M = 8
SEG = 32
L = M + SEG
NP = BH // 2
PW = 2 * BE
SCALE = BE ** -0.5
OLAG = 8

NT = (((1,), (1,)), ((), ()))


def _dot(a, b):
    return jnp.dot(a, b, preferred_element_type=f32)


def _dot_nt(a, b):
    return lax.dot_general(a, b, NT, preferred_element_type=f32)


def _recip(x):
    r = pl.reciprocal(x, approx=True)
    return r * (2.0 - x * r)


def _layernorm(x):
    m = jnp.mean(x, axis=-1, keepdims=True)
    xc = x - m
    v = jnp.mean(xc * xc, axis=-1, keepdims=True)
    return xc * lax.rsqrt(v + 1e-5)


def _greduce(x3, op):
    r = x3[0]
    for i in range(1, x3.shape[0]):
        r = op(r, x3[i])
    sh = G
    while sh < 8:
        r = op(r, pltpu.roll(r, sh, 0))
        sh *= 2
    return r


def _hedgehog_exp(p):
    t = p.shape[1]
    p3 = p.reshape(GR // 8, 8, t)
    mx = _greduce(p3, jnp.maximum)
    mn = _greduce(p3, jnp.minimum)
    ep = jnp.exp(p3 - mx[None])
    en = jnp.exp(mn[None] - p3)
    rp = _recip(_greduce(ep, jnp.add))
    rn = _recip(_greduce(en, jnp.add))
    return ep, en, rp, rn


def _kernel(x_ref, wqkv_ref, wphi_ref, wo_ref, mem_ref,
            bq_hbm, bk_hbm, bv_hbm, bo_hbm,
            out_ref,
            xs, xna, xnb, wq_s, wkv_s, kv_acc, kv_s, z_s,
            stage, wqkv_s, wo_s, sv_qkv, sv_o, sems):
    hbm = (bq_hbm, bk_hbm, bv_hbm, bo_hbm)

    def wcopy(t):
        return pltpu.make_async_copy(hbm[t], stage.at[t], sems.at[t])

    for t in range(4):
        wcopy(t).start()

    row = lax.broadcasted_iota(i32, (D, 32), 0)
    col = lax.broadcasted_iota(i32, (D, 32), 1)
    sel = (((row % GR) // G) == col).astype(bf16)
    rep = _dot(sel, wphi_ref[...])
    row = lax.broadcasted_iota(i32, (D, D), 0)
    col = lax.broadcasted_iota(i32, (D, D), 1)
    head = (row // GR) * G + row % G
    phit = jnp.where(head == col // AD, rep, 0.0).astype(bf16)
    wq_s[...] = _dot_nt(phit, wqkv_ref[:, 0:D]).astype(bf16)
    wkt = _dot_nt(phit, wqkv_ref[:, D:2 * D]).astype(bf16)
    wvt = wqkv_ref[:, 2 * D:3 * D].T
    for g in range(NG):
        wkv_s[g, 0:GR, :] = wkt[g * GR:(g + 1) * GR]
        wkv_s[g, GR:2 * GR, :] = wvt[g * GR:(g + 1) * GR]

    xs[...] = x_ref[...].astype(f32)

    def a_pass1(i, c):
        r0 = pl.multiple_of(i * TA, TA)
        xn = _layernorm(xs[pl.ds(r0, TA), :]).astype(bf16)
        xna[pl.ds(r0, TA), :] = xn
        for g in range(NG):
            y = _dot_nt(wkv_s[g], xn)
            ep, en, rp, rn = _hedgehog_exp(y[:GR])
            phi = jnp.concatenate([(ep * rp[None]).reshape(GR, TA),
                                   (en * rn[None]).reshape(GR, TA)], axis=0)
            zp = phi[:, 0:128]
            for j in range(1, TA // 128):
                zp = zp + phi[:, j * 128:(j + 1) * 128]
            z_s[g] += zp
            kv_acc[g] += _dot_nt(y[GR:].astype(bf16), phi.astype(bf16))
        return c

    def a_pass2(i, c):
        r0 = pl.multiple_of(i * TA, TA)
        xn = xna[pl.ds(r0, TA), :]
        outs = []
        for g in range(NG):
            p = _dot_nt(wq_s[g * GR:(g + 1) * GR, :], xn)
            ep, en, rp, rn = _hedgehog_exp(p)
            z = z_s[g]
            z = jnp.concatenate([z] * (TA // 128), axis=1).reshape(2, GR // 8, 8, TA)
            den = (_greduce(ep * z[0], jnp.add) * rp + _greduce(en * z[1], jnp.add) * rn) + 1e-6
            rd = _recip(den)
            phi = jnp.concatenate([(ep * (rp * rd)[None]).reshape(GR, TA),
                                   (en * (rn * rd)[None]).reshape(GR, TA)], axis=0)
            outs.append(_dot(kv_s[g], phi.astype(bf16)))
        o = jnp.concatenate(outs, axis=0).T.astype(bf16)
        xnew = xs[pl.ds(r0, TA), :] + _dot(o, wo_ref[...])
        xs[pl.ds(r0, TA), :] = xnew
        xnb[pl.ds(r0, TA), :] = _layernorm(xnew)
        return c

    def layer_a():
        kv_acc[...] = jnp.zeros_like(kv_acc)
        z_s[...] = jnp.zeros_like(z_s)
        lax.fori_loop(0, S // TA, a_pass1, 0)
        row = lax.broadcasted_iota(i32, (GR, 2 * GR), 0)
        col = lax.broadcasted_iota(i32, (GR, 2 * GR), 1)
        keep = (row // AD) == (col % G)
        for g in range(NG):
            kv_s[g] = jnp.where(keep, kv_acc[g], 0.0).astype(bf16)
            z_s[g] = jnp.broadcast_to(jnp.sum(z_s[g], axis=1, keepdims=True), (2 * GR, 128))
        lax.fori_loop(0, S // TA, a_pass2, 0)

    def b_prep():
        for t in range(4):
            wcopy(t).wait()

        def prep(j, c):
            r0 = pl.multiple_of(j * PW, PW)
            for t in range(3):
                wqkv_s[j, :, t * PW:(t + 1) * PW] = pltpu.bitcast(stage[t, pl.ds(r0, PW), :].T, u32)
            wo_s[j] = pltpu.bitcast(stage[3, pl.ds(r0, PW), :], u32)
            return c
        lax.fori_loop(0, NP, prep, 0)

    def layer_b():
        lane = lax.broadcasted_iota(i32, (L, 128), 1)
        lo = lane < 64
        zero = jnp.zeros((L, 128), f32)
        r = lax.broadcasted_iota(i32, (L, 2 * L), 0)
        c = lax.broadcasted_iota(i32, (L, 2 * L), 1)
        is_a = c < L
        key = jnp.where(is_a, c, c - L)
        valid = (r < M) | (r >= key)

        def blockdiag(k):
            kmid = k[:, 128:256]
            top = jnp.concatenate([k[:, :128], jnp.where(lo, kmid, 0.0), zero], axis=1)
            bot = jnp.concatenate([zero, jnp.where(lo, 0.0, kmid), k[:, 256:]], axis=1)
            return jnp.concatenate([top, bot], axis=0).astype(bf16)

        def softmax(s):
            s = jnp.where(valid, s * SCALE, -1e9)
            ma = jnp.max(jnp.where(is_a, s, -jnp.inf), axis=1, keepdims=True)
            mb = jnp.max(jnp.where(is_a, -jnp.inf, s), axis=1, keepdims=True)
            e = jnp.exp(s - jnp.where(is_a, ma, mb))
            la = jnp.sum(jnp.where(is_a, e, 0.0), axis=1, keepdims=True)
            lb = jnp.sum(jnp.where(is_a, 0.0, e), axis=1, keepdims=True)
            return (e * _recip(jnp.where(is_a, la, lb))).astype(bf16)

        def step(h, even):
            qs, ks, vs, ps, os_ = {}, {}, {}, {}, {}
            acc = None
            for t in range(NP + OLAG):
                if t < NP:
                    y = _dot(h, pltpu.bitcast(wqkv_s[t], bf16))
                    if even:
                        sv_qkv[t] = y[40:48]
                        y = y[:40]
                    else:
                        y = jnp.concatenate([y[:8], sv_qkv[t], y[8:]], axis=0)
                    qs[t] = y[:, :PW].astype(bf16)
                    ks[t] = blockdiag(y[:, PW:2 * PW])
                    vs[t] = blockdiag(y[:, 2 * PW:])
                j = t - 1
                if 0 <= j < NP:
                    ps[j] = softmax(_dot_nt(qs.pop(j), ks.pop(j)))
                j = t - 2
                if 0 <= j < NP:
                    o = _dot(ps.pop(j), vs.pop(j))
                    if even:
                        sv_o[j] = o[32:40]
                        o = o[:32]
                    else:
                        o = jnp.concatenate([o[:8], sv_o[j], o[8:]], axis=0)
                    os_[j] = o.astype(bf16)
                j = t - OLAG
                if 0 <= j < NP:
                    y = _dot(os_.pop(j), pltpu.bitcast(wo_s[j], bf16))
                    acc = y if acc is None else acc + y
            return acc

        def body(i, mem):
            r0 = pl.multiple_of(i * 64, 64)
            h = jnp.concatenate([mem, xnb[pl.ds(r0, 40), :]], axis=0).astype(bf16)
            y = step(h, True)
            xs[pl.ds(r0, 24), :] += y[8:]
            h = jnp.concatenate([y[:8], xnb[pl.ds(r0 + 40, 24), :]], axis=0).astype(bf16)
            y = step(h, False)
            xs[pl.ds(r0 + 24, 40), :] += y[8:]
            return y[:8]

        lax.fori_loop(0, S // 64, body, mem_ref[...].astype(f32))

    def layer(li, c):
        layer_a()

        @pl.when(li == 0)
        def _():
            b_prep()

        layer_b()
        return c

    lax.fori_loop(0, 2, layer, 0)
    out_ref[...] = xs[...].astype(bf16)


@functools.partial(jax.jit, static_argnames=("B_seg_len",))
def pallas_interleave_layers__linear_kernel_hedgehog__memory_aug_recurrent_mem_tr__prompt_kernel(
    A_x: jax.Array,
    A_wqkv: jax.Array,
    A_w_phi: jax.Array,
    A_wo: jax.Array,
    B_x: jax.Array,
    B_mem0: jax.Array,
    B_Wq: jax.Array,
    B_Wk: jax.Array,
    B_Wv: jax.Array,
    B_Wo: jax.Array,
    B_seg_len=SEG,
):
    assert B_seg_len == SEG
    HE = BH * BE
    x = A_x.reshape(S, D)
    wphi = jnp.pad(A_w_phi.transpose(2, 0, 1).reshape(AD, D), ((0, 32 - AD), (0, 0)))
    mem0 = B_mem0.reshape(M, D)
    bq = B_Wq.transpose(1, 2, 0).reshape(HE, D)
    bk = B_Wk.transpose(1, 2, 0).reshape(HE, D)
    bv = B_Wv.transpose(1, 2, 0).reshape(HE, D)
    bo = B_Wo.reshape(HE, D)

    vmem = pl.BlockSpec(memory_space=pltpu.VMEM)
    anyspec = pl.BlockSpec(memory_space=pl.ANY)
    out = pl.pallas_call(
        _kernel,
        out_shape=jax.ShapeDtypeStruct((S, D), bf16),
        in_specs=[vmem] * 5 + [anyspec] * 4,
        out_specs=vmem,
        scratch_shapes=[
            pltpu.VMEM((S, D), f32),
            pltpu.VMEM((S, D), bf16),
            pltpu.VMEM((S, D), f32),
            pltpu.VMEM((D, D), bf16),
            pltpu.VMEM((NG, 2 * GR, D), bf16),
            pltpu.VMEM((NG, GR, 2 * GR), f32),
            pltpu.VMEM((NG, GR, 2 * GR), bf16),
            pltpu.VMEM((NG, 2 * GR, 128), f32),
            pltpu.VMEM((4, HE, D), bf16),
            pltpu.VMEM((NP, D // 2, 3 * PW), u32),
            pltpu.VMEM((NP, PW // 2, D), u32),
            pltpu.VMEM((NP, 8, 3 * PW), f32),
            pltpu.VMEM((NP, 8, PW), f32),
            pltpu.SemaphoreType.DMA((4,)),
        ],
        compiler_params=pltpu.CompilerParams(vmem_limit_bytes=110 * 1024 * 1024),
    )(x, A_wqkv, wphi, A_wo, mem0, bq, bk, bv, bo)
    return out.reshape(1, S, D)
```

```python
import functools

import jax
import jax.numpy as jnp
from jax import lax
import jax.experimental.pallas as pl
import jax.experimental.pallas.tpu as pltpu

bf16 = jnp.bfloat16
f32 = jnp.float32
u32 = jnp.uint32
i32 = jnp.int32

S = 2048
D = 640
AH = 32
AD = 20
GR = 2 * AD
NG = AH // 2
CG = 4
CR = CG * GR
NC = NG // CG
TA = 256
NB = S // TA
BH = 32
BE = 192
HE = BH * BE
M = 8
SEG = 32
L = M + SEG
NP = BH // 2
PW = 2 * BE
SCALE = BE ** -0.5
NW = 3 * NP
WPB = NW // (2 * NB)

NT = (((1,), (1,)), ((), ()))

SEM_PHI, SEM_QKV, SEM_WO, SEM_MEM, SEM_BO, SEM_OUT = 0, 1, 2, 3, 4, 5
SEM_X = 6
SEM_W = SEM_X + NB
NSEM = SEM_W + NW


def _dot(a, b):
    return jnp.dot(a, b, preferred_element_type=f32)


def _dot_nt(a, b):
    return lax.dot_general(a, b, NT, preferred_element_type=f32)


def _pack(x):
    return pltpu.bitcast(x, u32)


def _unpack(x):
    return pltpu.bitcast(x, bf16)


def _recip(x):
    r = pl.reciprocal(x, approx=True)
    return r * (2.0 - x * r)


def _layernorm(x):
    m = jnp.mean(x, axis=-1, keepdims=True)
    xc = x - m
    v = jnp.mean(xc * xc, axis=-1, keepdims=True)
    return xc * lax.rsqrt(v + 1e-5)


def _freduce(x3, op):
    r = op(op(op(x3[0], x3[1]), op(x3[2], x3[3])), x3[4])
    r = op(r, pltpu.roll(r, 2, 0))
    return op(r, pltpu.roll(r, 4, 0))


def _hedgehog(p):
    t = p.shape[1]
    p3 = p.reshape(GR // 8, 8, t)
    ep = jnp.exp(p3 - _freduce(p3, jnp.maximum)[None])
    en = jnp.exp(_freduce(p3, jnp.minimum)[None] - p3)
    ep = ep * _recip(_freduce(ep, jnp.add))[None]
    en = en * _recip(_freduce(en, jnp.add))[None]
    return jnp.concatenate([ep.reshape(GR, t), en.reshape(GR, t)], axis=0).astype(bf16)


def _b_schedule():
    a, b, c = 3, 4, 3
    nin = NP - (a + b + c)
    out, o = [], 0
    for t in range(NP):
        out.append(("Q", t))
        if t >= 1:
            out.append(("S", t - 1))
        if t >= 2:
            out.append(("P", t - 2))
        if t >= NP - nin:
            out.append(("O", o))
            o += 1
    out += [("O", o + i) for i in range(a)]
    out += [("S", NP - 1), ("P", NP - 2)]
    out += [("O", o + a + i) for i in range(b)]
    out += [("P", NP - 1)]
    out += [("O", o + a + b + i) for i in range(c)]
    return out


def _kernel(x_hbm, wqkv_hbm, wphi_hbm, wo_hbm, mem_hbm, bq_hbm, bk_hbm, bv_hbm, bo_hbm,
            out_hbm,
            xin, wqkv_v, wphi_v, wo_v, mem_v, xs, xna, xnb, wq_s, wkv_s, ylast, kv_acc, kv_s, ot_s,
            stage, wb_s, bo_v, sv_o8, sv_e16, sems):
    bw_hbm = (bq_hbm, bk_hbm, bv_hbm)

    def whole(src, dst, slot):
        return pltpu.make_async_copy(src, dst, sems.at[slot])

    def x_copy(b):
        rows = pl.ds(pl.multiple_of(b * TA, TA), TA)
        return pltpu.make_async_copy(x_hbm.at[rows], xin.at[rows], sems.at[SEM_X + b])

    def w_start(q):
        t, j = divmod(q, NP)
        pltpu.make_async_copy(bw_hbm[t].at[pl.ds(j * PW, PW)], stage.at[q], sems.at[SEM_W + q]).start()

    def w_wait(q):
        pltpu.make_async_copy(stage.at[q], stage.at[q], sems.at[SEM_W + q]).wait()

    def out_copy(b):
        rows = pl.ds(pl.multiple_of(b * 64, 64), 64)
        return pltpu.make_async_copy(xin.at[rows], out_hbm.at[rows], sems.at[SEM_OUT])

    whole(wphi_hbm, wphi_v, SEM_PHI).start()
    whole(wqkv_hbm, wqkv_v, SEM_QKV).start()
    x_copy(0).start()
    for b in range(NB):
        if b + 1 < NB:
            x_copy(b + 1).start()
        for q in range(b * WPB, (b + 1) * WPB):
            w_start(q)
    whole(wo_hbm, wo_v, SEM_WO).start()
    whole(mem_hbm, mem_v, SEM_MEM).start()
    for q in range(NB * WPB, NW):
        w_start(q)
    whole(bo_hbm, bo_v, SEM_BO).start()

    whole(wphi_hbm, wphi_v, SEM_PHI).wait()
    row = lax.broadcasted_iota(i32, (CR, 32), 0)
    col = lax.broadcasted_iota(i32, (CR, 32), 1)
    sel = (((row % GR) // 2) == col).astype(bf16)
    row = lax.broadcasted_iota(i32, (CR, 256), 0)
    col = lax.broadcasted_iota(i32, (CR, 256), 1)
    head = (row // GR) * 2 + row % 2
    phit = []
    for c in range(NC):
        rep = _dot(sel, wphi_v[:, c * 128:c * 128 + 256])
        keep = (head + c * 2 * CG) == (col + c * 128) // AD
        phit.append(jnp.where(keep, rep, 0.0).astype(bf16))
    ylast[...] = jnp.zeros_like(ylast)
    whole(wqkv_hbm, wqkv_v, SEM_QKV).wait()
    wvt = wqkv_v[:, 2 * D:3 * D].T
    for c in range(NC):
        wk = _dot_nt(phit[c], wqkv_v[:, D + c * 128:D + c * 128 + 256]).astype(bf16)
        wkv_s[c] = _pack(jnp.concatenate([wk, wvt[c * CR:(c + 1) * CR]], axis=0))
    for c in range(NC):
        wq_s[c] = _pack(_dot_nt(phit[c], wqkv_v[:, c * 128:c * 128 + 256]).astype(bf16))

    def layer_a(first):
        def transposes(n):
            for u in range(WPB):
                q = n * WPB + u
                wb_s[q] = _pack(stage[q].T)

        def waits(n):
            for u in range(WPB):
                w_wait(n * WPB + u)

        def ln_block(b):
            rows = pl.ds(pl.multiple_of(b * TA, TA), TA)
            if first:
                x = xin[rows, :].astype(f32)
                xs[rows, :] = x
            else:
                x = xs[rows, :]
            xna[rows, :] = _layernorm(x).astype(bf16)

        def kv_update(c, y, ones):
            for u in range(CG):
                phi = _hedgehog(y[u * GR:(u + 1) * GR])
                vt = jnp.concatenate([y[CR + u * GR:CR + (u + 1) * GR], ones], axis=0).astype(bf16)
                kv_acc[c * CG + u] += _dot_nt(vt, phi)

        def pass1(i, carry):
            nxt = jnp.minimum(i + 1, NB - 1)
            if first:
                @pl.when(i + 1 < NB)
                def _():
                    x_copy(i + 1).wait()
                waits(i)
            xn = xna[pl.ds(pl.multiple_of(i * TA, TA), TA), :]
            ones = jnp.ones((8, TA), f32)
            yprev = ylast[...]
            ys = {}
            for c in range(NC):
                ys[c] = _dot_nt(_unpack(wkv_s[c]), xn)
                if c == 0:
                    live = jnp.where(i > 0, 1.0, 0.0)
                    rowi = lax.broadcasted_iota(i32, (2 * CR, TA), 0)
                    kv_update(NC - 1, jnp.where(rowi < CR, yprev, yprev * live), ones * live)
                else:
                    kv_update(c - 1, ys.pop(c - 1), ones)
            ylast[...] = ys.pop(NC - 1)
            ln_block(nxt)
            if first:
                transposes(i)
            return carry

        def front(i):
            xn = xna[pl.ds(pl.multiple_of(i * TA, TA), TA), :]
            sub = lax.broadcasted_iota(i32, (8, TA), 0) < 4

            def proj(c):
                return _dot_nt(_unpack(wq_s[c]), xn)

            def feat(c, p):
                for u in range(CG):
                    g = c * CG + u
                    y = _dot(kv_s[g], _hedgehog(p[u * GR:(u + 1) * GR]))
                    r = _recip(y[GR:] + 1e-6)
                    rr = pltpu.roll(r, 4, 0)
                    r0, r1 = jnp.where(sub, r, rr), jnp.where(sub, rr, r)
                    ot_s[g * GR:(g + 1) * GR, :] = y[:GR] * jnp.concatenate([r0, r0, r, r1, r1], axis=0)
            return proj, feat

        def back_load():
            return ot_s[...].T.astype(bf16)

        def back(i, o):
            rows = pl.ds(pl.multiple_of(i * TA, TA), TA)
            xs[rows, :] += _dot(o, wo_v[...])

        def pass2(i, has_back):
            if first:
                waits(NB + i)
            o = back_load() if has_back else None
            proj, feat = front(i)
            ps = {}
            for c in range(NC):
                ps[c] = proj(c)
                if c > 0:
                    feat(c - 1, ps.pop(c - 1))
            if has_back:
                back(i - 1, o)
            feat(NC - 1, ps.pop(NC - 1))
            if first:
                transposes(NB + i)

        kv_acc[...] = jnp.zeros_like(kv_acc)
        if first:
            x_copy(0).wait()
        ln_block(0)
        lax.fori_loop(0, NB, pass1, 0)
        kv_update(NC - 1, ylast[...], jnp.ones((8, TA), f32))
        row = lax.broadcasted_iota(i32, (GR + 8, 2 * GR), 0)
        col = lax.broadcasted_iota(i32, (GR + 8, 2 * GR), 1)
        keep = jnp.where(row < GR, row // AD, (row - GR) // 4) == col % 2
        for g in range(NG):
            kv_s[g] = jnp.where(keep, kv_acc[g], 0.0).astype(bf16)
        if first:
            whole(wo_hbm, wo_v, SEM_WO).wait()
        pass2(0, False)

        def loop2(i, carry):
            pass2(i, True)
            return carry
        lax.fori_loop(1, NB, loop2, 0)
        back(NB - 1, back_load())
        xnb[...] = _layernorm(xs[0:64, :])
        if first:
            whole(mem_hbm, mem_v, SEM_MEM).wait()
            whole(bo_hbm, bo_v, SEM_BO).wait()

    def layer_b(li):
        def blockdiag(k):
            n = k.shape[0]
            lo = lax.broadcasted_iota(i32, (n, 128), 1) < 64
            zero = jnp.zeros((n, 128), f32)
            kmid = k[:, 128:256]
            top = jnp.concatenate([k[:, :128], jnp.where(lo, kmid, zero), zero], axis=1)
            bot = jnp.concatenate([zero, jnp.where(lo, zero, kmid), k[:, 256:]], axis=1)
            return jnp.concatenate([top, bot], axis=0).astype(bf16)

        r = lax.broadcasted_iota(i32, (32, 2 * L), 0)
        c = lax.broadcasted_iota(i32, (32, 2 * L), 1)
        isa_e = c < L
        key = jnp.where(isa_e, c, c - L)
        valid_e = (r < M) | (r + 8 >= key)
        r = lax.broadcasted_iota(i32, (48, 112), 0)
        c = lax.broadcasted_iota(i32, (48, 112), 1)
        isa_o = c < 56
        key = jnp.where(isa_o, c, c - 56)
        valid_o = ((r < L) & (key < L) & ((r < M) | (r >= key))) | ((r >= L) & (key >= L) & (r + 8 >= key))

        def softmax(s, valid, isa):
            s = jnp.where(valid, s * SCALE, -1e9)
            ma = jnp.max(jnp.where(isa, s, -jnp.inf), axis=1, keepdims=True)
            mb = jnp.max(jnp.where(isa, -jnp.inf, s), axis=1, keepdims=True)
            e = jnp.exp(s - jnp.where(isa, ma, mb))
            la = jnp.sum(jnp.where(isa, e, 0.0), axis=1, keepdims=True)
            lb = jnp.sum(jnp.where(isa, 0.0, e), axis=1, keepdims=True)
            return (e * _recip(jnp.where(isa, la, lb))).astype(bf16)

        def step(hq, hkv, even):
            qs, kvs, ps, os_ = {}, {}, {}, {}
            acc = None
            for op, j in _b_schedule():
                if op == "Q":
                    for t in ((0, 1, 2) if even else (1, 2, 0)):
                        w = _unpack(wb_s[t * NP + j])
                        if t == 0:
                            qs[j] = _dot(hq, w).astype(bf16)
                            continue
                        cols = slice((t - 1) * PW, t * PW)
                        y = _dot(hkv, w)
                        if even:
                            sv_o8[j, :, cols] = y[40:48]
                            sv_e16[j, :, cols] = y[0:16]
                            y = y[:40]
                        else:
                            y = jnp.concatenate([y[:8], sv_o8[j, :, cols], y[8:], sv_e16[j, :, cols]], axis=0)
                        kvs[t, j] = blockdiag(y)
                elif op == "S":
                    s = _dot_nt(qs.pop(j), kvs.pop((1, j)))
                    ps[j] = softmax(s, valid_e, isa_e) if even else softmax(s, valid_o, isa_o)
                elif op == "P":
                    os_[j] = _dot(ps.pop(j), kvs.pop((2, j))).astype(bf16)
                else:
                    y = _dot(os_.pop(j), bo_v[j * PW:(j + 1) * PW, :])
                    acc = y if acc is None else acc + y
            return acc

        def body(i, mem):
            r0 = pl.multiple_of(i * 64, 64)
            xn = xnb[...]
            hkv = jnp.concatenate([mem, xn[0:40]], axis=0).astype(bf16)
            hq = jnp.concatenate([mem, xn[8:32]], axis=0).astype(bf16)
            ye = step(hq, hkv, True)
            mem = ye[:8]
            hkv = jnp.concatenate([mem, xn[40:64]], axis=0).astype(bf16)
            hq = jnp.concatenate([mem, xn[32:64], xn[0:8]], axis=0).astype(bf16)
            rn = pl.multiple_of(jnp.minimum(i + 1, S // 64 - 1) * 64, 64)
            xnb[...] = _layernorm(xs[pl.ds(rn, 64), :])
            yo = step(hq, hkv, False)
            xnew = xs[pl.ds(r0, 64), :] + jnp.concatenate([yo[40:48], ye[8:], yo[8:40]], axis=0)
            xs[pl.ds(r0, 64), :] = xnew
            xin[pl.ds(r0, 64), :] = xnew.astype(bf16)

            @pl.when(li == 1)
            def _():
                out_copy(i).start()
            return yo[:8]

        lax.fori_loop(0, S // 64, body, mem_v[...].astype(f32))

    def layer(li, carry):
        @pl.when(li == 0)
        def _():
            layer_a(True)

        @pl.when(li == 1)
        def _():
            layer_a(False)

        layer_b(li)
        return carry

    lax.fori_loop(0, 2, layer, 0)
    pltpu.make_async_copy(xin, out_hbm, sems.at[SEM_OUT]).wait()


@functools.partial(jax.jit, static_argnames=("B_seg_len",))
def pallas_interleave_layers__linear_kernel_hedgehog__memory_aug_recurrent_mem_tr__prompt_kernel(
    A_x: jax.Array,
    A_wqkv: jax.Array,
    A_w_phi: jax.Array,
    A_wo: jax.Array,
    B_x: jax.Array,
    B_mem0: jax.Array,
    B_Wq: jax.Array,
    B_Wk: jax.Array,
    B_Wv: jax.Array,
    B_Wo: jax.Array,
    B_seg_len=SEG,
):
    assert B_seg_len == SEG
    x = A_x.reshape(S, D)
    wphi = jnp.pad(A_w_phi.transpose(2, 0, 1).reshape(AD, D), ((0, 32 - AD), (0, 0)))
    mem0 = B_mem0.reshape(M, D)
    bq = B_Wq.transpose(1, 2, 0).reshape(HE, D)
    bk = B_Wk.transpose(1, 2, 0).reshape(HE, D)
    bv = B_Wv.transpose(1, 2, 0).reshape(HE, D)
    bo = B_Wo.reshape(HE, D)

    anyspec = pl.BlockSpec(memory_space=pl.ANY)
    out = pl.pallas_call(
        _kernel,
        out_shape=jax.ShapeDtypeStruct((S, D), bf16),
        in_specs=[anyspec] * 9,
        out_specs=anyspec,
        scratch_shapes=[
            pltpu.VMEM((S, D), bf16),
            pltpu.VMEM((D, 3 * D), bf16),
            pltpu.VMEM((32, D), bf16),
            pltpu.VMEM((D, D), bf16),
            pltpu.VMEM((M, D), bf16),
            pltpu.VMEM((S, D), f32),
            pltpu.VMEM((S, D), bf16),
            pltpu.VMEM((64, D), f32),
            pltpu.VMEM((NC, CR // 2, D), u32),
            pltpu.VMEM((NC, CR, D), u32),
            pltpu.VMEM((2 * CR, TA), f32),
            pltpu.VMEM((NG, GR + 8, 2 * GR), f32),
            pltpu.VMEM((NG, GR + 8, 2 * GR), bf16),
            pltpu.VMEM((D, TA), f32),
            pltpu.VMEM((NW, PW, D), bf16),
            pltpu.VMEM((NW, D // 2, PW), u32),
            pltpu.VMEM((HE, D), bf16),
            pltpu.VMEM((NP, 8, 2 * PW), f32),
            pltpu.VMEM((NP, 16, 2 * PW), f32),
            pltpu.SemaphoreType.DMA((NSEM,)),
        ],
        compiler_params=pltpu.CompilerParams(vmem_limit_bytes=110 * 1024 * 1024),
    )(x, A_wqkv, wphi, A_wo, mem0, bq, bk, bv, bo)
    return out.reshape(1, S, D)
```

```python
import functools

import jax
import jax.numpy as jnp
from jax import lax
import jax.experimental.pallas as pl
import jax.experimental.pallas.tpu as pltpu

bf16 = jnp.bfloat16
f32 = jnp.float32
u32 = jnp.uint32
i32 = jnp.int32

S = 2048
D = 640
AH = 32
AD = 20
GR = 2 * AD
NG = AH // 2
CG = 4
CR = CG * GR
NC = NG // CG
TA = 256
NB = S // TA
BH = 32
BE = 192
HE = BH * BE
M = 8
SEG = 32
L = M + SEG
NP = BH // 2
PW = 2 * BE
SCALE = BE ** -0.5
UB = 2
TB = 64 * UB
NI = S // TB
NW = 3 * NP
WPB = NW // (2 * NB)

NT = (((1,), (1,)), ((), ()))

SEM_PHI, SEM_QKV, SEM_WO, SEM_MEM, SEM_BO, SEM_OUT = 0, 1, 2, 3, 4, 5
SEM_X = 6
SEM_W = SEM_X + NB
NSEM = SEM_W + NW


def _dot(a, b):
    return jnp.dot(a, b, preferred_element_type=f32)


def _dot_nt(a, b):
    return lax.dot_general(a, b, NT, preferred_element_type=f32)


def _pack(x):
    return pltpu.bitcast(x, u32)


def _unpack(x):
    return pltpu.bitcast(x, bf16)


def _recip(x):
    r = pl.reciprocal(x, approx=True)
    return r * (2.0 - x * r)


def _layernorm(x):
    m = jnp.mean(x, axis=-1, keepdims=True)
    xc = x - m
    v = jnp.mean(xc * xc, axis=-1, keepdims=True)
    return xc * lax.rsqrt(v + 1e-5)


def _freduce(x3, op):
    r = op(op(op(x3[0], x3[1]), op(x3[2], x3[3])), x3[4])
    r = op(r, pltpu.roll(r, 2, 0))
    return op(r, pltpu.roll(r, 4, 0))


def _hedgehog(p):
    t = p.shape[1]
    p3 = p.reshape(GR // 8, 8, t)
    ep = jnp.exp(p3 - _freduce(p3, jnp.maximum)[None])
    en = jnp.exp(_freduce(p3, jnp.minimum)[None] - p3)
    ep = ep * _recip(_freduce(ep, jnp.add))[None]
    en = en * _recip(_freduce(en, jnp.add))[None]
    return jnp.concatenate([ep.reshape(GR, t), en.reshape(GR, t)], axis=0).astype(bf16)


def _b_schedule(a, b, c, d):
    nin = NP - (a + b + c + d)
    out, o = [], 0
    for t in range(NP):
        out.append(("Q", t))
        if t >= 1:
            out.append(("S", t - 1))
        if t >= 2:
            out.append(("P", t - 2))
        if t >= NP - nin:
            out.append(("O", o))
            o += 1
    out += [("O", o + i) for i in range(a)]
    out += [("S", NP - 1), ("P", NP - 2)]
    out += [("O", o + a + i) for i in range(b)]
    out += [("P", NP - 1)]
    out += [("O", o + a + b + i) for i in range(c)]
    if d:
        out.append(("M", NP - d))
    return out


def _kernel(x_hbm, wqkv_hbm, wphi_hbm, wo_hbm, mem_hbm, bq_hbm, bk_hbm, bv_hbm, bo_hbm,
            out_hbm,
            xin, wqkv_v, wphi_v, wo_v, mem_v, xa, xna, xnb, wq_s, wkv_s, ylast, kv_acc, kv_s, ot_s,
            stage, wb_s, bo_v, sv_o8, sv_e16, sems):
    bw_hbm = (bq_hbm, bk_hbm, bv_hbm)

    def whole(src, dst, slot):
        return pltpu.make_async_copy(src, dst, sems.at[slot])

    def x_copy(b):
        rows = pl.ds(pl.multiple_of(b * TA, TA), TA)
        return pltpu.make_async_copy(x_hbm.at[rows], xin.at[rows], sems.at[SEM_X + b])

    def w_start(q):
        t, j = divmod(q, NP)
        pltpu.make_async_copy(bw_hbm[t].at[pl.ds(j * PW, PW)], stage.at[q], sems.at[SEM_W + q]).start()

    def w_wait(q):
        pltpu.make_async_copy(stage.at[q], stage.at[q], sems.at[SEM_W + q]).wait()

    def out_copy(b):
        rows = pl.ds(pl.multiple_of(b * TB, TB), TB)
        return pltpu.make_async_copy(xin.at[rows], out_hbm.at[rows], sems.at[SEM_OUT])

    whole(wphi_hbm, wphi_v, SEM_PHI).start()
    whole(wqkv_hbm, wqkv_v, SEM_QKV).start()
    x_copy(0).start()
    for b in range(NB):
        if b + 1 < NB:
            x_copy(b + 1).start()
        for q in range(b * WPB, (b + 1) * WPB):
            w_start(q)
    whole(wo_hbm, wo_v, SEM_WO).start()
    whole(mem_hbm, mem_v, SEM_MEM).start()
    for q in range(NB * WPB, NW):
        w_start(q)
    whole(bo_hbm, bo_v, SEM_BO).start()

    whole(wphi_hbm, wphi_v, SEM_PHI).wait()
    row = lax.broadcasted_iota(i32, (AH, D), 0)
    col = lax.broadcasted_iota(i32, (AH, D), 1)
    dsel = col - AD * row
    wf = None
    for d in range(AD):
        y = _dot(wphi_v[d], (dsel == d).astype(bf16))
        wf = y if wf is None else y + wf
    wf = wf.astype(bf16)
    row = lax.broadcasted_iota(i32, (CR, AD), 0)
    col = lax.broadcasted_iota(i32, (CR, AD), 1)
    sel = (((row % GR) // 2) == col).astype(bf16)
    row = lax.broadcasted_iota(i32, (CR, 256), 0)
    col = lax.broadcasted_iota(i32, (CR, 256), 1)
    head = (row // GR) * 2 + row % 2
    phit = []
    for c in range(NC):
        rep = _dot(sel, wf[:, c * 128:c * 128 + 256])
        keep = (head + c * 2 * CG) == (col + c * 128) // AD
        phit.append(jnp.where(keep, rep, 0.0).astype(bf16))
    whole(wqkv_hbm, wqkv_v, SEM_QKV).wait()
    wvt = wqkv_v[:, 2 * D:3 * D].T
    for c in range(NC):
        wk = _dot_nt(phit[c], wqkv_v[:, D + c * 128:D + c * 128 + 256]).astype(bf16)
        wkv_s[c] = _pack(jnp.concatenate([wk, wvt[c * CR:(c + 1) * CR]], axis=0))
    for c in range(NC):
        wq_s[c] = _pack(_dot_nt(phit[c], wqkv_v[:, c * 128:c * 128 + 256]).astype(bf16))

    x_copy(0).wait()

    def layer_a(li):
        first = li == 0

        def transposes(n):
            for u in range(WPB):
                q = n * WPB + u
                wb_s[q] = _pack(stage[q].T)

        def waits(n):
            for u in range(WPB):
                w_wait(n * WPB + u)

        def x_in(rows):
            return xin[rows, :].astype(f32)

        def ln_block(b):
            rows = pl.ds(pl.multiple_of(b * TA, TA), TA)
            xna[rows, :] = _layernorm(x_in(rows)).astype(bf16)

        def kv_update(c, y, ones):
            for u in range(CG):
                phi = _hedgehog(y[u * GR:(u + 1) * GR])
                vt = jnp.concatenate([y[CR + u * GR:CR + (u + 1) * GR], ones], axis=0).astype(bf16)
                kv_acc[c * CG + u] += _dot_nt(vt, phi)

        def pass1(i, carry):
            nxt = jnp.minimum(i + 1, NB - 1)
            @pl.when(first)
            def _():
                @pl.when(i + 1 < NB)
                def _():
                    x_copy(i + 1).wait()
                waits(i)

            xn = xna[pl.ds(pl.multiple_of(i * TA, TA), TA), :]
            ones = jnp.ones((8, TA), f32)
            yprev = ylast[...]
            ys = {}
            for c in range(NC):
                ys[c] = _dot_nt(_unpack(wkv_s[c]), xn)
                if c == 0:
                    kv_update(NC - 1, yprev, jnp.where(i > 0, ones, 0.0))
                else:
                    kv_update(c - 1, ys.pop(c - 1), ones)
            ylast[...] = ys.pop(NC - 1)
            ln_block(nxt)
            transposes(i)
            return carry

        def front(i):
            xn = xna[pl.ds(pl.multiple_of(i * TA, TA), TA), :]
            sub = lax.broadcasted_iota(i32, (8, TA), 0) < 4

            def proj(c):
                return _dot_nt(_unpack(wq_s[c]), xn)

            def feat(c, p):
                for u in range(CG):
                    g = c * CG + u
                    y = _dot(kv_s[g], _hedgehog(p[u * GR:(u + 1) * GR]))
                    r = _recip(y[GR:] + 1e-6)
                    rr = pltpu.roll(r, 4, 0)
                    r0, r1 = jnp.where(sub, r, rr), jnp.where(sub, rr, r)
                    ot_s[g * GR:(g + 1) * GR, :] = y[:GR] * jnp.concatenate([r0, r0, r, r1, r1], axis=0)
            return proj, feat

        def back_load():
            return ot_s[...].T.astype(bf16)

        def back(i, o):
            rows = pl.ds(pl.multiple_of(i * TA, TA), TA)
            xa[rows, :] = x_in(rows) + _dot(o, wo_v[...])

        def pass2(i, has_back):
            if has_back:
                @pl.when(first)
                def _():
                    waits(NB + i)

            o = back_load() if has_back else None
            proj, feat = front(i)
            ps = {}
            for c in range(NC):
                ps[c] = proj(c)
                if c > 0:
                    feat(c - 1, ps.pop(c - 1))
            if has_back:
                back(i - 1, o)
            feat(NC - 1, ps.pop(NC - 1))
            transposes(NB + i)

        kv_acc[...] = jnp.zeros_like(kv_acc)
        ylast[...] = jnp.zeros_like(ylast)
        ln_block(0)
        lax.fori_loop(0, NB, pass1, 0)

        @pl.when(first)
        def _():
            whole(wo_hbm, wo_v, SEM_WO).wait()
            waits(NB)

        kv_update(NC - 1, ylast[...], jnp.ones((8, TA), f32))
        row = lax.broadcasted_iota(i32, (GR + 8, 2 * GR), 0)
        col = lax.broadcasted_iota(i32, (GR + 8, 2 * GR), 1)
        keep = jnp.where(row < GR, row // AD, (row - GR) // 4) == col % 2
        for g in range(NG):
            kv_s[g] = jnp.where(keep, kv_acc[g], 0.0).astype(bf16)
        pass2(0, False)

        def loop2(i, carry):
            pass2(i, True)
            return carry
        lax.fori_loop(1, NB, loop2, 0)
        back(NB - 1, back_load())
        xnb[...] = _layernorm(xa[0:64, :])

        @pl.when(first)
        def _():
            whole(mem_hbm, mem_v, SEM_MEM).wait()
            whole(bo_hbm, bo_v, SEM_BO).wait()

    def layer_b(li):
        def blockdiag(k):
            n = k.shape[0]
            lo = lax.broadcasted_iota(i32, (n, 128), 1) < 64
            zero = jnp.zeros((n, 128), f32)
            kmid = k[:, 128:256]
            top = jnp.concatenate([k[:, :128], jnp.where(lo, kmid, zero), zero], axis=1)
            bot = jnp.concatenate([zero, jnp.where(lo, zero, kmid), k[:, 256:]], axis=1)
            return jnp.concatenate([top, bot], axis=0).astype(bf16)

        r = lax.broadcasted_iota(i32, (32, 2 * L), 0)
        c = lax.broadcasted_iota(i32, (32, 2 * L), 1)
        isa_e = c < L
        key = jnp.where(isa_e, c, c - L)
        valid_e = (r < M) | (r + 8 >= key)
        r = lax.broadcasted_iota(i32, (48, 112), 0)
        c = lax.broadcasted_iota(i32, (48, 112), 1)
        isa_o = c < 56
        key = jnp.where(isa_o, c, c - 56)
        valid_o = ((r < L) & (key < L) & ((r < M) | (r >= key))) | ((r >= L) & (key >= L) & (r + 8 >= key))

        def softmax(s, valid, isa):
            s = jnp.where(valid, s * SCALE, -1e9)
            ma = jnp.max(jnp.where(isa, s, -jnp.inf), axis=1, keepdims=True)
            mb = jnp.max(jnp.where(isa, -jnp.inf, s), axis=1, keepdims=True)
            e = jnp.exp(s - jnp.where(isa, ma, mb))
            la = jnp.sum(jnp.where(isa, e, 0.0), axis=1, keepdims=True)
            lb = jnp.sum(jnp.where(isa, 0.0, e), axis=1, keepdims=True)
            return (e * _recip(jnp.where(isa, la, lb))).astype(bf16)

        def step(hq, hkv, even, first, last):
            qs, kvs, ps, os_ = {}, {}, {}, {}
            acc = None
            tail = (3, 4, 3, 0) if last else ((3, 4, 2, 3) if even else (3, 3, 2, 3))
            for op, j in _b_schedule(*tail):
                if op == "Q":
                    order = (0, 1, 2) if even else (1, 2, 0)
                    part, k0 = {}, 0
                    for k1 in ((2, 3, 5) if (j == 0 and not first) else (5,)):
                        for t in order:
                            h = hq if t == 0 else hkv
                            y = _dot(h[:, k0 * 128:k1 * 128], _unpack(wb_s[t * NP + j, k0 * 64:k1 * 64, :]))
                            part[t] = y + part[t] if t in part else y
                        k0 = k1
                    qs[j] = part[0].astype(bf16)
                    for t in (1, 2):
                        cols = slice((t - 1) * PW, t * PW)
                        y = part[t]
                        if even:
                            sv_o8[j, :, cols] = y[40:48]
                            sv_e16[j, :, cols] = y[0:16]
                            y = y[:40]
                        else:
                            y = jnp.concatenate([y[:8], sv_o8[j, :, cols], y[8:], sv_e16[j, :, cols]], axis=0)
                        kvs[t, j] = blockdiag(y)
                elif op == "S":
                    s = _dot_nt(qs.pop(j), kvs.pop((1, j)))
                    ps[j] = softmax(s, valid_e, isa_e) if even else softmax(s, valid_o, isa_o)
                elif op == "P":
                    os_[j] = _dot(ps.pop(j), kvs.pop((2, j))).astype(bf16)
                elif op == "M":
                    o = jnp.concatenate([os_.pop(jj) for jj in range(j, NP)], axis=1)
                    acc = _dot(o, bo_v[j * PW:, :]) + acc
                else:
                    y = _dot(os_.pop(j), bo_v[j * PW:(j + 1) * PW, :])
                    acc = y if acc is None else y + acc
            return acc

        def body(i, mem):
            for u in range(UB):
                r0 = pl.multiple_of((i * UB + u) * 64, 64)
                xn = xnb[...] if u == 0 else _layernorm(xa[pl.ds(r0, 64), :])
                hkv = jnp.concatenate([mem, xn[0:40]], axis=0).astype(bf16)
                hq = jnp.concatenate([mem, xn[8:32]], axis=0).astype(bf16)
                ye = step(hq, hkv, True, u == 0, False)
                mem = ye[:8]
                xin[pl.ds(r0 + 16, 16), :] = (xa[pl.ds(r0 + 16, 16), :] + ye[16:]).astype(bf16)
                hkv = jnp.concatenate([mem, xn[40:64]], axis=0).astype(bf16)
                hq = jnp.concatenate([mem, xn[32:64], xn[0:8]], axis=0).astype(bf16)
                yo = step(hq, hkv, False, False, u == UB - 1)
                mem = yo[:8]
                y = jnp.concatenate([yo[40:48], ye[8:16]], axis=0)
                xin[pl.ds(r0, 16), :] = (xa[pl.ds(r0, 16), :] + y).astype(bf16)
                xin[pl.ds(r0 + 32, 32), :] = (xa[pl.ds(r0 + 32, 32), :] + yo[8:40]).astype(bf16)
            rn = pl.multiple_of(jnp.minimum(i + 1, NI - 1) * TB, TB)
            xnb[...] = _layernorm(xa[pl.ds(rn, 64), :])

            @pl.when(li == 1)
            def _():
                out_copy(i).start()
            return mem

        lax.fori_loop(0, NI, body, mem_v[...].astype(f32))

    def layer(li, carry):
        layer_a(li)
        layer_b(li)
        return carry

    lax.fori_loop(0, 2, layer, 0)
    pltpu.make_async_copy(xin, out_hbm, sems.at[SEM_OUT]).wait()


@functools.partial(jax.jit, static_argnames=("B_seg_len",))
def pallas_interleave_layers__linear_kernel_hedgehog__memory_aug_recurrent_mem_tr__prompt_kernel(
    A_x: jax.Array,
    A_wqkv: jax.Array,
    A_w_phi: jax.Array,
    A_wo: jax.Array,
    B_x: jax.Array,
    B_mem0: jax.Array,
    B_Wq: jax.Array,
    B_Wk: jax.Array,
    B_Wv: jax.Array,
    B_Wo: jax.Array,
    B_seg_len=SEG,
):
    assert B_seg_len == SEG
    x = A_x.reshape(S, D)
    wphi = A_w_phi.transpose(1, 2, 0)
    mem0 = B_mem0.reshape(M, D)
    bq = B_Wq.transpose(1, 2, 0).reshape(HE, D)
    bk = B_Wk.transpose(1, 2, 0).reshape(HE, D)
    bv = B_Wv.transpose(1, 2, 0).reshape(HE, D)
    bo = B_Wo.reshape(HE, D)

    anyspec = pl.BlockSpec(memory_space=pl.ANY)
    out = pl.pallas_call(
        _kernel,
        out_shape=jax.ShapeDtypeStruct((S, D), bf16),
        in_specs=[anyspec] * 9,
        out_specs=anyspec,
        scratch_shapes=[
            pltpu.VMEM((S, D), bf16),
            pltpu.VMEM((D, 3 * D), bf16),
            pltpu.VMEM((AD, AD, AH), bf16),
            pltpu.VMEM((D, D), bf16),
            pltpu.VMEM((M, D), bf16),
            pltpu.VMEM((S, D), f32),
            pltpu.VMEM((S, D), bf16),
            pltpu.VMEM((64, D), f32),
            pltpu.VMEM((NC, CR // 2, D), u32),
            pltpu.VMEM((NC, CR, D), u32),
            pltpu.VMEM((2 * CR, TA), f32),
            pltpu.VMEM((NG, GR + 8, 2 * GR), f32),
            pltpu.VMEM((NG, GR + 8, 2 * GR), bf16),
            pltpu.VMEM((D, TA), f32),
            pltpu.VMEM((NW, PW, D), bf16),
            pltpu.VMEM((NW, D // 2, PW), u32),
            pltpu.VMEM((HE, D), bf16),
            pltpu.VMEM((NP, 8, 2 * PW), f32),
            pltpu.VMEM((NP, 16, 2 * PW), f32),
            pltpu.SemaphoreType.DMA((NSEM,)),
        ],
        compiler_params=pltpu.CompilerParams(vmem_limit_bytes=110 * 1024 * 1024),
    )(x, A_wqkv, wphi, A_wo, mem0, bq, bk, bv, bo)
    return out.reshape(1, S, D)
```

```python
import functools

import jax
import jax.numpy as jnp
from jax import lax
import jax.experimental.pallas as pl
import jax.experimental.pallas.tpu as pltpu

bf16 = jnp.bfloat16
f32 = jnp.float32
u32 = jnp.uint32
i32 = jnp.int32

CFG = dict(
    TA=512, TS1=128, TS2=256, W1=2, F1=1, F2=2,
    pe="q0 k0 v0 S1 P2", po="v0 P3 S1 k0 q0",
    te=(3, 4, 2, 3), to=(2, 3, 2, 1, 3), tl=(3, 3, 2, 2, 0), UB=2,
)
CFG.update(arr=1, wot=1, po='q0 S1 k0 v0 P3', W1=0)

S = 2048
D = 640
AH = 32
AD = 20
GR = 2 * AD
NG = AH // 2
CG = 4
CR = CG * GR
NC = NG // CG
TA = CFG["TA"]
TS1 = CFG["TS1"]
TS2 = CFG["TS2"]
NB = S // TA
BH = 32
BE = 192
HE = BH * BE
M = 8
SEG = 32
L = M + SEG
NP = BH // 2
PW = 2 * BE
SCALE = BE ** -0.5
UB = CFG["UB"]
TB = 64 * UB
NI = S // TB
NW = 3 * NP
W1 = CFG["W1"]
W2 = NW // NB - W1

NT = (((1,), (1,)), ((), ()))

SEM_PHI, SEM_QKV, SEM_X0, SEM_BO, SEM_OUT = 0, 1, 2, 3, 4
SEM_IT = 5
NSEM = SEM_IT + 2 * NB


def _dot(a, b):
    return jnp.dot(a, b, preferred_element_type=f32)


def _dot_nt(a, b):
    return lax.dot_general(a, b, NT, preferred_element_type=f32)


def _pack(x):
    return pltpu.bitcast(x, u32)


def _unpack(x):
    return pltpu.bitcast(x, bf16)


def _recip(x):
    r = pl.reciprocal(x, approx=True)
    return r * (2.0 - x * r)


def _layernorm(x):
    m = jnp.mean(x, axis=-1, keepdims=True)
    xc = x - m
    v = jnp.mean(xc * xc, axis=-1, keepdims=True)
    return xc * lax.rsqrt(v + 1e-5)


def _freduce(x3, op):
    r = op(op(op(x3[0], x3[1]), op(x3[2], x3[3])), x3[4])
    r = op(r, pltpu.roll(r, 2, 0))
    return op(r, pltpu.roll(r, 4, 0))


def _hedgehog(p):
    t = p.shape[1]
    p3 = p.reshape(GR // 8, 8, t)
    ep = jnp.exp(p3 - _freduce(p3, jnp.maximum)[None])
    en = jnp.exp(_freduce(p3, jnp.minimum)[None] - p3)
    ep = ep * _recip(_freduce(ep, jnp.add))[None]
    en = en * _recip(_freduce(en, jnp.add))[None]
    return jnp.concatenate([ep.reshape(GR, t), en.reshape(GR, t)], axis=0).astype(bf16)


def _b_schedule(period, tail):
    ops = [(t[0], int(t[1:])) for t in period.split()]
    maxlag = max(lag for _, lag in ops)
    merged, tail = tail[-1], tail[:-1]
    assert len(tail) == maxlag + 1
    nin = NP - sum(tail) - merged
    out, o = [], 0
    for t in range(NP + maxlag + 1):
        if t >= NP:
            out += [("O", o + i) for i in range(tail[t - NP])]
            o += tail[t - NP]
        out += [(op, t - lag) for op, lag in ops if 0 <= t - lag < NP]
        if NP - nin <= t < NP:
            out.append(("O", o))
            o += 1
    if merged:
        out.append(("M", o))
    return out


def _kernel(x_hbm, wqkv_hbm, wphi_hbm, wo_hbm, mem_hbm, bq_hbm, bk_hbm, bv_hbm, bo_hbm,
            out_hbm,
            xin, wqkv_v, wphi_v, wo_v, mem_v, xa, xna, xnb, wq_s, wkv_s, ylast, kv_acc, kv_s,
            stage, wb_s, bo_v, sv_o8, sv_e16, sv_mo, sv_q, sems):
    bw_hbm = (bq_hbm, bk_hbm, bv_hbm)

    def copy(src, dst, slot):
        return pltpu.make_async_copy(src, dst, sems.at[slot])

    def w_copy(q, slot):
        t, j = divmod(q, NP)
        return copy(bw_hbm[t].at[pl.ds(j * PW, PW)], stage.at[q], slot)

    def x_copy(r0, n, slot):
        return copy(x_hbm.at[pl.ds(r0, n)], xin.at[pl.ds(r0, n)], slot)

    def w_first(n):
        return n * W1 if isinstance(n, int) and n <= NB else NB * W1 + (n - NB) * W2

    def out_copy(b):
        rows = pl.ds(pl.multiple_of(b * TB, TB), TB)
        return copy(xin.at[rows], out_hbm.at[rows], SEM_OUT)

    copy(wphi_hbm, wphi_v, SEM_PHI).start()
    copy(wqkv_hbm, wqkv_v, SEM_QKV).start()
    x_copy(0, TS1, SEM_X0).start()
    for b in range(NB):
        x_copy(b * TA + TS1, TA if b + 1 < NB else TA - TS1, SEM_IT + b).start()
        for q in range(b * W1, (b + 1) * W1):
            w_copy(q, SEM_IT + b).start()
    copy(wo_hbm, wo_v, SEM_IT + NB).start()
    for b in range(NB):
        for q in range(NB * W1 + b * W2, NB * W1 + (b + 1) * W2):
            w_copy(q, SEM_IT + NB + b).start()
    copy(mem_hbm, mem_v, SEM_BO).start()
    if CFG.get("wot", 0):
        for n in range(5):
            copy(bo_hbm.at[:, pl.ds(n * 128, 128)], bo_v.at[n], SEM_BO).start()
    else:
        copy(bo_hbm, bo_v, SEM_BO).start()

    copy(wphi_hbm, wphi_v, SEM_PHI).wait()
    row = lax.broadcasted_iota(i32, (AH, D), 0)
    col = lax.broadcasted_iota(i32, (AH, D), 1)
    dsel = col - AD * row
    wf = None
    for d in range(AD):
        y = _dot(wphi_v[d], (dsel == d).astype(bf16))
        wf = y if wf is None else y + wf
    wf = wf.astype(bf16)
    row = lax.broadcasted_iota(i32, (CR, AD), 0)
    col = lax.broadcasted_iota(i32, (CR, AD), 1)
    sel = (((row % GR) // 2) == col).astype(bf16)
    row = lax.broadcasted_iota(i32, (CR, 256), 0)
    col = lax.broadcasted_iota(i32, (CR, 256), 1)
    head = (row // GR) * 2 + row % 2
    phit = []
    for c in range(NC):
        rep = _dot(sel, wf[:, c * 128:c * 128 + 256])
        keep = (head + c * 2 * CG) == (col + c * 128) // AD
        phit.append(jnp.where(keep, rep, 0.0).astype(bf16))
    copy(wqkv_hbm, wqkv_v, SEM_QKV).wait()
    wvt = wqkv_v[:, 2 * D:3 * D].T
    for c in range(NC):
        wk = _dot_nt(phit[c], wqkv_v[:, D + c * 128:D + c * 128 + 256]).astype(bf16)
        wkv_s[c] = _pack(jnp.concatenate([wk, wvt[c * CR:(c + 1) * CR]], axis=0))
    for c in range(NC):
        wq_s[c] = _pack(_dot_nt(phit[c], wqkv_v[:, c * 128:c * 128 + 256]).astype(bf16))

    x_copy(0, TS1, SEM_X0).wait()

    def layer_a(li):
        first = li == 0

        def transposes(q0, n):
            for u in range(n):
                wb_s[q0 + u] = _pack(stage[q0 + u].T)

        def w_wait(q0, n, slot):
            copy(stage.at[pl.ds(q0, n)], stage.at[pl.ds(q0, n)], slot).wait()

        def ln_rows(r0, n):
            rows = pl.ds(pl.multiple_of(r0, n), n)
            xn = _layernorm(xin[rows, :].astype(f32)).astype(bf16)
            xna[pl.ds(pl.multiple_of(r0 // 2, n // 2), n // 2), :] = _pack(xn)
            return xn

        def xn_rows(r0, n):
            return _unpack(xna[pl.ds(pl.multiple_of(r0 // 2, n // 2), n // 2), :])

        def kv_update(c, y, ones):
            for u in range(CG):
                phi = _hedgehog(y[u * GR:(u + 1) * GR])
                vt = jnp.concatenate([y[CR + u * GR:CR + (u + 1) * GR], ones], axis=0).astype(bf16)
                kv_acc[c * CG + u] += _dot_nt(vt, phi)

        def pass1(i, carry):
            @pl.when(first)
            def _():
                @pl.when(i + 1 < NB)
                def _():
                    x_copy(0, TA, SEM_IT + i).wait()

                @pl.when(i + 1 == NB)
                def _():
                    x_copy(0, TA - TS1, SEM_IT + i).wait()
                w_wait(i * W1, W1, SEM_IT + i)

            ones = jnp.ones((8, TS1), f32)
            pend = (NC - 1, ylast[...], jnp.where(i > 0, ones, 0.0))
            for s in range(TA // TS1):
                r0 = i * TA + s * TS1
                xn = xn_rows(r0, TS1) if s == 0 else ln_rows(r0, TS1)
                for c in range(NC):
                    y = _dot_nt(_unpack(wkv_s[c]), xn)
                    kv_update(*pend)
                    pend = (c, y, ones)
            ylast[...] = pend[1]
            ln_rows(jnp.minimum(i + 1, NB - 1) * TA, TS1)
            transposes(i * W1, W1)
            return carry

        def pass2(i, carry):
            @pl.when(first)
            def _():
                @pl.when(i == 0)
                def _():
                    copy(wo_hbm, wo_v, SEM_IT + NB).wait()
                w_wait(NB * W1 + i * W2, W2, SEM_IT + NB + i)

            sub = lax.broadcasted_iota(i32, (8, TS2), 0) < 4
            ns = TA // TS2
            ot = {}

            def feat(s, c, p):
                for u in range(CG):
                    g = c * CG + u
                    y = _dot(kv_s[g], _hedgehog(p[u * GR:(u + 1) * GR]))
                    r = _recip(y[GR:] + 1e-6)
                    rr = pltpu.roll(r, 4, 0)
                    r0, r1 = jnp.where(sub, r, rr), jnp.where(sub, rr, r)
                    ot[s, g] = y[:GR] * jnp.concatenate([r0, r0, r, r1, r1], axis=0)

            def back(s, lo, hi):
                o = jnp.concatenate([ot[s, g][:, lo:hi] for g in range(NG)], axis=0).T.astype(bf16)
                rows = pl.ds(pl.multiple_of(i * TA + s * TS2 + lo, hi - lo), hi - lo)
                xa[rows, :] = xin[rows, :].astype(f32) + _dot(o, wo_v[...])

            pend = []
            for s in range(ns):
                xn = xn_rows(i * TA + s * TS2, TS2)
                for c in range(NC):
                    pend.append((s, c, _dot_nt(_unpack(wq_s[c]), xn)))
                    if len(pend) > CFG["F2"]:
                        feat(*pend.pop(0))
                if 1 <= s < ns - 1:
                    back(s - 1, 0, TS2)
            half = TS2 // 2 if TS2 > 128 else TS2
            back(ns - 2, 0, half)
            while pend:
                feat(*pend.pop(0))
            if half < TS2:
                back(ns - 2, half, TS2)
            back(ns - 1, 0, TS2)
            transposes(NB * W1 + i * W2, W2)
            return carry

        kv_acc[...] = jnp.zeros_like(kv_acc)
        ylast[...] = jnp.zeros_like(ylast)
        ln_rows(0, TS1)
        lax.fori_loop(0, NB, pass1, 0)
        kv_update(NC - 1, ylast[...], jnp.ones((8, TS1), f32))
        row = lax.broadcasted_iota(i32, (GR + 8, 2 * GR), 0)
        col = lax.broadcasted_iota(i32, (GR + 8, 2 * GR), 1)
        keep = jnp.where(row < GR, row // AD, (row - GR) // 4) == col % 2
        for g in range(NG):
            kv_s[g] = jnp.where(keep, kv_acc[g], 0.0).astype(bf16)
        lax.fori_loop(0, NB, pass2, 0)
        xnb[...] = _layernorm(xa[0:64, :])

        @pl.when(first)
        def _():
            copy(mem_hbm, mem_v, SEM_BO).wait()
            copy(bo_v, bo_v, SEM_BO).wait()

    def layer_b(li):
        def blockdiag(k):
            n = k.shape[0]
            lo = lax.broadcasted_iota(i32, (n, 128), 1) < 64
            zero = jnp.zeros((n, 128), f32)
            kmid = k[:, 128:256]
            top = jnp.concatenate([k[:, :128], jnp.where(lo, kmid, zero), zero], axis=1)
            bot = jnp.concatenate([zero, jnp.where(lo, zero, kmid), k[:, 256:]], axis=1)
            return jnp.concatenate([top, bot], axis=0).astype(bf16)

        r = lax.broadcasted_iota(i32, (32, 2 * L), 0)
        c = lax.broadcasted_iota(i32, (32, 2 * L), 1)
        isa_e = c < L
        key = jnp.where(isa_e, c, c - L)
        valid_e = (r < M) | (r + 8 >= key)
        r = lax.broadcasted_iota(i32, (48, 112), 0)
        c = lax.broadcasted_iota(i32, (48, 112), 1)
        if CFG.get("arr", 0):
            isa_o = (c < L) | ((c >= 2 * L) & (c < 2 * L + 16))
            key = jnp.where(c < L, c, jnp.where(c < 2 * L + 16, c - L, c - L - 16))
        else:
            isa_o = c < 56
            key = jnp.where(isa_o, c, c - 56)
        pos = jnp.where(r < 32, r + 8, r - 24)
        valid_o = ((r < L) & (key < L) & ((r < M) | (pos >= key))) | ((r >= L) & (key >= L) & (r + 8 >= key))
        lane = lax.broadcasted_iota(i32, (8, 128), 1)
        lo16 = lax.broadcasted_iota(i32, (16, 128), 1) < 64

        def head8_scores(jq, r0, rows, c0, cb_off):
            q0, qa, qb, q2 = [sv_q[jq, r0:r0 + 8, cb * 128:(cb + 1) * 128] for cb in range(4)]
            s = jnp.zeros((8, 128), f32)
            for t, (ref, j, rr) in enumerate(rows):
                kb = [jnp.broadcast_to(ref[j, rr:rr + 1, cb * 128:(cb + 1) * 128], (8, 128)) for cb in range(3)]
                sa = jnp.sum(q0 * kb[0] + qa * kb[1], axis=1, keepdims=True)
                sb = jnp.sum(q2 * kb[2] + qb * kb[1], axis=1, keepdims=True)
                s = jnp.where(lane == c0 + t, sa, s)
                s = jnp.where(lane == c0 + t + cb_off, sb, s)
            return s[:, :112]

        def softmax(s, valid, isa):
            s = jnp.where(valid, s * SCALE, -1e9)
            ma = jnp.max(jnp.where(isa, s, -jnp.inf), axis=1, keepdims=True)
            mb = jnp.max(jnp.where(isa, -jnp.inf, s), axis=1, keepdims=True)
            e = jnp.exp(s - jnp.where(isa, ma, mb))
            la = jnp.sum(jnp.where(isa, e, 0.0), axis=1, keepdims=True)
            lb = jnp.sum(jnp.where(isa, 0.0, e), axis=1, keepdims=True)
            return (e * _recip(jnp.where(isa, la, lb))).astype(bf16)

        def wo_rows(a, b):
            if CFG.get("wot", 0):
                return jnp.concatenate([bo_v[n, a:b, :] for n in range(5)], axis=1)
            return bo_v[a:b, :]

        def step(hq, hkv, even, first, last, qslot):
            sched = _b_schedule(CFG["pe"] if even else CFG["po"],
                                CFG["tl"] if last else (CFG["te"] if even else CFG["to"]))
            widx = dict(q=0, k=NP, v=2 * NP)

            def proj(op, j, k0, k1):
                h = hq if op == "q" else hkv
                return _dot(h[:, k0 * 128:k1 * 128], _unpack(wb_s[widx[op] + j, k0 * 64:k1 * 64, :]))

            part, kdone = {}, 0
            for k1 in (() if first else (2, 3)):
                for op in [op for op, j in sched if op in widx and j == 0]:
                    y = proj(op, 0, kdone, k1)
                    part[op] = y + part[op] if op in part else y
                kdone = k1

            val, acc = {}, None
            for op, j in sched:
                if op in widx:
                    y = proj(op, j, kdone, 5) + part[op] if (j == 0 and part) else proj(op, j, 0, 5)
                    if op == "q":
                        val["q", j] = y[:32].astype(bf16)
                        if not even:
                            qm = y[32:, 128:256]
                            sv_q[qslot + j] = jnp.concatenate(
                                [y[32:, :128], jnp.where(lo16, qm, 0.0), jnp.where(lo16, 0.0, qm), y[32:, 256:]], axis=1)
                        continue
                    cols = slice(0, PW) if op == "k" else slice(PW, 2 * PW)
                    if even:
                        sv_o8[j, :, cols] = y[40:48]
                        sv_e16[j, :, cols] = y[0:16]
                        y = y[:40]
                    elif CFG.get("arr", 0):
                        if op == "k":
                            sv_mo[j] = y[:8]
                        main = blockdiag(jnp.concatenate([y[:8], sv_o8[j, :, cols], y[8:]], axis=0))
                        extra = jnp.zeros((32, PW), bf16) if op == "k" else blockdiag(sv_e16[j, :, cols])
                        val[op, j] = jnp.concatenate([main, extra], axis=0)
                        continue
                    elif op == "k":
                        sv_mo[j] = y[:8]
                        y = jnp.concatenate([y[:8], sv_o8[j, :, cols], y[8:], jnp.zeros((16, PW), f32)], axis=0)
                    else:
                        y = jnp.concatenate([y[:8], sv_o8[j, :, cols], y[8:], sv_e16[j, :, cols]], axis=0)
                    val[op, j] = blockdiag(y)
                elif op == "S":
                    s = _dot_nt(val.pop(("q", j)), val.pop(("k", j)))
                    if even:
                        val["p", j] = softmax(s, valid_e, isa_e)
                    else:
                        so = head8_scores(qslot + j, 0, [(sv_mo, j, t) for t in range(8)]
                                          + [(sv_o8, j, t) for t in range(8)], 0, L if CFG.get('arr', 0) else 56)
                        se = head8_scores(qslot + j, 8, [(sv_e16, j, t) for t in range(16)], *((2 * L, 16) if CFG.get('arr', 0) else (L, 56)))
                        val["p", j] = softmax(jnp.concatenate([s, so, se], axis=0), valid_o, isa_o)
                elif op == "P":
                    val["o", j] = _dot(val.pop(("p", j)), val.pop(("v", j))).astype(bf16)
                elif op == "M":
                    o = jnp.concatenate([val.pop(("o", jj)) for jj in range(j, NP)], axis=1)
                    acc = _dot(o, wo_rows(j * PW, HE)) + acc
                else:
                    y = _dot(val.pop(("o", j)), wo_rows(j * PW, (j + 1) * PW))
                    acc = y if acc is None else y + acc
            return acc

        def body(i, mem):
            qslot = (i % 2) * NP
            for u in range(UB):
                r0 = pl.multiple_of((i * UB + u) * 64, 64)

                def add_rows(off, y):
                    rows = pl.ds(r0 + off, y.shape[0])
                    xin[rows, :] = (xa[rows, :] + y).astype(bf16)

                xn = xnb[...] if u == 0 else _layernorm(xa[pl.ds(r0, 64), :])
                hkv = jnp.concatenate([mem, xn[0:40]], axis=0).astype(bf16)
                hq = jnp.concatenate([mem, xn[8:32]], axis=0).astype(bf16)
                ye = step(hq, hkv, True, u == 0, False, qslot)
                mem = ye[:8]
                add_rows(16, ye[16:])
                hq = jnp.concatenate([mem, xn[40:64], xn[32:40], xn[0:8]], axis=0).astype(bf16)
                yo = step(hq, hq[:32], False, False, u == UB - 1, qslot)
                mem = yo[:8]
                add_rows(48, yo[16:32])
                add_rows(32, jnp.concatenate([yo[32:40], yo[8:16]], axis=0))
                add_rows(0, jnp.concatenate([yo[40:48], ye[8:16]], axis=0))
            rn = pl.multiple_of(jnp.minimum(i + 1, NI - 1) * TB, TB)
            xnb[...] = _layernorm(xa[pl.ds(rn, 64), :])

            @pl.when(li == 1)
            def _():
                out_copy(i).start()
            return mem

        lax.fori_loop(0, NI, body, mem_v[...].astype(f32))

    def layer(li, carry):
        if not CFG.get("noA"):
            layer_a(li)
        if not CFG.get("noB"):
            layer_b(li)
        return carry

    lax.fori_loop(0, 2, layer, 0)
    copy(xin, out_hbm, SEM_OUT).wait()


@functools.partial(jax.jit, static_argnames=("B_seg_len",))
def pallas_interleave_layers__linear_kernel_hedgehog__memory_aug_recurrent_mem_tr__prompt_kernel(
    A_x: jax.Array,
    A_wqkv: jax.Array,
    A_w_phi: jax.Array,
    A_wo: jax.Array,
    B_x: jax.Array,
    B_mem0: jax.Array,
    B_Wq: jax.Array,
    B_Wk: jax.Array,
    B_Wv: jax.Array,
    B_Wo: jax.Array,
    B_seg_len=SEG,
):
    assert B_seg_len == SEG
    x = A_x.reshape(S, D)
    wphi = A_w_phi.transpose(1, 2, 0)
    mem0 = B_mem0.reshape(M, D)
    bq = B_Wq.transpose(1, 2, 0).reshape(HE, D)
    bk = B_Wk.transpose(1, 2, 0).reshape(HE, D)
    bv = B_Wv.transpose(1, 2, 0).reshape(HE, D)
    bo = B_Wo.reshape(HE, D)

    anyspec = pl.BlockSpec(memory_space=pl.ANY)
    out = pl.pallas_call(
        _kernel,
        out_shape=jax.ShapeDtypeStruct((S, D), bf16),
        in_specs=[anyspec] * 9,
        out_specs=anyspec,
        scratch_shapes=[
            pltpu.VMEM((S, D), bf16),
            pltpu.VMEM((D, 3 * D), bf16),
            pltpu.VMEM((AD, AD, AH), bf16),
            pltpu.VMEM((D, D), bf16),
            pltpu.VMEM((M, D), bf16),
            pltpu.VMEM((S, D), f32),
            pltpu.VMEM((S // 2, D), u32),
            pltpu.VMEM((64, D), f32),
            pltpu.VMEM((NC, CR // 2, D), u32),
            pltpu.VMEM((NC, CR, D), u32),
            pltpu.VMEM((2 * CR, TS1), f32),
            pltpu.VMEM((NG, GR + 8, 2 * GR), f32),
            pltpu.VMEM((NG, GR + 8, 2 * GR), bf16),
            pltpu.VMEM((NW, PW, D), bf16),
            pltpu.VMEM((NW, D // 2, PW), u32),
            pltpu.VMEM((5, HE, 128) if CFG.get('wot', 0) else (HE, D), bf16),
            pltpu.VMEM((NP, 8, 2 * PW), f32),
            pltpu.VMEM((NP, 16, 2 * PW), f32),
            pltpu.VMEM((NP, 8, PW), f32),
            pltpu.VMEM((2 * NP, 16, 512), f32),
            pltpu.SemaphoreType.DMA((NSEM,)),
        ],
        compiler_params=pltpu.CompilerParams(vmem_limit_bytes=110 * 1024 * 1024,
                                             disable_bounds_checks=True),
    )(x, A_wqkv, wphi, A_wo, mem0, bq, bk, bv, bo)
    return out.reshape(1, S, D)
```

```python
import functools

import jax
import jax.numpy as jnp
from jax import lax
import jax.experimental.pallas as pl
import jax.experimental.pallas.tpu as pltpu

bf16 = jnp.bfloat16
f32 = jnp.float32
u32 = jnp.uint32
i32 = jnp.int32

CFG = dict(
    TA=512, TS1=128, TS2=256, W1=4, F1=1, F2=2,
    pe="q0 k0 v0 S1 P2", po="q0 S1 k0 v0 P3", de=1, do=0, dyn=0,
    te=(3, 4, 2, 3), to=(2, 2, 1, 1, 2), tl=(2, 2, 1, 2, 0), UB=2,
)

S = 2048
D = 640
AH = 32
AD = 20
GR = 2 * AD
NG = AH // 2
CG = 4
CR = CG * GR
NC = NG // CG
TA = CFG["TA"]
TS1 = CFG["TS1"]
TS2 = CFG["TS2"]
NB = S // TA
BH = 32
BE = 192
HE = BH * BE
M = 8
SEG = 32
L = M + SEG
NP = BH // 2
PW = 2 * BE
SCALE = BE ** -0.5
UB = CFG["UB"]
TB = 64 * UB
NI = S // TB
NW = 3 * NP
W1 = CFG["W1"]
W2 = NW // NB - W1

NT = (((1,), (1,)), ((), ()))

SEM_PHI, SEM_QKV, SEM_X0, SEM_BO, SEM_OUT = 0, 1, 2, 3, 4
SEM_IT = 5
NSEM = SEM_IT + 2 * NB


def _dot(a, b):
    return jnp.dot(a, b, preferred_element_type=f32)


def _dot_nt(a, b):
    return lax.dot_general(a, b, NT, preferred_element_type=f32)


def _pack(x):
    return pltpu.bitcast(x, u32)


def _unpack(x):
    return pltpu.bitcast(x, bf16)


def _recip(x):
    r = pl.reciprocal(x, approx=True)
    return r * (2.0 - x * r)


def _layernorm(x):
    m = jnp.mean(x, axis=-1, keepdims=True)
    xc = x - m
    v = jnp.mean(xc * xc, axis=-1, keepdims=True)
    return xc * lax.rsqrt(v + 1e-5)


def _freduce(x3, op):
    r = op(op(op(x3[0], x3[1]), op(x3[2], x3[3])), x3[4])
    r = op(r, pltpu.roll(r, 2, 0))
    return op(r, pltpu.roll(r, 4, 0))


def _hedgehog(p):
    t = p.shape[1]
    p3 = p.reshape(GR // 8, 8, t)
    ep = jnp.exp(p3 - _freduce(p3, jnp.maximum)[None])
    en = jnp.exp(_freduce(p3, jnp.minimum)[None] - p3)
    ep = ep * _recip(_freduce(ep, jnp.add))[None]
    en = en * _recip(_freduce(en, jnp.add))[None]
    return jnp.concatenate([ep.reshape(GR, t), en.reshape(GR, t)], axis=0).astype(bf16)


def _b_schedule(period, tail):
    ops = [(t[0], int(t[1:])) for t in period.split()]
    maxlag = max(lag for _, lag in ops)
    merged, tail = tail[-1], tail[:-1]
    assert len(tail) == maxlag + 1
    nin = NP - sum(tail) - merged
    out, o = [], 0
    for t in range(NP + maxlag + 1):
        if t >= NP:
            out += [("O", o + i) for i in range(tail[t - NP])]
            o += tail[t - NP]
        out += [(op, t - lag) for op, lag in ops if 0 <= t - lag < NP]
        if NP - nin <= t < NP:
            out.append(("O", o))
            o += 1
    if merged:
        out.append(("M", o))
    return out


def _kernel(x_hbm, wqkv_hbm, wphi_hbm, wo_hbm, mem_hbm, bq_hbm, bk_hbm, bv_hbm, bo_hbm,
            out_hbm,
            xin, wqkv_v, wphi_v, wo_v, mem_v, xa, xna, xnb, wq_s, wkv_s, ylast, kv_acc, kv_s,
            stage, wbq_s, wbkv_s, bo_v, sv_o16, sv_e16, sv_q, sems):
    bw_hbm = (bq_hbm, bk_hbm, bv_hbm)

    def copy(src, dst, slot):
        return pltpu.make_async_copy(src, dst, sems.at[slot])

    def w_start(q, slot):
        t, j = divmod(q, NP)
        if t < 2:
            copy(bw_hbm[t].at[j], stage.at[q], slot).start()
        else:
            for hh in range(2):
                copy(bv_hbm.at[2 * j + hh], stage.at[q, :, hh], slot).start()

    def x_copy(r0, n, slot):
        return copy(x_hbm.at[pl.ds(r0, n)], xin.at[pl.ds(r0, n)], slot)

    def w_first(n):
        return n * W1 if isinstance(n, int) and n <= NB else NB * W1 + (n - NB) * W2

    def out_copy(b):
        rows = pl.ds(pl.multiple_of(b * TB, TB), TB)
        return copy(xin.at[rows], out_hbm.at[rows], SEM_OUT)

    copy(wphi_hbm, wphi_v, SEM_PHI).start()
    copy(wqkv_hbm, wqkv_v, SEM_QKV).start()
    x_copy(0, TS1, SEM_X0).start()
    for b in range(NB):
        x_copy(b * TA + TS1, TA if b + 1 < NB else TA - TS1, SEM_IT + b).start()
        for q in range(b * W1, (b + 1) * W1):
            w_start(q, SEM_IT + b)
    copy(wo_hbm, wo_v, SEM_IT + NB).start()
    for b in range(NB):
        for q in range(NB * W1 + b * W2, NB * W1 + (b + 1) * W2):
            w_start(q, SEM_IT + NB + b)
    if CFG.get("wot", 0):
        for n in range(5):
            copy(bo_hbm.at[:, pl.ds(n * 128, 128)], bo_v.at[n], SEM_BO).start()
    else:
        copy(bo_hbm, bo_v, SEM_BO).start()

    copy(wphi_hbm, wphi_v, SEM_PHI).wait()
    row = lax.broadcasted_iota(i32, (AH, D), 0)
    col = lax.broadcasted_iota(i32, (AH, D), 1)
    dsel = col - AD * row
    wf = None
    for d in range(AD):
        y = _dot(wphi_v[d], (dsel == d).astype(bf16))
        wf = y if wf is None else y + wf
    wf = wf.astype(bf16)
    row = lax.broadcasted_iota(i32, (CR, AD), 0)
    col = lax.broadcasted_iota(i32, (CR, AD), 1)
    sel = (((row % GR) // 2) == col).astype(bf16)
    row = lax.broadcasted_iota(i32, (CR, 256), 0)
    col = lax.broadcasted_iota(i32, (CR, 256), 1)
    head = (row // GR) * 2 + row % 2
    phit = []
    for c in range(NC):
        rep = _dot(sel, wf[:, c * 128:c * 128 + 256])
        keep = (head + c * 2 * CG) == (col + c * 128) // AD
        phit.append(jnp.where(keep, rep, 0.0).astype(bf16))
    copy(wqkv_hbm, wqkv_v, SEM_QKV).wait()
    wvt = wqkv_v[:, 2 * D:3 * D].T
    for c in range(NC):
        wk = _dot_nt(phit[c], wqkv_v[:, D + c * 128:D + c * 128 + 256]).astype(bf16)
        wkv_s[c] = _pack(jnp.concatenate([wk, wvt[c * CR:(c + 1) * CR]], axis=0))
    for c in range(NC):
        wq_s[c] = _pack(_dot_nt(phit[c], wqkv_v[:, c * 128:c * 128 + 256]).astype(bf16))

    x_copy(0, TS1, SEM_X0).wait()
    copy(mem_hbm, mem_v, SEM_X0).start()

    def stage_q(y):
        lo = lax.broadcasted_iota(i32, (y.shape[0], 128), 1) < 64
        y = y * SCALE
        qm = y[:, 128:256]
        return jnp.concatenate([y[:, :128], jnp.where(lo, qm, 0.0), jnp.where(lo, 0.0, qm), y[:, 256:]], axis=1)

    def layer_a(li):
        first = li == 0

        def transposes(dst, base, q0, n):
            for u in range(n):
                dst[q0 + u] = _pack(stage[base + q0 + u].reshape(PW, D).T)

        def w_wait(q0, n, slot):
            copy(stage.at[pl.ds(q0, n)], stage.at[pl.ds(q0, n)], slot).wait()

        def ln_rows(r0, n):
            rows = pl.ds(pl.multiple_of(r0, n), n)
            xn = _layernorm(xin[rows, :].astype(f32)).astype(bf16)
            xna[pl.ds(pl.multiple_of(r0 // 2, n // 2), n // 2), :] = _pack(xn)
            return xn

        def xn_rows(r0, n):
            return _unpack(xna[pl.ds(pl.multiple_of(r0 // 2, n // 2), n // 2), :])

        def kv_update(c, y, ones):
            for u in range(CG):
                phi = _hedgehog(y[u * GR:(u + 1) * GR])
                vt = jnp.concatenate([y[CR + u * GR:CR + (u + 1) * GR], ones], axis=0).astype(bf16)
                kv_acc[c * CG + u] += _dot_nt(vt, phi)

        def pass1(i, carry):
            @pl.when(first)
            def _():
                @pl.when(i + 1 < NB)
                def _():
                    x_copy(0, TA, SEM_IT + i).wait()

                @pl.when(i + 1 == NB)
                def _():
                    x_copy(0, TA - TS1, SEM_IT + i).wait()
                w_wait(i * W1, W1, SEM_IT + i)

            ones = jnp.ones((8, TS1), f32)
            pend = (NC - 1, ylast[...], jnp.where(i > 0, ones, 0.0))
            for s in range(TA // TS1):
                r0 = i * TA + s * TS1
                xn = xn_rows(r0, TS1) if s == 0 else ln_rows(r0, TS1)
                for c in range(NC):
                    y = _dot_nt(_unpack(wkv_s[c]), xn)
                    kv_update(*pend)
                    pend = (c, y, ones)
            ylast[...] = pend[1]
            ln_rows(jnp.minimum(i + 1, NB - 1) * TA, TS1)
            transposes(wbq_s, 0, i * W1, W1)
            return carry

        def pass2(i, carry):
            @pl.when(first)
            def _():
                @pl.when(i == 0)
                def _():
                    copy(wo_hbm, wo_v, SEM_IT + NB).wait()
                w_wait(NB * W1 + i * W2, W2, SEM_IT + NB + i)

            sub = lax.broadcasted_iota(i32, (8, TS2), 0) < 4
            ns = TA // TS2
            ot = {}

            def feat(s, c, p):
                for u in range(CG):
                    g = c * CG + u
                    y = _dot(kv_s[g], _hedgehog(p[u * GR:(u + 1) * GR]))
                    r = _recip(y[GR:] + 1e-6)
                    rr = pltpu.roll(r, 4, 0)
                    r0, r1 = jnp.where(sub, r, rr), jnp.where(sub, rr, r)
                    ot[s, g] = y[:GR] * jnp.concatenate([r0, r0, r, r1, r1], axis=0)

            def back(s, lo, hi, extra=()):
                o = jnp.concatenate([ot[s, g][:, lo:hi] for g in range(NG)], axis=0).T.astype(bf16)
                rows = pl.ds(pl.multiple_of(i * TA + s * TS2 + lo, hi - lo), hi - lo)
                if not extra:
                    xa[rows, :] = xin[rows, :].astype(f32) + _dot(o, wo_v[...])
                    return
                ys = []
                for n in range(5):
                    ys.append(_dot(o, wo_v[:, n * 128:(n + 1) * 128]))
                    for _ in range(extra[n]):
                        pieces.pop(0)()
                xa[rows, :] = xin[rows, :].astype(f32) + jnp.concatenate(ys, axis=1)

            transposes(wbkv_s, NP, i * W2, W2)
            pend = []
            for s in range(ns):
                xn = xn_rows(i * TA + s * TS2, TS2)
                for c in range(NC):
                    pend.append((s, c, _dot_nt(_unpack(wq_s[c]), xn)))
                    if len(pend) > CFG["F2"]:
                        feat(*pend.pop(0))
                if 1 <= s < ns - 1:
                    back(s - 1, 0, TS2)
            half = TS2 // 2
            back(ns - 2, 0, half)
            while pend:
                feat(*pend.pop(0))
            xn0 = _layernorm(xa[0:64, :])
            xnb[...] = xn0
            h8 = xn0[0:16].astype(bf16)
            qparts = {}

            def q_piece(u, n):
                j = i * (NP // NB) + u
                qparts[u, n] = _dot(h8, _unpack(wbq_s[j, :, n * 128:(n + 1) * 128]))[:8]
                if n == 2:
                    sv_q[j, 8:16, :] = stage_q(jnp.concatenate([qparts[u, m] for m in range(3)], axis=1))

            if CFG.get("D0"):
                back(ns - 2, half, TS2)
                back(ns - 1, 0, TS2)
                return carry
            pieces = [functools.partial(q_piece, u, n) for u in range(NP // NB) for n in range(3)]
            qf = CFG.get("qf", (0, 0, 1, 1, 1, 1, 1, 1, 1, 1, 1, 1, 1, 1, 0))
            back(ns - 2, half, TS2, qf[0:5])
            back(ns - 1, 0, half, qf[5:10])
            back(ns - 1, half, TS2, qf[10:15])
            assert not pieces
            return carry

        kv_acc[...] = jnp.zeros_like(kv_acc)
        ylast[...] = jnp.zeros_like(ylast)
        ln_rows(0, TS1)
        lax.fori_loop(0, NB, pass1, 0)
        kv_update(NC - 1, ylast[...], jnp.ones((8, TS1), f32))
        row = lax.broadcasted_iota(i32, (GR + 8, 2 * GR), 0)
        col = lax.broadcasted_iota(i32, (GR + 8, 2 * GR), 1)
        keep = jnp.where(row < GR, row // AD, (row - GR) // 4) == col % 2
        for g in range(NG):
            kv_s[g] = jnp.where(keep, kv_acc[g], 0.0).astype(bf16)
        lax.fori_loop(0, NB, pass2, 0)

        @pl.when(first)
        def _():
            copy(mem_hbm, mem_v, SEM_X0).wait()
            if not CFG.get("late"):
                copy(bo_v, bo_v, SEM_BO).wait()

    def layer_b(li):
        lo40 = lax.broadcasted_iota(i32, (L, 128), 1) < 64
        zero40 = jnp.zeros((L, 128), f32)

        def blockdiag_k(k):
            kmid = k[:, 128:256]
            top = jnp.concatenate([k[:, :128], jnp.where(lo40, kmid, zero40), zero40], axis=1)
            bot = jnp.concatenate([zero40, jnp.where(lo40, zero40, kmid), k[:, 256:]], axis=1)
            return jnp.concatenate([top, bot], axis=0).astype(bf16)

        def blockdiag_v(v):
            t = [v[:, cb * 128:(cb + 1) * 128] for cb in range(3)]
            top = jnp.concatenate([jnp.where(lo40, x, zero40) for x in t], axis=1)
            bot = jnp.concatenate([jnp.where(lo40, zero40, x) for x in t], axis=1)
            return jnp.concatenate([top, bot], axis=0).astype(bf16)

        r = lax.broadcasted_iota(i32, (32, 2 * L), 0)
        c = lax.broadcasted_iota(i32, (32, 2 * L), 1)
        isa = c < L
        key = jnp.where(isa, c, c - L)
        valid = (r < M) | (r >= key) | (key >= 32)
        lane = lax.broadcasted_iota(i32, (8, 128), 1)
        sub = lax.broadcasted_iota(i32, (8, 128), 0)
        lo8 = lane < 64
        lo16 = lax.broadcasted_iota(i32, (16, 128), 1) < 64

        def bcast(ref, j, t, cb):
            return jnp.broadcast_to(ref[j, t:t + 1, cb * 128:(cb + 1) * 128], (8, 128))

        def head8(jq, r0, kv, j):
            q0, qa, qb, q2 = [sv_q[jq, r0:r0 + 8, cb * 128:(cb + 1) * 128] for cb in range(4)]
            ss = []
            for t in range(16):
                k1 = bcast(kv, j, t, 1)
                sa = jnp.sum(q0 * bcast(kv, j, t, 0) + qa * k1, axis=1, keepdims=True)
                sb = jnp.sum(q2 * bcast(kv, j, t, 2) + qb * k1, axis=1, keepdims=True)
                ss.append((sa, sb))
            if True:
                cs = []
                for t, (sa, sb) in enumerate(ss):
                    s = jnp.where(lo8, sa, sb)
                    cs.append(jnp.where(sub >= t - 8, s, -1e9) if t > 8 else s)
                m = cs
                while len(m) > 1:
                    m = [jnp.maximum(m[a], m[a + 1]) for a in range(0, len(m), 2)]
                l, acc = None, None
                for t in range(16):
                    e = jnp.exp(cs[t] - m[0])
                    pv = [e * bcast(kv, j, t, 3 + cb) for cb in range(3)]
                    l = e if l is None else l + e
                    acc = pv if acc is None else [a + b for a, b in zip(acc, pv)]
                rl = _recip(l)
                return jnp.concatenate([a * rl for a in acc], axis=1)

        def softmax(s):
            s = jnp.where(valid, s * SCALE, -1e9)
            ma = jnp.max(jnp.where(isa, s, -jnp.inf), axis=1, keepdims=True)
            mb = jnp.max(jnp.where(isa, -jnp.inf, s), axis=1, keepdims=True)
            e = jnp.exp(s - jnp.where(isa, ma, mb))
            la = jnp.sum(jnp.where(isa, e, 0.0), axis=1, keepdims=True)
            lb = jnp.sum(jnp.where(isa, 0.0, e), axis=1, keepdims=True)
            return e * _recip(jnp.where(isa, la, lb))

        def wo_rows(j0, j1):
            return jnp.concatenate([bo_v[j * PW + hh * BE + cb * 64:j * PW + hh * BE + cb * 64 + 64, :]
                                    for j in range(j0, j1) for cb in range(3) for hh in range(2)], axis=0)

        def tie(x, dep, zero):
            d = pltpu.bitcast(dep[:, :128] + dep[:, 128:256] + dep[:, 256:], i32) & zero
            top = pltpu.bitcast(pltpu.bitcast(x[:8], i32) | d[:, :x.shape[1]], f32)
            return jnp.concatenate([top, x[8:]], axis=0)

        def step(h, even, first, last, qslot, zero, o1e):
            sched = _b_schedule(CFG["pe"] if even else CFG["po"],
                                CFG["tl"] if last else (CFG["te"] if even else CFG["to"]))
            widx = dict(q=(wbq_s, 0), k=(wbkv_s, 0), v=(wbkv_s, NP))
            kv = sv_e16 if even else sv_o16
            dl = CFG["de"] if even else CFG["do"]

            def proj(op, j, k0, k1):
                hh = h if (op == "q") != even else h[:32]
                return _dot(hh[:, k0 * 128:k1 * 128], _unpack(widx[op][0][widx[op][1] + j, k0 * 64:k1 * 64, :]))

            part, kdone = {}, 0
            for k1 in (() if first else (2, 3)):
                for op in [op for op, j in sched if op in widx and j == 0]:
                    y = proj(op, 0, kdone, k1)
                    part[op] = y + part[op] if op in part else y
                kdone = k1

            val, acc, o1 = {}, None, {}

            def lhs_o(j):
                o = val.pop(("o", j))
                if even:
                    return o
                return jnp.concatenate([o, jnp.concatenate([o1e[j], o1[j]], axis=0).astype(bf16)], axis=0)

            for op, j in sched:
                if op in widx:
                    y = proj(op, j, kdone, 5) + part[op] if (j == 0 and part) else proj(op, j, 0, 5)
                    if op == "q":
                        val["q", j] = y[:32].astype(bf16)
                        if not even:
                            sv_q[qslot + j] = stage_q(y[32:])
                        continue
                    cols = slice(0, PW) if op == "k" else slice(PW, 2 * PW)
                    kv[j, 0:8, cols] = y[0:8]
                    if even:
                        sv_e16[j, 8:16, cols] = y[32:40]
                        sv_o16[j, 8:16, cols] = y[40:48]
                        y = y[:40]
                    else:
                        y = jnp.concatenate([y, sv_o16[j, 8:16, cols]], axis=0)
                    val[op, j] = blockdiag_k(y) if op == "k" else blockdiag_v(y)
                elif op == "S":
                    if CFG.get("D0"):
                        if not even:
                            o1e[j] = head8(qslot + j, 8, sv_e16, j)
                            o1[j] = head8(qslot + j, 0, sv_o16, j)
                    else:
                        o1[j] = head8(qslot + j, 8 if even else 0, kv, j)
                    s = _dot_nt(val.pop(("q", j)), val.pop(("k", j)))
                    if CFG.get("D0") and not even and j - CFG["ds"] >= 0:
                        s = tie(s, o1e[j - CFG["ds"]], zero)
                    val["p", j] = softmax(s)
                elif op == "P":
                    p = val.pop(("p", j))
                    if dl is not None and j - dl in o1:
                        p = tie(p, o1[j - dl], zero)
                    val["o", j] = _dot(p.astype(bf16), val.pop(("v", j))).astype(bf16)
                elif op == "M":
                    o = jnp.concatenate([lhs_o(jj) for jj in range(j, NP)], axis=1)
                    acc = _dot(o, wo_rows(j, NP)) + acc
                else:
                    y = _dot(lhs_o(j), wo_rows(j, j + 1))
                    acc = y if acc is None else y + acc
            return acc, o1

        def body(i, mem):
            zero = i // NI
            qslot = zero if CFG.get("dyn", 1) else 0
            rn = pl.multiple_of(jnp.minimum(i + 1, NI - 1) * TB, TB)
            xns = [xnb[...]] + [_layernorm(xa[pl.ds(pl.multiple_of((i * UB + u) * 64, 64), 64), :]) for u in range(1, UB)]
            xns.append(_layernorm(xa[pl.ds(rn, 64), :]))
            for u in range(UB):
                r0 = pl.multiple_of((i * UB + u) * 64, 64)

                def add_rows(off, y):
                    rows = pl.ds(r0 + off, y.shape[0])
                    xin[rows, :] = (xa[rows, :] + y).astype(bf16)

                xn = xns[u]
                h = jnp.concatenate([mem, xn[8:32], xn[0:8], xn[32:40]], axis=0).astype(bf16)
                ye, o1e = step(h, True, u == 0, False, qslot, zero, None)
                mem = ye[:8]
                add_rows(16, ye[16:])
                h = jnp.concatenate([mem, xn[40:64], xn[32:40], xns[u + (0 if CFG.get('D0') else 1)][0:8]], axis=0).astype(bf16)
                yo, _ = step(h, False, False, u == UB - 1, qslot, zero, o1e)
                mem = yo[:8]
                add_rows(48, yo[16:32])
                add_rows(0, jnp.concatenate([yo[32:40], ye[8:16]], axis=0))
                add_rows(32, jnp.concatenate([yo[40:48], yo[8:16]], axis=0))
            xnb[...] = xns[UB]

            @pl.when(li == 1)
            def _():
                out_copy(i).start()
            return mem

        lax.fori_loop(0, CFG.get('NIT', NI), body, mem_v[...].astype(f32))

    def layer(li, carry):
        if not CFG.get("noA"):
            layer_a(li)
        if not CFG.get("noB"):
            layer_b(li)
        return carry

    lax.fori_loop(0, 2, layer, 0)
    n = CFG.get('NIT', NI) * TB
    copy(xin.at[pl.ds(0, n)], out_hbm.at[pl.ds(0, n)], SEM_OUT).wait()


@functools.partial(jax.jit, static_argnames=("B_seg_len",))
def pallas_interleave_layers__linear_kernel_hedgehog__memory_aug_recurrent_mem_tr__prompt_kernel(
    A_x: jax.Array,
    A_wqkv: jax.Array,
    A_w_phi: jax.Array,
    A_wo: jax.Array,
    B_x: jax.Array,
    B_mem0: jax.Array,
    B_Wq: jax.Array,
    B_Wk: jax.Array,
    B_Wv: jax.Array,
    B_Wo: jax.Array,
    B_seg_len=SEG,
):
    assert B_seg_len == SEG
    x = A_x.reshape(S, D)
    wphi = A_w_phi.transpose(1, 2, 0)
    mem0 = B_mem0.reshape(M, D)
    bq = B_Wq.transpose(1, 2, 0).reshape(NP, 3, 2, 64, D)
    bk = B_Wk.transpose(1, 2, 0).reshape(NP, 3, 2, 64, D)
    bv = B_Wv.transpose(1, 2, 0).reshape(BH, 3, 64, D)
    bo = B_Wo.reshape(HE, D)

    anyspec = pl.BlockSpec(memory_space=pl.ANY)
    out = pl.pallas_call(
        _kernel,
        out_shape=jax.ShapeDtypeStruct((S, D), bf16),
        in_specs=[anyspec] * 9,
        out_specs=anyspec,
        scratch_shapes=[
            pltpu.VMEM((S, D), bf16),
            pltpu.VMEM((D, 3 * D), bf16),
            pltpu.VMEM((AD, AD, AH), bf16),
            pltpu.VMEM((D, D), bf16),
            pltpu.VMEM((M, D), bf16),
            pltpu.VMEM((S, D), f32),
            pltpu.VMEM((S // 2, D), u32),
            pltpu.VMEM((64, D), f32),
            pltpu.VMEM((NC, CR // 2, D), u32),
            pltpu.VMEM((NC, CR, D), u32),
            pltpu.VMEM((2 * CR, TS1), f32),
            pltpu.VMEM((NG, GR + 8, 2 * GR), f32),
            pltpu.VMEM((NG, GR + 8, 2 * GR), bf16),
            pltpu.VMEM((NW, 3, 2, 64, D), bf16),
            pltpu.VMEM((NP, D // 2, PW), u32),
            pltpu.VMEM((2 * NP, D // 2, PW), u32),
            pltpu.VMEM((5, HE, 128) if CFG.get('wot', 0) else (HE, D), bf16),
            pltpu.VMEM((NP, 16, 2 * PW), f32),
            pltpu.VMEM((NP, 16, 2 * PW), f32),
            pltpu.VMEM((NP, 16, 512), f32),
            pltpu.SemaphoreType.DMA((NSEM,)),
        ],
        compiler_params=pltpu.CompilerParams(vmem_limit_bytes=110 * 1024 * 1024,
                                             disable_bounds_checks=True),
    )(x, A_wqkv, wphi, A_wo, mem0, bq, bk, bv, bo)
    return out.reshape(1, S, D)
```

```python
import functools

import jax
import jax.numpy as jnp
from jax import lax
import jax.experimental.pallas as pl
import jax.experimental.pallas.tpu as pltpu

bf16 = jnp.bfloat16
f32 = jnp.float32
u32 = jnp.uint32
i32 = jnp.int32

CFG = dict(
    TA=512, TS1=128, TS2=256, W1=4, F1=1, F2=2,
    pe="q0 k0 v0 S1 P2", po="q0 S1 k0 v0 P3", de=1, do=0, dyn=0, e2=1, w128=1, a2=1, z2=1, x2=1, x3=2, ge='b', go='b',
    te=(3, 4, 2, 3), to=(2, 2, 1, 1, 2), tl=(2, 2, 1, 2, 0), UB=2,
)
CFG.update(pe='k0 q0 v0 S1 P2', po='q0 k0 q0 S1 v0 q0 P3', te=(3,4,2,3), to=(1,2,2,1,2), tl=(2,2,1,2,0))

S = 2048
D = 640
AH = 32
AD = 20
GR = 2 * AD
NG = AH // 2
CG = 4
CR = CG * GR
NC = NG // CG
TA = CFG["TA"]
TS1 = CFG["TS1"]
TS2 = CFG["TS2"]
NB = S // TA
BH = 32
BE = 192
HE = BH * BE
M = 8
SEG = 32
L = M + SEG
NP = BH // 2
PW = 2 * BE
SCALE = BE ** -0.5
LOG2E = 1.4426950408889634
UB = CFG["UB"]
TB = 64 * UB
NI = S // TB
NW = 3 * NP
W1 = CFG["W1"]
W2 = NW // NB - W1

NT = (((1,), (1,)), ((), ()))

SEM_PHI, SEM_QKV, SEM_X0, SEM_BO, SEM_OUT = 0, 1, 2, 3, 4
SEM_IT = 5
NSEM = SEM_IT + 2 * NB


def _dot(a, b):
    return jnp.dot(a, b, preferred_element_type=f32)


def _dot_nt(a, b):
    return lax.dot_general(a, b, NT, preferred_element_type=f32)


def _pack(x):
    return pltpu.bitcast(x, u32)


def _unpack(x):
    return pltpu.bitcast(x, bf16)


def _recip(x):
    r = pl.reciprocal(x, approx=True)
    return r if CFG.get("nn") else r * (2.0 - x * r)


def _layernorm(x):
    m = jnp.mean(x, axis=-1, keepdims=True)
    xc = x - m
    v = jnp.mean(xc * xc, axis=-1, keepdims=True)
    return xc * lax.rsqrt(v + 1e-5)


def _freduce(x3, op):
    r = op(op(op(x3[0], x3[1]), op(x3[2], x3[3])), x3[4])
    r = op(r, pltpu.roll(r, 2, 0))
    return op(r, pltpu.roll(r, 4, 0))


def _hedgehog(p):
    t = p.shape[1]
    p3 = p.reshape(GR // 8, 8, t)
    ex = jnp.exp2 if CFG.get("a2") else jnp.exp
    ep = ex(p3 - _freduce(p3, jnp.maximum)[None])
    en = ex(_freduce(p3, jnp.minimum)[None] - p3)
    ep = ep * _recip(_freduce(ep, jnp.add))[None]
    en = en * _recip(_freduce(en, jnp.add))[None]
    return jnp.concatenate([ep.reshape(GR, t), en.reshape(GR, t)], axis=0).astype(bf16)


def _b_schedule(period, tail):
    if "O" not in period:
        period += " O0"
    ops = [(t[0], int(t[1:])) for t in period.split()]
    maxlag = max(lag for _, lag in ops)
    merged, tail = tail[-1], tail[:-1]
    assert len(tail) == maxlag + 1
    nin = NP - sum(tail) - merged
    out, o = [], 0
    for t in range(NP + maxlag + 1):
        if t >= NP:
            out += [("O", o + i) for i in range(tail[t - NP])]
            o += tail[t - NP]
        for op, lag in ops:
            if op != "O":
                if 0 <= t - lag < NP:
                    out.append((op, t - lag))
            elif NP - nin <= t < NP:
                out.append(("O", o))
                o += 1
    if merged:
        out.append(("M", o))
    return out


def _kernel(x_hbm, wqkv_hbm, wphi_hbm, wo_hbm, mem_hbm, bq_hbm, bk_hbm, bv_hbm, bo_hbm,
            out_hbm,
            xin, wqkv_v, wphi_v, wo_v, mem_v, xa, xna, xnb, wq_s, wkv_s, ylast, kv_acc, kv_s,
            stage, wbq_s, wbkv_s, bo_v, sv_o16, sv_e16, sv_q, sems):
    bw_hbm = (bq_hbm, bk_hbm, bv_hbm)

    def copy(src, dst, slot):
        return pltpu.make_async_copy(src, dst, sems.at[slot])

    def w_start(q, slot):
        t, j = divmod(q, NP)
        if t < 2:
            copy(bw_hbm[t].at[j], stage.at[q], slot).start()
        else:
            for hh in range(2):
                copy(bv_hbm.at[2 * j + hh], stage.at[q, :, hh], slot).start()

    def x_copy(r0, n, slot):
        return copy(x_hbm.at[pl.ds(r0, n)], xin.at[pl.ds(r0, n)], slot)

    def w_first(n):
        return n * W1 if isinstance(n, int) and n <= NB else NB * W1 + (n - NB) * W2

    def out_copy(b):
        rows = pl.ds(pl.multiple_of(b * TB, TB), TB)
        return copy(xin.at[rows], out_hbm.at[rows], SEM_OUT)

    copy(wphi_hbm, wphi_v, SEM_PHI).start()
    copy(wqkv_hbm, wqkv_v, SEM_QKV).start()
    x_copy(0, TS1, SEM_X0).start()
    for b in range(NB):
        x_copy(b * TA + TS1, TA if b + 1 < NB else TA - TS1, SEM_IT + b).start()
        for q in range(b * W1, (b + 1) * W1):
            w_start(q, SEM_IT + b)
    copy(wo_hbm, wo_v, SEM_IT + NB).start()
    for b in range(NB):
        for q in range(NB * W1 + b * W2, NB * W1 + (b + 1) * W2):
            w_start(q, SEM_IT + NB + b)
    if CFG.get("wot", 0) == 2:
        copy(bo_hbm.bitcast(u32), bo_v, SEM_BO).start()
    elif CFG.get("wot", 0):
        for n in range(5):
            copy(bo_hbm.at[:, pl.ds(n * 128, 128)], bo_v.at[n], SEM_BO).start()
    else:
        copy(bo_hbm, bo_v, SEM_BO).start()

    kv_acc[...] = jnp.zeros_like(kv_acc)
    ylast[...] = jnp.zeros_like(ylast)
    copy(wphi_hbm, wphi_v, SEM_PHI).wait()
    row = lax.broadcasted_iota(i32, (AH, D), 0)
    col = lax.broadcasted_iota(i32, (AH, D), 1)
    dsel = col - AD * row
    wf = None
    for d in range(AD):
        y = _dot(wphi_v[d], (dsel == d).astype(bf16))
        wf = y if wf is None else y + wf
    wf = wf.astype(bf16)
    row = lax.broadcasted_iota(i32, (CR, AD), 0)
    col = lax.broadcasted_iota(i32, (CR, AD), 1)
    sel = (((row % GR) // 2) == col).astype(bf16)
    row = lax.broadcasted_iota(i32, (CR, 256), 0)
    col = lax.broadcasted_iota(i32, (CR, 256), 1)
    head = (row // GR) * 2 + row % 2
    phit = []
    for c in range(NC):
        rep = _dot(sel, wf[:, c * 128:c * 128 + 256])
        keep = (head + c * 2 * CG) == (col + c * 128) // AD
        phit.append(jnp.where(keep, rep, 0.0).astype(bf16))
    copy(wqkv_hbm, wqkv_v, SEM_QKV).wait()
    wvt = wqkv_v[:, 2 * D:3 * D].T
    for c in range(NC):
        wk = (_dot_nt(phit[c], wqkv_v[:, D + c * 128:D + c * 128 + 256]) * (LOG2E if CFG.get('a2') else 1.0)).astype(bf16)
        wkv_s[c] = _pack(jnp.concatenate([wk, wvt[c * CR:(c + 1) * CR]], axis=0))
    for c in range(NC):
        wq_s[c] = _pack((_dot_nt(phit[c], wqkv_v[:, c * 128:c * 128 + 256]) * (LOG2E if CFG.get('a2') else 1.0)).astype(bf16))

    x_copy(0, TS1, SEM_X0).wait()
    copy(mem_hbm, mem_v, SEM_X0).start()

    def stage_q(y):
        lo = lax.broadcasted_iota(i32, (y.shape[0], 128), 1) < 64
        y = y * (SCALE * LOG2E if CFG.get('e2') else SCALE)
        qm = y[:, 128:256]
        return jnp.concatenate([y[:, :128], jnp.where(lo, qm, 0.0), jnp.where(lo, 0.0, qm), y[:, 256:]], axis=1)

    def layer_a(li):
        first = li == 0

        def transposes(dst, base, q0, n):
            for u in range(n):
                dst[q0 + u] = _pack(stage[base + q0 + u].reshape(PW, D).T)

        def w_wait(q0, n, slot):
            copy(stage.at[pl.ds(q0, n)], stage.at[pl.ds(q0, n)], slot).wait()

        def ln_rows(r0, n):
            rows = pl.ds(pl.multiple_of(r0, n), n)
            xn = _layernorm(xin[rows, :].astype(f32)).astype(bf16)
            xna[pl.ds(pl.multiple_of(r0 // 2, n // 2), n // 2), :] = _pack(xn)
            return xn

        def xn_rows(r0, n):
            return _unpack(xna[pl.ds(pl.multiple_of(r0 // 2, n // 2), n // 2), :])

        def kv_update(c, y, ones):
            for u in range(CG):
                phi = _hedgehog(y[u * GR:(u + 1) * GR])
                vt = jnp.concatenate([y[CR + u * GR:CR + (u + 1) * GR], ones], axis=0).astype(bf16)
                kv_acc[c * CG + u] += _dot_nt(vt, phi)

        def pass1(i, carry):
            @pl.when(first)
            def _():
                @pl.when(i + 1 < NB)
                def _():
                    x_copy(0, TA, SEM_IT + i).wait()

                @pl.when(i + 1 == NB)
                def _():
                    x_copy(0, TA - TS1, SEM_IT + i).wait()
                w_wait(i * W1, W1, SEM_IT + i)

            ones = jnp.ones((8, TS1), f32)
            F1 = CFG["F1"]
            pend = [(NC - F1 + a, ylast[a], jnp.where(i > 0, ones, 0.0)) for a in range(F1)]
            for s in range(TA // TS1):
                r0 = i * TA + s * TS1
                xn = xn_rows(r0, TS1) if s == 0 else ln_rows(r0, TS1)
                for c in range(NC):
                    sp = CFG.get("sp", 0)
                    lastp = s == TA // TS1 - 1 and c == NC - 1
                    if sp == 1 or (sp == 2 and lastp):
                        y = jnp.concatenate([_dot_nt(_unpack(wkv_s[c, :CR // 2]), xn), _dot_nt(_unpack(wkv_s[c, CR // 2:]), xn)], axis=0)
                        kv_update(*pend.pop(0))
                    elif sp == 3:
                        y1 = _dot_nt(_unpack(wkv_s[c, :CR // 2]), xn)
                        kv_update(*pend.pop(0))
                        y = jnp.concatenate([y1, _dot_nt(_unpack(wkv_s[c, CR // 2:]), xn)], axis=0)
                    elif sp == 4 and lastp:
                        y = jnp.concatenate([_dot_nt(_unpack(wkv_s[c, a * 40:(a + 1) * 40]), xn) for a in range(4)], axis=0)
                        kv_update(*pend.pop(0))
                    else:
                        y = _dot_nt(_unpack(wkv_s[c]), xn)
                        kv_update(*pend.pop(0))
                    pend.append((c, y, ones))
            for a in range(F1):
                ylast[a] = pend[a][1]
            ln_rows(jnp.minimum(i + 1, NB - 1) * TA, TS1)
            transposes(wbq_s, 0, i * W1, W1)
            return carry

        def pass2(i, carry):
            @pl.when(first)
            def _():
                @pl.when(i == 0)
                def _():
                    copy(wo_hbm, wo_v, SEM_IT + NB).wait()
                w_wait(NB * W1 + i * W2, W2, SEM_IT + NB + i)

            sub = lax.broadcasted_iota(i32, (8, TS2), 0) < 4
            ns = TA // TS2
            ot = {}

            def feat(s, c, p):
                for u in range(CG):
                    g = c * CG + u
                    y = _dot(kv_s[g], _hedgehog(p[u * GR:(u + 1) * GR]))
                    r = _recip(y[GR:] + 1e-6)
                    rr = pltpu.roll(r, 4, 0)
                    r0, r1 = jnp.where(sub, r, rr), jnp.where(sub, rr, r)
                    ot[s, g] = y[:GR] * jnp.concatenate([r0, r0, r, r1, r1], axis=0)

            def back(s, lo, hi, extra=()):
                o = jnp.concatenate([ot[s, g][:, lo:hi] for g in range(NG)], axis=0).T.astype(bf16)
                rows = pl.ds(pl.multiple_of(i * TA + s * TS2 + lo, hi - lo), hi - lo)
                if not extra:
                    xa[rows, :] = xin[rows, :].astype(f32) + _dot(o, wo_v[...])
                    return
                ys = []
                for n in range(5):
                    ys.append(_dot(o, wo_v[:, n * 128:(n + 1) * 128]))
                    for _ in range(extra[n]):
                        pieces.pop(0)()
                xa[rows, :] = xin[rows, :].astype(f32) + jnp.concatenate(ys, axis=1)

            transposes(wbkv_s, NP, i * W2, W2)
            if CFG.get("z2"):
                kv_acc[...] = jnp.zeros_like(kv_acc)
                ylast[...] = jnp.zeros_like(ylast)
            pend = []
            for s in range(ns):
                xn = xn_rows(i * TA + s * TS2, TS2)
                for c in range(NC):
                    pend.append((s, c, _dot_nt(_unpack(wq_s[c]), xn)))
                    if len(pend) > CFG["F2"]:
                        feat(*pend.pop(0))
                if 1 <= s < ns - 1:
                    back(s - 1, 0, TS2)
            half = TS2 // 2
            back(ns - 2, 0, half)
            while pend:
                feat(*pend.pop(0))
            xn0 = _layernorm(xa[0:64, :])
            xnb[...] = xn0
            h8 = xn0[0:16].astype(bf16)
            qparts = {}

            def q_piece(u, n):
                j = i * (NP // NB) + u
                qparts[u, n] = _dot(h8, _unpack(wbq_s[j, :, n * 128:(n + 1) * 128]))[:8]
                if n == 2:
                    sv_q[j, 8:16, :] = stage_q(jnp.concatenate([qparts[u, m] for m in range(3)], axis=1))

            pieces = [functools.partial(q_piece, u, n) for u in range(NP // NB) for n in range(3)]
            qf = CFG.get("qf", (0, 0, 1, 1, 1, 1, 1, 1, 1, 1, 1, 1, 1, 1, 0))
            back(ns - 2, half, TS2, qf[0:5])
            back(ns - 1, 0, half, qf[5:10])
            back(ns - 1, half, TS2, qf[10:15])
            assert not pieces
            return carry

        ln_rows(0, TS1)
        lax.fori_loop(0, NB, pass1, 0)
        for a in range(CFG["F1"]):
            kv_update(NC - CFG["F1"] + a, ylast[a], jnp.ones((8, TS1), f32))
        row = lax.broadcasted_iota(i32, (GR + 8, 2 * GR), 0)
        col = lax.broadcasted_iota(i32, (GR + 8, 2 * GR), 1)
        keep = jnp.where(row < GR, row // AD, (row - GR) // 4) == col % 2
        for g in range(NG):
            kv_s[g] = jnp.where(keep, kv_acc[g], 0.0).astype(bf16)
        if not CFG.get("z2"):
            kv_acc[...] = jnp.zeros_like(kv_acc)
            ylast[...] = jnp.zeros_like(ylast)
        lax.fori_loop(0, NB, pass2, 0)

        @pl.when(first)
        def _():
            copy(mem_hbm, mem_v, SEM_X0).wait()
            if not CFG.get("late"):
                copy(bo_v, bo_v, SEM_BO).wait()

    def layer_b(li):
        lo40 = lax.broadcasted_iota(i32, (L, 128), 1) < 64
        zero40 = jnp.zeros((L, 128), f32)

        def blockdiag_k(k):
            kmid = k[:, 128:256]
            top = jnp.concatenate([k[:, :128], jnp.where(lo40, kmid, zero40), zero40], axis=1)
            bot = jnp.concatenate([zero40, jnp.where(lo40, zero40, kmid), k[:, 256:]], axis=1)
            return jnp.concatenate([top, bot] + padrows, axis=0).astype(bf16)

        def blockdiag_v(v):
            t = [v[:, cb * 128:(cb + 1) * 128] for cb in range(3)]
            top = jnp.concatenate([jnp.where(lo40, x, zero40) for x in t], axis=1)
            bot = jnp.concatenate([jnp.where(lo40, zero40, x) for x in t], axis=1)
            return jnp.concatenate([top, bot] + padrows, axis=0).astype(bf16)

        SW = 128 if CFG.get("w128") else 2 * L

        def pos(a):
            return jnp.where(a < 8, a, jnp.where(a < 16, a + 24, jnp.where(a < 32, a, a - 24)))

        masks = {}
        for n in (16, 32):
            r = lax.broadcasted_iota(i32, (n, SW), 0)
            c = lax.broadcasted_iota(i32, (n, SW), 1)
            isa = c < L
            key = jnp.where(isa, c, c - L)
            masks[n] = (((r < M) | (pos(r) >= pos(key))) & (key < L), isa)
        padrows = [jnp.zeros((SW - 2 * L, PW), f32)] if SW > 2 * L else []
        lane = lax.broadcasted_iota(i32, (8, 128), 1)
        sub = lax.broadcasted_iota(i32, (8, 128), 0)
        lo8 = lane < 64
        lo16 = lax.broadcasted_iota(i32, (16, 128), 1) < 64

        def bcast(ref, j, t, cb):
            return jnp.broadcast_to(ref[j, t:t + 1, cb * 128:(cb + 1) * 128], (8, 128))

        def attn8(q, kv, j, nk):
            q0, qa, qb, q2 = [q[:, cb * 128:(cb + 1) * 128] for cb in range(4)]
            ch = CFG.get("ch", 32)
            mx, l, acc = None, None, None
            for t0 in range(0, nk, ch):
                cs = []
                for t in range(t0, min(t0 + ch, nk)):
                    k1 = bcast(kv, j, t, 1)
                    sa = jnp.sum(q0 * bcast(kv, j, t, 0) + qa * k1, axis=1, keepdims=True)
                    sb = jnp.sum(q2 * bcast(kv, j, t, 2) + qb * k1, axis=1, keepdims=True)
                    s = jnp.where(lo8, sa, sb)
                    cs.append(jnp.where(sub >= t - (nk - 8), s, -1e9) if t > nk - 8 else s)
                m = cs if mx is None else cs + [mx]
                while len(m) > 1:
                    m = [jnp.maximum(m[a], m[a + 1]) if a + 1 < len(m) else m[a] for a in range(0, len(m), 2)]
                if mx is not None:
                    sc = jnp.exp2(mx - m[0])
                    l, acc = l * sc, [a * sc for a in acc]
                mx = m[0]
                for t, s in enumerate(cs):
                    e = jnp.exp2(s - mx)
                    pv = [e * bcast(kv, j, t0 + t, 3 + cb) for cb in range(3)]
                    l = e if l is None else l + e
                    acc = pv if acc is None else [a + b for a, b in zip(acc, pv)]
            rl = _recip(l)
            return jnp.concatenate([a * rl for a in acc], axis=1)

        def softmax(s):
            valid, isa = masks[s.shape[0]]
            s = jnp.where(valid, s * (SCALE * LOG2E if CFG.get('e2') else SCALE), -1e9)
            ma = jnp.max(jnp.where(isa, s, -jnp.inf), axis=1, keepdims=True)
            mb = jnp.max(jnp.where(isa, -jnp.inf, s), axis=1, keepdims=True)
            e = (jnp.exp2 if CFG.get('e2') else jnp.exp)(s - jnp.where(isa, ma, mb))
            la = jnp.sum(jnp.where(isa, e, 0.0), axis=1, keepdims=True)
            lb = jnp.sum(jnp.where(isa, 0.0, e), axis=1, keepdims=True)
            return e * _recip(jnp.where(isa, la, lb))

        def wo_rows(j0, j1):
            starts = [j * PW + hh * BE + cb * 64 for j in range(j0, j1) for cb in range(3) for hh in range(2)]
            if CFG.get("wot", 0) == 2:
                return _unpack(jnp.concatenate([bo_v[a // 2:a // 2 + 32, :] for a in starts], axis=0))
            if CFG.get("wot", 0) == 1:
                return jnp.concatenate([jnp.concatenate([bo_v[n, a:a + 64, :] for n in range(5)], axis=1) for a in starts], axis=0)
            return jnp.concatenate([bo_v[a:a + 64, :] for a in starts], axis=0)

        def tie(x, dep, zero):
            d = pltpu.bitcast(dep[:, :128] + dep[:, 128:256] + dep[:, 256:], i32) & zero
            top = pltpu.bitcast(pltpu.bitcast(x[:8], i32) | d[:, :x.shape[1]], f32)
            return jnp.concatenate([top, x[8:]], axis=0)

        def step(h, even, u, zero, o1e):
            first, last = even and u == 0, (not even) and u == UB - 1
            eo = "e" if even else "o"

            def opt(name):
                return CFG.get(name + eo + str(u), CFG[name + eo])

            period = opt("p")
            sched = _b_schedule(period, CFG["tl"] if last else opt("t"))
            widx = dict(q=(wbq_s, 0), k=(wbkv_s, 0), v=(wbkv_s, NP))
            kv = sv_e16 if even else sv_o16
            dl = opt("d")
            ext = CFG.get("ext", ()) if even else ()

            def proj(op, j, k0, k1, n0=0, n1=3):
                hh = h if (op == "q") != even else h[:32]
                w = widx[op][0][widx[op][1] + j, k0 * 64:k1 * 64, n0 * 128:n1 * 128]
                return _dot(hh[:, k0 * 128:k1 * 128], _unpack(w))

            part, kdone = {}, 0
            for k1 in (() if first else (2, 3)):
                for op in dict.fromkeys(op for op, j in sched if op in widx and j == 0):
                    y = proj(op, 0, kdone, k1)
                    part[op] = y + part[op] if op in part else y
                kdone = k1

            val, acc, o1 = {}, None, {}

            def lhs_o(j):
                o = val.pop(("o", j))
                if j in ext:
                    x = jnp.concatenate([val.pop(("x2", j)), val.pop(("x3", j))], axis=0).astype(bf16)
                    return jnp.concatenate([o, x], axis=0)
                if even:
                    return o
                return jnp.concatenate([o, jnp.concatenate([o1e[j], o1[j]], axis=0).astype(bf16)], axis=0)

            for op, j in sched:
                if op in widx:
                    done = val.setdefault((op, j, "n"), [])
                    n0, n1 = (len(done), len(done) + 1) if period.count(op) == 3 else (0, 3)
                    if j == 0 and part:
                        done.append(proj(op, j, kdone, 5, n0, n1) + part[op][:, n0 * 128:n1 * 128])
                    else:
                        done.append(proj(op, j, 0, 5, n0, n1))
                    for jj in val.pop("waiting", []):
                        val["gate", jj] = done[-1][:8, :128]
                    if n1 < 3:
                        continue
                    y = jnp.concatenate(done, axis=1)
                    if op == "q":
                        if j in ext:
                            val["q", j] = y[:16].astype(bf16)
                            val["q2", j] = stage_q(y[16:32])
                            continue
                        val["q", j] = y[:32].astype(bf16)
                        if not even:
                            sv_q[j] = stage_q(y[32:])
                        continue
                    cols = slice(0, PW) if op == "k" else slice(PW, 2 * PW)
                    kv[j, 0:8, cols] = y[0:8]
                    if even:
                        sv_e16[j, 8:16, cols] = y[32:40]
                        if j in ext:
                            sv_e16[j, 16:32, cols] = y[16:32]
                        sv_o16[j, 8:16, cols] = y[40:48]
                        y = y[:40]
                    else:
                        y = jnp.concatenate([y, sv_o16[j, 8:16, cols]], axis=0)
                    val[op, j] = blockdiag_k(y) if op == "k" else blockdiag_v(y)
                    if opt("g") == op or (opt("g") == "b" and ("k", j) in val and ("v", j) in val):
                        val["waiting"] = [j]
                elif op == "S":
                    r0 = 8 if even else 0
                    q1 = sv_q[j, r0:r0 + 8, :]
                    if ("gate", j) in val:
                        g = pltpu.bitcast(val.pop(("gate", j)), i32) & zero
                        q1 = pltpu.bitcast(pltpu.bitcast(q1, i32) | jnp.concatenate([g] * 4, axis=1), f32)
                    o1[j] = attn8(q1, kv, j, 16)
                    if j in ext:
                        q2 = val.pop(("q2", j))
                        val["x2", j] = attn8(q2[:8], kv, j, 24)
                        val["x3", j] = attn8(q2[8:], kv, j, 32)
                    val["p", j] = softmax(_dot_nt(val.pop(("q", j)), val.pop(("k", j))))
                elif op == "P":
                    p = val.pop(("p", j))
                    if dl is not None and j - dl in o1:
                        p = tie(p, o1[j - dl], zero)
                    for nm in ("x2", "x3"):
                        if (nm, j - CFG[nm]) in val:
                            p = tie(p, val[nm, j - CFG[nm]], zero)
                    val["o", j] = _dot(p.astype(bf16), val.pop(("v", j))).astype(bf16)
                elif op == "M":
                    o = jnp.concatenate([lhs_o(jj) for jj in range(j, NP)], axis=1)
                    acc = _dot(o, wo_rows(j, NP)) + acc
                else:
                    y = _dot(lhs_o(j), wo_rows(j, j + 1))
                    acc = y if acc is None else y + acc
                    for jj in val.pop("waiting", []):
                        val["gate", jj] = acc[:8, :128]
            return acc, o1

        def body(i, mem):
            zero = i // NI
            rn = pl.multiple_of(jnp.minimum(i + 1, NI - 1) * TB, TB)
            xns = [xnb[...]] + [_layernorm(xa[pl.ds(pl.multiple_of((i * UB + u) * 64, 64), 64), :]) for u in range(1, UB)]
            xns.append(_layernorm(xa[pl.ds(rn, 64), :]))
            for u in range(UB):
                r0 = pl.multiple_of((i * UB + u) * 64, 64)

                def add_rows(off, y):
                    rows = pl.ds(r0 + off, y.shape[0])
                    xin[rows, :] = (xa[rows, :] + y).astype(bf16)

                xn = xns[u]
                h = jnp.concatenate([mem, xn[24:32], xn[8:24], xn[0:8], xn[32:40]], axis=0).astype(bf16)
                ye, o1e = step(h, True, u, zero, None)
                mem = ye[:8]
                add_rows(16, jnp.concatenate([ye[24:32], ye[8:16]], axis=0))
                h = jnp.concatenate([mem, xn[56:64], xn[40:56], xn[32:40], xns[u + 1][0:8]], axis=0).astype(bf16)
                yo, _ = step(h, False, u, zero, o1e)
                mem = yo[:8]
                add_rows(48, jnp.concatenate([yo[24:32], yo[8:16]], axis=0))
                add_rows(0, jnp.concatenate([yo[32:40], ye[16:24]], axis=0))
                add_rows(32, jnp.concatenate([yo[40:48], yo[16:24]], axis=0))
            xnb[...] = xns[UB]

            @pl.when(li == 1)
            def _():
                out_copy(i).start()
            return mem

        lax.fori_loop(0, CFG.get('NIT', NI), body, mem_v[...].astype(f32))

    def layer(li, carry):
        if not CFG.get("noA"):
            layer_a(li)
        if not CFG.get("noB"):
            layer_b(li)
        return carry

    lax.fori_loop(0, 2, layer, 0)
    n = CFG.get('NIT', NI) * TB
    copy(xin.at[pl.ds(0, n)], out_hbm.at[pl.ds(0, n)], SEM_OUT).wait()


@functools.partial(jax.jit, static_argnames=("B_seg_len",))
def pallas_interleave_layers__linear_kernel_hedgehog__memory_aug_recurrent_mem_tr__prompt_kernel(
    A_x: jax.Array,
    A_wqkv: jax.Array,
    A_w_phi: jax.Array,
    A_wo: jax.Array,
    B_x: jax.Array,
    B_mem0: jax.Array,
    B_Wq: jax.Array,
    B_Wk: jax.Array,
    B_Wv: jax.Array,
    B_Wo: jax.Array,
    B_seg_len=SEG,
):
    assert B_seg_len == SEG
    x = A_x.reshape(S, D)
    wphi = A_w_phi.transpose(1, 2, 0)
    mem0 = B_mem0.reshape(M, D)
    bq = B_Wq.transpose(1, 2, 0).reshape(NP, 3, 2, 64, D)
    bk = B_Wk.transpose(1, 2, 0).reshape(NP, 3, 2, 64, D)
    bv = B_Wv.transpose(1, 2, 0).reshape(BH, 3, 64, D)
    bo = B_Wo.reshape(HE, D)

    anyspec = pl.BlockSpec(memory_space=pl.ANY)
    out = pl.pallas_call(
        _kernel,
        out_shape=jax.ShapeDtypeStruct((S, D), bf16),
        in_specs=[anyspec] * 9,
        out_specs=anyspec,
        scratch_shapes=[
            pltpu.VMEM((S, D), bf16),
            pltpu.VMEM((D, 3 * D), bf16),
            pltpu.VMEM((AD, AD, AH), bf16),
            pltpu.VMEM((D, D), bf16),
            pltpu.VMEM((M, D), bf16),
            pltpu.VMEM((S, D), f32),
            pltpu.VMEM((S // 2, D), u32),
            pltpu.VMEM((64, D), f32),
            pltpu.VMEM((NC, CR // 2, D), u32),
            pltpu.VMEM((NC, CR, D), u32),
            pltpu.VMEM((CFG['F1'], 2 * CR, TS1), f32),
            pltpu.VMEM((NG, GR + 8, 2 * GR), f32),
            pltpu.VMEM((NG, GR + 8, 2 * GR), bf16),
            pltpu.VMEM((NW, 3, 2, 64, D), bf16),
            pltpu.VMEM((NP, D // 2, PW), u32),
            pltpu.VMEM((2 * NP, D // 2, PW), u32),
            [pltpu.VMEM((HE, D), bf16), pltpu.VMEM((5, HE, 128), bf16), pltpu.VMEM((HE // 2, D), u32)][CFG.get('wot', 0)],
            pltpu.VMEM((NP, 16, 2 * PW), f32),
            pltpu.VMEM((NP, 32, 2 * PW), f32),
            pltpu.VMEM((NP, 16, 512), f32),
            pltpu.SemaphoreType.DMA((NSEM,)),
        ],
        compiler_params=pltpu.CompilerParams(vmem_limit_bytes=110 * 1024 * 1024,
                                             disable_bounds_checks=True),
    )(x, A_wqkv, wphi, A_wo, mem0, bq, bk, bv, bo)
    return out.reshape(1, S, D)
```

```python
import functools

import jax
import jax.numpy as jnp
from jax import lax
import jax.experimental.pallas as pl
import jax.experimental.pallas.tpu as pltpu

bf16 = jnp.bfloat16
f32 = jnp.float32
u32 = jnp.uint32
i32 = jnp.int32

CFG = dict(
    pe="k0 q0 v0 S1 P2", po="q0 k0 q0 S1 v0 q0 P3",
    te=(3, 4, 2, 3), to=(1, 2, 2, 1, 2), tl=(2, 2, 1, 2, 0),
    de=1, do=0, ge="b", go="b",
)
CFG.update(nwo=16)

S = 2048
D = 640
LOG2E = 1.4426950408889634
AH = 32
AD = 20
GR = 2 * AD
NG = AH // 2
CG = 4
CR = CG * GR
NC = NG // CG
TA = 512
TS1 = 128
TS2 = 256
NB = S // TA
BH = 32
BE = 192
HE = BH * BE
M = 8
SEG = 32
L = M + SEG
NP = BH // 2
PW = 2 * BE
QSCALE = BE ** -0.5 * LOG2E
MASKED = -1e9 * LOG2E
UB = CFG.get("UB", 2)
TB = 64 * UB
NI = S // TB
NW = 3 * NP
WI = NW // NB
NWO = CFG.get("nwo", 4)

NT = (((1,), (1,)), ((), ()))

SEM_PHI, SEM_K, SEM_QV, SEM_OUT = 0, 1, 2, 3
SEM_X = 4
SEM_W = SEM_X + NB
SEM_WO = SEM_W + NB
NSEM = SEM_WO + NWO


def _dot(a, b):
    return jnp.dot(a, b, preferred_element_type=f32)


def _dot_nt(a, b):
    return lax.dot_general(a, b, NT, preferred_element_type=f32)


def _pack(x):
    return pltpu.bitcast(x, u32)


def _unpack(x):
    return pltpu.bitcast(x, bf16)


def _recip(x):
    r = pl.reciprocal(x, approx=True)
    return r * (2.0 - x * r)


def _layernorm(x):
    m = jnp.mean(x, axis=-1, keepdims=True)
    xc = x - m
    v = jnp.mean(xc * xc, axis=-1, keepdims=True)
    return xc * lax.rsqrt(v + 1e-5)


def _freduce(x3, op):
    r = op(op(op(x3[0], x3[1]), op(x3[2], x3[3])), x3[4])
    r = op(r, pltpu.roll(r, 2, 0))
    return op(r, pltpu.roll(r, 4, 0))


def _hedgehog(p):
    t = p.shape[1]
    p3 = p.reshape(GR // 8, 8, t)
    ep = jnp.exp2(p3 - _freduce(p3, jnp.maximum)[None])
    en = jnp.exp2(_freduce(p3, jnp.minimum)[None] - p3)
    ep = ep * _recip(_freduce(ep, jnp.add))[None]
    en = en * _recip(_freduce(en, jnp.add))[None]
    return jnp.concatenate([ep.reshape(GR, t), en.reshape(GR, t)], axis=0).astype(bf16)


def _stage_q(y):
    lo = lax.broadcasted_iota(i32, (y.shape[0], 128), 1) < 64
    y = y * QSCALE
    qm = y[:, 128:256]
    return jnp.concatenate([y[:, :128], jnp.where(lo, qm, 0.0), jnp.where(lo, 0.0, qm), y[:, 256:]], axis=1)


def _after(x, dep, zero):
    d = pltpu.bitcast(dep, i32) & zero
    return pltpu.bitcast(pltpu.bitcast(x, i32) | jnp.concatenate([d] * (x.shape[1] // 128), axis=1), f32)


def _b_schedule(period, tail):
    if "O" not in period:
        period += " O0"
    ops = [(t[0], int(t[1:])) for t in period.split()]
    maxlag = max(lag for _, lag in ops)
    merged, tail = tail[-1], tail[:-1]
    assert len(tail) == maxlag + 1
    nin = NP - sum(tail) - merged
    out, o = [], 0
    for t in range(NP + maxlag + 1):
        if t >= NP:
            out += [("O", o + i) for i in range(tail[t - NP])]
            o += tail[t - NP]
        for op, lag in ops:
            if op != "O":
                if 0 <= t - lag < NP:
                    out.append((op, t - lag))
            elif NP - nin <= t < NP:
                out.append(("O", o))
                o += 1
    if merged:
        out.append(("M", o))
    return out


def _kernel(x_hbm, wqkv_hbm, wphi_hbm, wo_hbm, mem_hbm, bq_hbm, bk_hbm, bv_hbm, bo_hbm,
            out_hbm,
            xin, wqkv_v, wphi_v, wo_v, mem_v, xa, xna, xnb, wq_s, wkv_s, ylast, kv_acc, kv_s,
            stage, wb_s, bo_v, bo_s, sv_o, sv_e, sv_q, sems):
    def copy(src, dst, slot):
        return pltpu.make_async_copy(src, dst, sems.at[slot])

    def a_copy(t, slot):
        return copy(wqkv_hbm.at[:, pl.ds(t * D, D)], wqkv_v.at[t], slot)

    def x_copy(r0, n, slot):
        return copy(x_hbm.at[pl.ds(r0, n)], xin.at[pl.ds(r0, n)], slot)

    def w_start(q0, q1, slot):
        while q0 < q1:
            t, j = divmod(q0, NP)
            n = min(q1 - q0, NP - j)
            if t < 2:
                copy((bq_hbm, bk_hbm)[t].at[pl.ds(j, n)], stage.at[pl.ds(q0, n)], slot).start()
            else:
                for hh in range(2):
                    copy(bv_hbm.at[pl.ds(j, n), hh], stage.at[pl.ds(q0, n), :, hh], slot).start()
            q0 += n

    def bo_copy(b):
        rows = pl.ds(pl.multiple_of(b * (HE // NWO), HE // NWO), HE // NWO)
        return copy(bo_hbm.at[rows], bo_v.at[rows], SEM_WO + b)

    def out_copy(b):
        rows = pl.ds(pl.multiple_of(b * TB, TB), TB)
        return copy(xin.at[rows], out_hbm.at[rows], SEM_OUT)

    first_copies = [a_copy(2, SEM_QV), a_copy(0, SEM_QV), x_copy(0, TS1, SEM_QV), copy(mem_hbm, mem_v, SEM_QV)]
    copy(wphi_hbm, wphi_v, SEM_PHI).start()
    a_copy(1, SEM_K).start()
    for cp in first_copies:
        cp.start()
    for b in range(NB):
        x_copy(b * TA + TS1, TA if b + 1 < NB else TA - TS1, SEM_X + b).start()
    copy(wo_hbm, wo_v, SEM_X + NB - 1).start()
    for b in range(NB):
        w_start(b * WI, (b + 1) * WI, SEM_W + b)
    for b in range(NWO):
        bo_copy(b).start()

    kv_acc[...] = jnp.zeros_like(kv_acc)
    ylast[...] = jnp.zeros_like(ylast)
    copy(wphi_hbm, wphi_v, SEM_PHI).wait()
    row = lax.broadcasted_iota(i32, (AH, D), 0)
    col = lax.broadcasted_iota(i32, (AH, D), 1)
    dsel = col - AD * row
    wf = None
    for d in range(AD):
        y = _dot(wphi_v[d], (dsel == d).astype(bf16))
        wf = y if wf is None else y + wf
    wf = wf.astype(bf16)
    row = lax.broadcasted_iota(i32, (CR, AD), 0)
    col = lax.broadcasted_iota(i32, (CR, AD), 1)
    sel = (((row % GR) // 2) == col).astype(bf16)
    row = lax.broadcasted_iota(i32, (CR, 256), 0)
    col = lax.broadcasted_iota(i32, (CR, 256), 1)
    head = (row // GR) * 2 + row % 2
    phit = []
    for c in range(NC):
        rep = _dot(sel, wf[:, c * 128:c * 128 + 256])
        keep = (head + c * 2 * CG) == (col + c * 128) // AD
        phit.append(jnp.where(keep, rep, 0.0).astype(bf16))

    def fold(t, c):
        return _pack((_dot_nt(phit[c], wqkv_v[t, :, c * 128:c * 128 + 256]) * LOG2E).astype(bf16))

    a_copy(1, SEM_K).wait()
    for c in range(NC):
        wkv_s[c, :CR // 2] = fold(1, c)
    for cp in first_copies:
        cp.wait()
    wvt = wqkv_v[2].T
    for c in range(NC):
        wkv_s[c, CR // 2:] = _pack(wvt[c * CR:(c + 1) * CR])
        wq_s[c] = fold(0, c)

    def layer_a(li):
        first = li == 0

        def ln_rows(r0, n):
            rows = pl.ds(pl.multiple_of(r0, n), n)
            xn = _layernorm(xin[rows, :].astype(f32)).astype(bf16)
            xna[pl.ds(pl.multiple_of(r0 // 2, n // 2), n // 2), :] = _pack(xn)
            return xn

        def xn_rows(r0, n):
            return _unpack(xna[pl.ds(pl.multiple_of(r0 // 2, n // 2), n // 2), :])

        def kv_update(c, y, ones):
            for u in range(CG):
                phi = _hedgehog(y[u * GR:(u + 1) * GR])
                vt = jnp.concatenate([y[CR + u * GR:CR + (u + 1) * GR], ones], axis=0).astype(bf16)
                kv_acc[c * CG + u] += _dot_nt(vt, phi)

        def pass1(i, carry):
            @pl.when(first)
            def _():
                @pl.when(i + 1 < NB)
                def _():
                    x_copy(pl.multiple_of(i * TA + TS1, TS1), TA, SEM_X + i).wait()

                @pl.when(i + 1 == NB)
                def _():
                    x_copy(S - TA + TS1, TA - TS1, SEM_X + NB - 1).wait()
                    copy(wo_hbm, wo_v, SEM_X + NB - 1).wait()

            ones = jnp.ones((8, TS1), f32)
            pend = (NC - 1, ylast[...], jnp.where(i > 0, ones, 0.0))
            for s in range(TA // TS1):
                r0 = i * TA + s * TS1
                xn = xn_rows(r0, TS1) if s == 0 else ln_rows(r0, TS1)
                for c in range(NC):
                    y = _dot_nt(_unpack(wkv_s[c]), xn)
                    kv_update(*pend)
                    pend = (c, y, ones)
            ylast[...] = pend[1]
            ln_rows(jnp.minimum(i + 1, NB - 1) * TA, TS1)
            return carry

        def pass2(i, carry):
            @pl.when(first)
            def _():
                chunk = stage.at[pl.ds(i * WI, WI)]
                copy(chunk, chunk, SEM_W + i).wait()

            sub = lax.broadcasted_iota(i32, (8, TS2), 0) < 4
            ot = {}

            def feat(s, c, p):
                for u in range(CG):
                    g = c * CG + u
                    y = _dot(kv_s[g], _hedgehog(p[u * GR:(u + 1) * GR]))
                    r = _recip(y[GR:] + 1e-6)
                    rr = pltpu.roll(r, 4, 0)
                    r0, r1 = jnp.where(sub, r, rr), jnp.where(sub, rr, r)
                    ot[s, g] = y[:GR] * jnp.concatenate([r0, r0, r, r1, r1], axis=0)

            def back(s, half, fill=()):
                lo = half * 128
                o = jnp.concatenate([ot[s, g][:, lo:lo + 128] for g in range(NG)], axis=0).T.astype(bf16)
                rows = pl.ds(pl.multiple_of(i * TA + s * TS2 + lo, 128), 128)
                ys = []
                for n in range(5) if fill else ():
                    ys.append(_dot(o, wo_v[:, n * 128:(n + 1) * 128]))
                    if fill[n] is not None:
                        q_piece(*fill[n])
                y = jnp.concatenate(ys, axis=1) if fill else _dot(o, wo_v[...])
                xa[rows, :] = xin[rows, :].astype(f32) + y

            for u in range(WI):
                wb_s[i * WI + u] = _pack(stage[i * WI + u].reshape(PW, D).T)
            kv_acc[...] = jnp.zeros_like(kv_acc)
            ylast[...] = jnp.zeros_like(ylast)
            pend = []
            for s in range(2):
                xn = xn_rows(i * TA + s * TS2, TS2)
                for c in range(NC):
                    pend.append((s, c, _dot_nt(_unpack(wq_s[c]), xn)))
                    if len(pend) > 2:
                        feat(*pend.pop(0))
            back(0, 0)
            while pend:
                feat(*pend.pop(0))
            xn0 = _layernorm(xa[0:64, :])
            xnb[...] = xn0
            h8 = xn0[0:16].astype(bf16)
            qparts = {}

            def q_piece(u, n):
                j = i * (NP // NB) + u
                qparts[u, n] = _dot_nt(h8, stage[j, n].reshape(128, D))[:8]
                if n == 2:
                    sv_q[j, 8:16, :] = _stage_q(jnp.concatenate([qparts[u, m] for m in range(3)], axis=1))

            fill = [None, None] + [(u, n) for u in range(NP // NB) for n in range(3)] + [None]
            back(0, 1, fill[0:5])
            back(1, 0, fill[5:10])
            back(1, 1, fill[10:15])
            return carry

        ln_rows(0, TS1)
        lax.fori_loop(0, NB, pass1, 0)
        kv_update(NC - 1, ylast[...], jnp.ones((8, TS1), f32))
        row = lax.broadcasted_iota(i32, (GR + 8, 2 * GR), 0)
        col = lax.broadcasted_iota(i32, (GR + 8, 2 * GR), 1)
        keep = jnp.where(row < GR, row // AD, (row - GR) // 4) == col % 2
        for g in range(NG):
            kv_s[g] = jnp.where(keep, kv_acc[g], 0.0).astype(bf16)
        lax.fori_loop(0, NB, pass2, 0)

        @pl.when(first)
        def _():
            def repack(b, carry):
                bo_copy(b).wait()
                for u in range(NP // NWO):
                    j = b * (NP // NWO) + u
                    rows = [bo_v[pl.ds(pl.multiple_of(j * PW + hh * BE + cb * 64, 64), 64), :]
                            for cb in range(3) for hh in range(2)]
                    bo_s[j] = _pack(jnp.concatenate(rows, axis=0))
                return carry
            lax.fori_loop(0, NWO, repack, 0)

    def layer_b(li):
        lo40 = lax.broadcasted_iota(i32, (L, 128), 1) < 64
        zero40 = jnp.zeros((L, 128), f32)
        pad = jnp.zeros((128 - 2 * L, PW), f32)

        def blockdiag_k(k):
            kmid = k[:, 128:256]
            top = jnp.concatenate([k[:, :128], jnp.where(lo40, kmid, zero40), zero40], axis=1)
            bot = jnp.concatenate([zero40, jnp.where(lo40, zero40, kmid), k[:, 256:]], axis=1)
            return jnp.concatenate([top, bot, pad], axis=0).astype(bf16)

        def blockdiag_v(v):
            t = [v[:, cb * 128:(cb + 1) * 128] for cb in range(3)]
            top = jnp.concatenate([jnp.where(lo40, x, zero40) for x in t], axis=1)
            bot = jnp.concatenate([jnp.where(lo40, zero40, x) for x in t], axis=1)
            return jnp.concatenate([top, bot, pad], axis=0).astype(bf16)

        r = lax.broadcasted_iota(i32, (32, 128), 0)
        c = lax.broadcasted_iota(i32, (32, 128), 1)
        isa = c < L
        key = jnp.where(isa, c, c - L)
        valid = ((r < M) | (r >= key) | (key >= 32)) & (key < L)
        sub = lax.broadcasted_iota(i32, (8, 128), 0)
        lo8 = lax.broadcasted_iota(i32, (8, 128), 1) < 64

        def head8(q, kv, j):
            def bcast(t, cb):
                return jnp.broadcast_to(kv[j, t:t + 1, cb * 128:(cb + 1) * 128], (8, 128))

            q0, qa, qb, q2 = [q[:, cb * 128:(cb + 1) * 128] for cb in range(4)]
            cs = []
            for t in range(16):
                k1 = bcast(t, 1)
                sa = jnp.sum(q0 * bcast(t, 0) + qa * k1, axis=1, keepdims=True)
                sb = jnp.sum(q2 * bcast(t, 2) + qb * k1, axis=1, keepdims=True)
                s = jnp.where(lo8, sa, sb)
                cs.append(jnp.where(sub >= t - 8, s, MASKED) if t > 8 else s)
            m = cs
            while len(m) > 1:
                m = [jnp.maximum(m[a], m[a + 1]) for a in range(0, len(m), 2)]
            l, acc = None, None
            for t in range(16):
                e = jnp.exp2(cs[t] - m[0])
                pv = [e * bcast(t, 3 + cb) for cb in range(3)]
                l = e if l is None else l + e
                acc = pv if acc is None else [a + b for a, b in zip(acc, pv)]
            rl = _recip(l)
            return jnp.concatenate([a * rl for a in acc], axis=1)

        def softmax(s):
            s = jnp.where(valid, s * QSCALE, MASKED)
            ma = jnp.max(jnp.where(isa, s, -jnp.inf), axis=1, keepdims=True)
            mb = jnp.max(jnp.where(isa, -jnp.inf, s), axis=1, keepdims=True)
            e = jnp.exp2(s - jnp.where(isa, ma, mb))
            la = jnp.sum(jnp.where(isa, e, 0.0), axis=1, keepdims=True)
            lb = jnp.sum(jnp.where(isa, 0.0, e), axis=1, keepdims=True)
            return e * _recip(jnp.where(isa, la, lb))

        def step(h, even, u, zero, o1e):
            first, last = even and u == 0, (not even) and u == UB - 1
            eo = "e" if even else "o"

            def opt(name):
                return CFG.get(name + eo + str(u), CFG[name + eo])

            period = opt("p")
            sched = _b_schedule(period, CFG["tl"] if last else opt("t"))
            widx = dict(q=0, k=NP, v=2 * NP)
            kv = sv_e if even else sv_o

            def proj(op, j, k0, k1, n0=0, n1=3):
                hh = h if (op == "q") != even else h[:32]
                w = wb_s[widx[op] + j, k0 * 64:k1 * 64, n0 * 128:n1 * 128]
                return _dot(hh[:, k0 * 128:k1 * 128], _unpack(w))

            part, kdone = {}, 0
            for k1 in (() if first else (2, 3)):
                for op in dict.fromkeys(op for op, j in sched if op in widx and j == 0):
                    y = proj(op, 0, kdone, k1)
                    part[op] = y + part[op] if op in part else y
                kdone = k1

            val, acc, o1 = {}, None, {}

            def lhs_o(j):
                o = val.pop(("o", j))
                if even:
                    return o
                return jnp.concatenate([o, jnp.concatenate([o1e[j], o1[j]], axis=0).astype(bf16)], axis=0)

            for op, j in sched:
                if op in widx:
                    done = val.setdefault((op, j, "n"), [])
                    n0, n1 = (len(done), len(done) + 1) if period.count(op) == 3 else (0, 3)
                    if j == 0 and part:
                        done.append(proj(op, j, kdone, 5, n0, n1) + part[op][:, n0 * 128:n1 * 128])
                    else:
                        done.append(proj(op, j, 0, 5, n0, n1))
                    if "waiting" in val:
                        val["gate", val.pop("waiting")] = done[-1][:8, :128]
                    if n1 < 3:
                        continue
                    y = jnp.concatenate(done, axis=1)
                    if op == "q":
                        val["q", j] = y[:32]
                        if not even:
                            sv_q[j] = _stage_q(y[32:])
                        continue
                    cols = slice(0, PW) if op == "k" else slice(PW, 2 * PW)
                    kv[j, 0:8, cols] = y[0:8]
                    if even:
                        sv_e[j, 8:16, cols] = y[32:40]
                        sv_o[j, 8:16, cols] = y[40:48]
                        y = y[:40]
                    else:
                        y = jnp.concatenate([y, sv_o[j, 8:16, cols]], axis=0)
                    val[op, j] = blockdiag_k(y) if op == "k" else blockdiag_v(y)
                    if opt("g") == op or (opt("g") == "b" and ("k", j) in val and ("v", j) in val):
                        val["waiting"] = j
                elif op == "S":
                    q1 = sv_q[j, 8:16, :] if even else sv_q[j, 0:8, :]
                    if ("gate", j) in val:
                        q1 = _after(q1, val.pop(("gate", j)), zero)
                    o1[j] = head8(q1, kv, j)
                    val["p", j] = softmax(_dot_nt(val.pop(("q", j)).astype(bf16), val.pop(("k", j))))
                elif op == "P":
                    p = val.pop(("p", j))
                    if j - opt("d") in o1:
                        dep = o1[j - opt("d")]
                        dep = dep[:, :128] + dep[:, 128:256] + dep[:, 256:]
                        p = jnp.concatenate([_after(p[:8], dep, zero), p[8:]], axis=0)
                    val["o", j] = _dot(p.astype(bf16), val.pop(("v", j))).astype(bf16)
                elif op == "M":
                    o = jnp.concatenate([lhs_o(jj) for jj in range(j, NP)], axis=1)
                    acc = _dot(o, _unpack(jnp.concatenate([bo_s[jj] for jj in range(j, NP)], axis=0))) + acc
                else:
                    y = _dot(lhs_o(j), _unpack(bo_s[j]))
                    acc = y if acc is None else y + acc
                    if "waiting" in val:
                        val["gate", val.pop("waiting")] = acc[:8, :128]
            return acc, o1

        def body(i, mem):
            zero = i // NI
            rn = pl.multiple_of(jnp.minimum(i + 1, NI - 1) * TB, TB)
            xns = [xnb[...]] + [_layernorm(xa[pl.ds(pl.multiple_of((i * UB + u) * 64, 64), 64), :])
                                for u in range(1, UB)]
            xns.append(_layernorm(xa[pl.ds(rn, 64), :]))
            for u in range(UB):
                r0 = pl.multiple_of((i * UB + u) * 64, 64)

                def add_rows(off, y):
                    rows = pl.ds(r0 + off, y.shape[0])
                    xin[rows, :] = (xa[rows, :] + y).astype(bf16)

                xn = xns[u]
                h = jnp.concatenate([mem, xn[8:32], xn[0:8], xn[32:40]], axis=0).astype(bf16)
                ye, o1e = step(h, True, u, zero, None)
                mem = ye[:8]
                add_rows(16, ye[16:])
                h = jnp.concatenate([mem, xn[40:64], xn[32:40], xns[u + 1][0:8]], axis=0).astype(bf16)
                yo, _ = step(h, False, u, zero, o1e)
                mem = yo[:8]
                add_rows(48, yo[16:32])
                add_rows(0, jnp.concatenate([yo[32:40], ye[8:16]], axis=0))
                add_rows(32, jnp.concatenate([yo[40:48], yo[8:16]], axis=0))
            xnb[...] = xns[UB]

            @pl.when(li == 1)
            def _():
                out_copy(i).start()
            return mem

        lax.fori_loop(0, CFG.get("NIT", NI), body, mem_v[...].astype(f32))

    def layer(li, carry):
        layer_a(li)
        layer_b(li)
        return carry

    lax.fori_loop(0, 2, layer, 0)
    nrows = CFG.get("NIT", NI) * TB
    copy(xin.at[pl.ds(0, nrows)], out_hbm.at[pl.ds(0, nrows)], SEM_OUT).wait()


@jax.jit
def pallas_interleave_layers__linear_kernel_hedgehog__memory_aug_recurrent_mem_tr__prompt_kernel(
    A_x: jax.Array,
    A_wqkv: jax.Array,
    A_w_phi: jax.Array,
    A_wo: jax.Array,
    B_x: jax.Array,
    B_mem0: jax.Array,
    B_Wq: jax.Array,
    B_Wk: jax.Array,
    B_Wv: jax.Array,
    B_Wo: jax.Array,
    B_seg_len=SEG,
):
    del B_x, B_seg_len
    x = A_x.reshape(S, D)
    wphi = A_w_phi.transpose(1, 2, 0)
    mem0 = B_mem0.reshape(M, D)
    bq = B_Wq.transpose(1, 2, 0).reshape(NP, 3, 2, 64, D)
    bk = B_Wk.transpose(1, 2, 0).reshape(NP, 3, 2, 64, D)
    bv = B_Wv.transpose(1, 2, 0).reshape(NP, 2, 3, 64, D)
    bo = B_Wo.reshape(HE, D)

    anyspec = pl.BlockSpec(memory_space=pl.ANY)
    out = pl.pallas_call(
        _kernel,
        out_shape=jax.ShapeDtypeStruct((S, D), bf16),
        in_specs=[anyspec] * 9,
        out_specs=anyspec,
        scratch_shapes=[
            pltpu.VMEM((S, D), bf16),
            pltpu.VMEM((3, D, D), bf16),
            pltpu.VMEM((AD, AD, AH), bf16),
            pltpu.VMEM((D, D), bf16),
            pltpu.VMEM((M, D), bf16),
            pltpu.VMEM((S, D), f32),
            pltpu.VMEM((S // 2, D), u32),
            pltpu.VMEM((64, D), f32),
            pltpu.VMEM((NC, CR // 2, D), u32),
            pltpu.VMEM((NC, CR, D), u32),
            pltpu.VMEM((2 * CR, TS1), f32),
            pltpu.VMEM((NG, GR + 8, 2 * GR), f32),
            pltpu.VMEM((NG, GR + 8, 2 * GR), bf16),
            pltpu.VMEM((NW, 3, 2, 64, D), bf16),
            pltpu.VMEM((NW, D // 2, PW), u32),
            pltpu.VMEM((HE, D), bf16),
            pltpu.VMEM((NP, PW // 2, D), u32),
            pltpu.VMEM((NP, 16, 2 * PW), f32),
            pltpu.VMEM((NP, 16, 2 * PW), f32),
            pltpu.VMEM((NP, 16, 512), f32),
            pltpu.SemaphoreType.DMA((NSEM,)),
        ],
        compiler_params=pltpu.CompilerParams(vmem_limit_bytes=110 * 1024 * 1024,
                                             disable_bounds_checks=True),
    )(x, A_wqkv, wphi, A_wo, mem0, bq, bk, bv, bo)
    return out.reshape(1, S, D)
```

```python
import jax
import jax.numpy as jnp
from jax import lax
import jax.experimental.pallas as pl
import jax.experimental.pallas.tpu as pltpu

bf16 = jnp.bfloat16
f32 = jnp.float32
u32 = jnp.uint32
i32 = jnp.int32

CFG = dict(
    pe="k0 q0 v0 S1 P2", po="q0 k0 q0 S1 v0 q0 P3",
    te=(3, 4, 2, 3), to=(1, 2, 2, 1, 2), tl=(2, 2, 1, 2, 0),
    de=1, do=0, ge="b", go="b",
)
CFG.update(po1='k0 q0 S1 q0 v0 q0 P2', tl=(1, 3, 2, 0), go1='k')

S = 2048
D = 640
LOG2E = 1.4426950408889634
AH = 32
AD = 20
GR = 2 * AD
NG = AH // 2
CG = 4
CR = CG * GR
NC = NG // CG
TA = 512
TS1 = 128
TS2 = 256
NB = S // TA
BH = 32
BE = 192
HE = BH * BE
M = 8
SEG = 32
L = M + SEG
NP = BH // 2
PW = 2 * BE
QSCALE = BE ** -0.5 * LOG2E
MASKED = -1e9 * LOG2E
UB = 2
TB = 64 * UB
NI = S // TB
NW = 3 * NP
WI = NW // NB
NWO = 16

NT = (((1,), (1,)), ((), ()))

SEM_PHI, SEM_K, SEM_QV, SEM_OUT = 0, 1, 2, 3
SEM_X = 4
SEM_W = SEM_X + NB
SEM_WO = SEM_W + NB
NSEM = SEM_WO + NWO


def _dot(a, b):
    return jnp.dot(a, b, preferred_element_type=f32)


def _dot_nt(a, b):
    return lax.dot_general(a, b, NT, preferred_element_type=f32)


def _pack(x):
    return pltpu.bitcast(x, u32)


def _unpack(x):
    return pltpu.bitcast(x, bf16)


def _recip(x):
    r = pl.reciprocal(x, approx=True)
    return r * (2.0 - x * r)


def _layernorm(x):
    m = jnp.mean(x, axis=-1, keepdims=True)
    xc = x - m
    v = jnp.mean(xc * xc, axis=-1, keepdims=True)
    return xc * lax.rsqrt(v + 1e-5)


def _freduce(x3, op):
    r = op(op(op(x3[0], x3[1]), op(x3[2], x3[3])), x3[4])
    r = op(r, pltpu.roll(r, 2, 0))
    return op(r, pltpu.roll(r, 4, 0))


def _hedgehog(p):
    t = p.shape[1]
    p3 = p.reshape(GR // 8, 8, t)
    ep = jnp.exp2(p3 - _freduce(p3, jnp.maximum)[None])
    en = jnp.exp2(_freduce(p3, jnp.minimum)[None] - p3)
    ep = ep * _recip(_freduce(ep, jnp.add))[None]
    en = en * _recip(_freduce(en, jnp.add))[None]
    return jnp.concatenate([ep.reshape(GR, t), en.reshape(GR, t)], axis=0).astype(bf16)


def _stage_q(y):
    lo = lax.broadcasted_iota(i32, (y.shape[0], 128), 1) < 64
    y = y * QSCALE
    qm = y[:, 128:256]
    return jnp.concatenate([y[:, :128], jnp.where(lo, qm, 0.0), jnp.where(lo, 0.0, qm), y[:, 256:]], axis=1)


def _after(x, dep, zero):
    d = pltpu.bitcast(dep, i32) & zero
    return pltpu.bitcast(pltpu.bitcast(x, i32) | jnp.concatenate([d] * (x.shape[1] // 128), axis=1), f32)


def _b_schedule(period, tail):
    if "O" not in period:
        period += " O0"
    ops = [(t[0], int(t[1:])) for t in period.split()]
    maxlag = max(lag for _, lag in ops)
    merged, tail = tail[-1], tail[:-1]
    assert len(tail) == maxlag + 1
    nin = NP - sum(tail) - merged
    out, o = [], 0
    for t in range(NP + maxlag + 1):
        if t >= NP:
            out += [("O", o + i) for i in range(tail[t - NP])]
            o += tail[t - NP]
        for op, lag in ops:
            if op != "O":
                if 0 <= t - lag < NP:
                    out.append((op, t - lag))
            elif NP - nin <= t < NP:
                out.append(("O", o))
                o += 1
    if merged:
        out.append(("M", o))
    return out


def _kernel(x_hbm, wqkv_hbm, wphi_hbm, wo_hbm, mem_hbm, bq_hbm, bk_hbm, bv_hbm, bo_hbm,
            out_hbm,
            xin, wqkv_v, wphi_v, wo_v, mem_v, xa, xna, xnb, wq_s, wkv_s, ylast, kv_acc, kv_s,
            stage, wb_s, bo_v, bo_s, sv_o, sv_e, sv_q, sems):
    def copy(src, dst, slot):
        return pltpu.make_async_copy(src, dst, sems.at[slot])

    def a_copy(t, slot):
        return copy(wqkv_hbm.at[:, pl.ds(t * D, D)], wqkv_v.at[t], slot)

    def x_copy(r0, n, slot):
        return copy(x_hbm.at[pl.ds(r0, n)], xin.at[pl.ds(r0, n)], slot)

    def w_start(q0, q1, slot):
        while q0 < q1:
            t, j = divmod(q0, NP)
            n = min(q1 - q0, NP - j)
            if t < 2:
                copy((bq_hbm, bk_hbm)[t].at[pl.ds(j, n)], stage.at[pl.ds(q0, n)], slot).start()
            else:
                for hh in range(2):
                    copy(bv_hbm.at[pl.ds(j, n), hh], stage.at[pl.ds(q0, n), :, hh], slot).start()
            q0 += n

    def bo_copy(b):
        rows = pl.ds(pl.multiple_of(b * (HE // NWO), HE // NWO), HE // NWO)
        return copy(bo_hbm.at[rows], bo_v.at[rows], SEM_WO + b)

    def out_copy(b):
        rows = pl.ds(pl.multiple_of(b * TB, TB), TB)
        return copy(xin.at[rows], out_hbm.at[rows], SEM_OUT)

    first_copies = [a_copy(2, SEM_QV), a_copy(0, SEM_QV), x_copy(0, TS1, SEM_QV), copy(mem_hbm, mem_v, SEM_QV)]
    copy(wphi_hbm, wphi_v, SEM_PHI).start()
    a_copy(1, SEM_K).start()
    for cp in first_copies:
        cp.start()
    for b in range(NB):
        x_copy(b * TA + TS1, TA if b + 1 < NB else TA - TS1, SEM_X + b).start()
    copy(wo_hbm, wo_v, SEM_X + NB - 1).start()
    for b in range(NB):
        w_start(b * WI, (b + 1) * WI, SEM_W + b)
    for b in range(NWO):
        bo_copy(b).start()

    kv_acc[...] = jnp.zeros_like(kv_acc)
    ylast[...] = jnp.zeros_like(ylast)
    copy(wphi_hbm, wphi_v, SEM_PHI).wait()
    row = lax.broadcasted_iota(i32, (AH, D), 0)
    col = lax.broadcasted_iota(i32, (AH, D), 1)
    dsel = col - AD * row
    wf = None
    for d in range(AD):
        y = _dot(wphi_v[d], (dsel == d).astype(bf16))
        wf = y if wf is None else y + wf
    wf = wf.astype(bf16)
    row = lax.broadcasted_iota(i32, (CR, AD), 0)
    col = lax.broadcasted_iota(i32, (CR, AD), 1)
    sel = (((row % GR) // 2) == col).astype(bf16)
    row = lax.broadcasted_iota(i32, (CR, 256), 0)
    col = lax.broadcasted_iota(i32, (CR, 256), 1)
    head = (row // GR) * 2 + row % 2
    phit = []
    for c in range(NC):
        rep = _dot(sel, wf[:, c * 128:c * 128 + 256])
        keep = (head + c * 2 * CG) == (col + c * 128) // AD
        phit.append(jnp.where(keep, rep, 0.0).astype(bf16))

    def fold(t, c):
        return _pack((_dot_nt(phit[c], wqkv_v[t, :, c * 128:c * 128 + 256]) * LOG2E).astype(bf16))

    a_copy(1, SEM_K).wait()
    for c in range(NC):
        wkv_s[c, :CR // 2] = fold(1, c)
    for cp in first_copies:
        cp.wait()
    wvt = wqkv_v[2].T
    for c in range(NC):
        wkv_s[c, CR // 2:] = _pack(wvt[c * CR:(c + 1) * CR])
        wq_s[c] = fold(0, c)

    def layer_a(li):
        first = li == 0

        def ln_rows(r0, n):
            rows = pl.ds(pl.multiple_of(r0, n), n)
            xn = _layernorm(xin[rows, :].astype(f32)).astype(bf16)
            xna[pl.ds(pl.multiple_of(r0 // 2, n // 2), n // 2), :] = _pack(xn)
            return xn

        def xn_rows(r0, n):
            return _unpack(xna[pl.ds(pl.multiple_of(r0 // 2, n // 2), n // 2), :])

        def kv_update(c, y, ones):
            for u in range(CG):
                phi = _hedgehog(y[u * GR:(u + 1) * GR])
                vt = jnp.concatenate([y[CR + u * GR:CR + (u + 1) * GR], ones], axis=0).astype(bf16)
                kv_acc[c * CG + u] += _dot_nt(vt, phi)

        def pass1(i, carry):
            @pl.when(first)
            def _():
                @pl.when(i + 1 < NB)
                def _():
                    x_copy(pl.multiple_of(i * TA + TS1, TS1), TA, SEM_X + i).wait()

                @pl.when(i + 1 == NB)
                def _():
                    x_copy(S - TA + TS1, TA - TS1, SEM_X + NB - 1).wait()
                    copy(wo_hbm, wo_v, SEM_X + NB - 1).wait()

            ones = jnp.ones((8, TS1), f32)
            pend = (NC - 1, ylast[...], jnp.where(i > 0, ones, 0.0))
            for s in range(TA // TS1):
                r0 = i * TA + s * TS1
                xn = xn_rows(r0, TS1) if s == 0 else ln_rows(r0, TS1)
                for c in range(NC):
                    y = _dot_nt(_unpack(wkv_s[c]), xn)
                    kv_update(*pend)
                    pend = (c, y, ones)
            ylast[...] = pend[1]
            ln_rows(jnp.minimum(i + 1, NB - 1) * TA, TS1)
            return carry

        def pass2(i, carry):
            @pl.when(first)
            def _():
                chunk = stage.at[pl.ds(i * WI, WI)]
                copy(chunk, chunk, SEM_W + i).wait()

            sub = lax.broadcasted_iota(i32, (8, TS2), 0) < 4
            ot = {}

            def feat(s, c, p):
                for u in range(CG):
                    g = c * CG + u
                    y = _dot(kv_s[g], _hedgehog(p[u * GR:(u + 1) * GR]))
                    r = _recip(y[GR:] + 1e-6)
                    rr = pltpu.roll(r, 4, 0)
                    r0, r1 = jnp.where(sub, r, rr), jnp.where(sub, rr, r)
                    ot[s, g] = y[:GR] * jnp.concatenate([r0, r0, r, r1, r1], axis=0)

            def back(s, half, fill=()):
                lo = half * 128
                o = jnp.concatenate([ot[s, g][:, lo:lo + 128] for g in range(NG)], axis=0).T.astype(bf16)
                rows = pl.ds(pl.multiple_of(i * TA + s * TS2 + lo, 128), 128)
                ys = []
                for n in range(5) if fill else ():
                    ys.append(_dot(o, wo_v[:, n * 128:(n + 1) * 128]))
                    if fill[n] is not None:
                        q_piece(*fill[n])
                y = jnp.concatenate(ys, axis=1) if fill else _dot(o, wo_v[...])
                xa[rows, :] = xin[rows, :].astype(f32) + y

            for u in range(WI):
                wb_s[i * WI + u] = _pack(stage[i * WI + u].reshape(PW, D).T)
            kv_acc[...] = jnp.zeros_like(kv_acc)
            ylast[...] = jnp.zeros_like(ylast)
            pend = []
            for s in range(2):
                xn = xn_rows(i * TA + s * TS2, TS2)
                for c in range(NC):
                    pend.append((s, c, _dot_nt(_unpack(wq_s[c]), xn)))
                    if len(pend) > 2:
                        feat(*pend.pop(0))
            back(0, 0)
            while pend:
                feat(*pend.pop(0))
            xn0 = _layernorm(xa[0:64, :])
            xnb[...] = xn0
            h8 = xn0[0:16].astype(bf16)
            qparts = {}

            def q_piece(u, n):
                j = i * (NP // NB) + u
                qparts[u, n] = _dot_nt(h8, stage[j, n].reshape(128, D))[:8]
                if n == 2:
                    sv_q[j, 8:16, :] = _stage_q(jnp.concatenate([qparts[u, m] for m in range(3)], axis=1))

            fill = [None, None] + [(u, n) for u in range(NP // NB) for n in range(3)] + [None]
            back(0, 1, fill[0:5])
            back(1, 0, fill[5:10])
            back(1, 1, fill[10:15])
            return carry

        ln_rows(0, TS1)
        lax.fori_loop(0, NB, pass1, 0)
        kv_update(NC - 1, ylast[...], jnp.ones((8, TS1), f32))
        row = lax.broadcasted_iota(i32, (GR + 8, 2 * GR), 0)
        col = lax.broadcasted_iota(i32, (GR + 8, 2 * GR), 1)
        keep = jnp.where(row < GR, row // AD, (row - GR) // 4) == col % 2
        for g in range(NG):
            kv_s[g] = jnp.where(keep, kv_acc[g], 0.0).astype(bf16)
        lax.fori_loop(0, NB, pass2, 0)

        @pl.when(first)
        def _():
            def repack(b, carry):
                bo_copy(b).wait()
                for u in range(NP // NWO):
                    j = b * (NP // NWO) + u
                    rows = [bo_v[pl.ds(pl.multiple_of(j * PW + hh * BE + cb * 64, 64), 64), :]
                            for cb in range(3) for hh in range(2)]
                    bo_s[j] = _pack(jnp.concatenate(rows, axis=0))
                return carry
            lax.fori_loop(0, NWO, repack, 0)

    def layer_b(li):
        lo40 = lax.broadcasted_iota(i32, (L, 128), 1) < 64
        zero40 = jnp.zeros((L, 128), f32)
        pad = jnp.zeros((128 - 2 * L, PW), f32)

        def blockdiag_k(k):
            kmid = k[:, 128:256]
            top = jnp.concatenate([k[:, :128], jnp.where(lo40, kmid, zero40), zero40], axis=1)
            bot = jnp.concatenate([zero40, jnp.where(lo40, zero40, kmid), k[:, 256:]], axis=1)
            return jnp.concatenate([top, bot, pad], axis=0).astype(bf16)

        def blockdiag_v(v):
            t = [v[:, cb * 128:(cb + 1) * 128] for cb in range(3)]
            top = jnp.concatenate([jnp.where(lo40, x, zero40) for x in t], axis=1)
            bot = jnp.concatenate([jnp.where(lo40, zero40, x) for x in t], axis=1)
            return jnp.concatenate([top, bot, pad], axis=0).astype(bf16)

        r = lax.broadcasted_iota(i32, (32, 128), 0)
        c = lax.broadcasted_iota(i32, (32, 128), 1)
        isa = c < L
        key = jnp.where(isa, c, c - L)
        valid = ((r < M) | (r >= key) | (key >= 32)) & (key < L)
        sub = lax.broadcasted_iota(i32, (8, 128), 0)
        lo8 = lax.broadcasted_iota(i32, (8, 128), 1) < 64

        def head8(q, kv, j):
            def bcast(t, cb):
                return jnp.broadcast_to(kv[j, t:t + 1, cb * 128:(cb + 1) * 128], (8, 128))

            q0, qa, qb, q2 = [q[:, cb * 128:(cb + 1) * 128] for cb in range(4)]
            cs = []
            for t in range(16):
                k1 = bcast(t, 1)
                sa = jnp.sum(q0 * bcast(t, 0) + qa * k1, axis=1, keepdims=True)
                sb = jnp.sum(q2 * bcast(t, 2) + qb * k1, axis=1, keepdims=True)
                s = jnp.where(lo8, sa, sb)
                cs.append(jnp.where(sub >= t - 8, s, MASKED) if t > 8 else s)
            m = cs
            while len(m) > 1:
                m = [jnp.maximum(m[a], m[a + 1]) for a in range(0, len(m), 2)]
            l, acc = None, None
            for t in range(16):
                e = jnp.exp2(cs[t] - m[0])
                pv = [e * bcast(t, 3 + cb) for cb in range(3)]
                l = e if l is None else l + e
                acc = pv if acc is None else [a + b for a, b in zip(acc, pv)]
            rl = _recip(l)
            return jnp.concatenate([a * rl for a in acc], axis=1)

        def softmax(s):
            s = jnp.where(valid, s * QSCALE, MASKED)
            ma = jnp.max(jnp.where(isa, s, -jnp.inf), axis=1, keepdims=True)
            mb = jnp.max(jnp.where(isa, -jnp.inf, s), axis=1, keepdims=True)
            e = jnp.exp2(s - jnp.where(isa, ma, mb))
            la = jnp.sum(jnp.where(isa, e, 0.0), axis=1, keepdims=True)
            lb = jnp.sum(jnp.where(isa, 0.0, e), axis=1, keepdims=True)
            return e * _recip(jnp.where(isa, la, lb))

        def step(h, even, u, zero, o1e):
            first, last = even and u == 0, (not even) and u == UB - 1
            eo = "e" if even else "o"

            def opt(name):
                return CFG.get(name + eo + str(u), CFG[name + eo])

            period = opt("p")
            sched = _b_schedule(period, CFG["tl"] if last else opt("t"))
            widx = dict(q=0, k=NP, v=2 * NP)
            kv = sv_e if even else sv_o

            def proj(op, j, k0, k1, n0=0, n1=3):
                hh = h if (op == "q") != even else h[:32]
                w = wb_s[widx[op] + j, k0 * 64:k1 * 64, n0 * 128:n1 * 128]
                return _dot(hh[:, k0 * 128:k1 * 128], _unpack(w))

            part, kdone = {}, 0
            for k1 in (() if first else (2, 3)):
                for op in dict.fromkeys(op for op, j in sched if op in widx and j == 0):
                    y = proj(op, 0, kdone, k1)
                    part[op] = y + part[op] if op in part else y
                kdone = k1

            val, acc, o1 = {}, None, {}

            def lhs_o(j):
                o = val.pop(("o", j))
                if even:
                    return o
                return jnp.concatenate([o, jnp.concatenate([o1e[j], o1[j]], axis=0).astype(bf16)], axis=0)

            for op, j in sched:
                if op in widx:
                    done = val.setdefault((op, j, "n"), [])
                    n0, n1 = (len(done), len(done) + 1) if period.count(op) == 3 else (0, 3)
                    if j == 0 and part:
                        done.append(proj(op, j, kdone, 5, n0, n1) + part[op][:, n0 * 128:n1 * 128])
                    else:
                        done.append(proj(op, j, 0, 5, n0, n1))
                    if "waiting" in val:
                        val["gate", val.pop("waiting")] = done[-1][:8, :128]
                    if n1 < 3:
                        continue
                    y = jnp.concatenate(done, axis=1)
                    if op == "q":
                        val["q", j] = y[:32]
                        if not even:
                            sv_q[j] = _stage_q(y[32:])
                        continue
                    cols = slice(0, PW) if op == "k" else slice(PW, 2 * PW)
                    kv[j, 0:8, cols] = y[0:8]
                    if even:
                        sv_e[j, 8:16, cols] = y[32:40]
                        sv_o[j, 8:16, cols] = y[40:48]
                        y = y[:40]
                    else:
                        y = jnp.concatenate([y, sv_o[j, 8:16, cols]], axis=0)
                    val[op, j] = blockdiag_k(y) if op == "k" else blockdiag_v(y)
                    if opt("g") == op or (opt("g") == "b" and ("k", j) in val and ("v", j) in val):
                        val["waiting"] = j
                elif op == "S":
                    q1 = sv_q[j, 8:16, :] if even else sv_q[j, 0:8, :]
                    if ("gate", j) in val:
                        q1 = _after(q1, val.pop(("gate", j)), zero)
                    o1[j] = head8(q1, kv, j)
                    val["p", j] = softmax(_dot_nt(val.pop(("q", j)).astype(bf16), val.pop(("k", j))))
                elif op == "P":
                    p = val.pop(("p", j))
                    if j - opt("d") in o1:
                        dep = o1[j - opt("d")]
                        dep = dep[:, :128] + dep[:, 128:256] + dep[:, 256:]
                        p = jnp.concatenate([_after(p[:8], dep, zero), p[8:]], axis=0)
                    val["o", j] = _dot(p.astype(bf16), val.pop(("v", j))).astype(bf16)
                elif op == "M":
                    o = jnp.concatenate([lhs_o(jj) for jj in range(j, NP)], axis=1)
                    acc = _dot(o, _unpack(jnp.concatenate([bo_s[jj] for jj in range(j, NP)], axis=0))) + acc
                else:
                    y = _dot(lhs_o(j), _unpack(bo_s[j]))
                    acc = y if acc is None else y + acc
                    if "waiting" in val:
                        val["gate", val.pop("waiting")] = acc[:8, :128]
            return acc, o1

        def body(i, mem):
            zero = i // NI
            rn = pl.multiple_of(jnp.minimum(i + 1, NI - 1) * TB, TB)
            xns = [xnb[...]] + [_layernorm(xa[pl.ds(pl.multiple_of((i * UB + u) * 64, 64), 64), :])
                                for u in range(1, UB)]
            xns.append(_layernorm(xa[pl.ds(rn, 64), :]))
            for u in range(UB):
                r0 = pl.multiple_of((i * UB + u) * 64, 64)

                def add_rows(off, y):
                    rows = pl.ds(r0 + off, y.shape[0])
                    xin[rows, :] = (xa[rows, :] + y).astype(bf16)

                xn = xns[u]
                h = jnp.concatenate([mem, xn[8:32], xn[0:8], xn[32:40]], axis=0).astype(bf16)
                ye, o1e = step(h, True, u, zero, None)
                mem = ye[:8]
                add_rows(16, ye[16:])
                h = jnp.concatenate([mem, xn[40:64], xn[32:40], xns[u + 1][0:8]], axis=0).astype(bf16)
                yo, _ = step(h, False, u, zero, o1e)
                mem = yo[:8]
                add_rows(48, yo[16:32])
                add_rows(0, jnp.concatenate([yo[32:40], ye[8:16]], axis=0))
                add_rows(32, jnp.concatenate([yo[40:48], yo[8:16]], axis=0))
            xnb[...] = xns[UB]

            @pl.when(li == 1)
            def _():
                out_copy(i).start()
            return mem

        lax.fori_loop(0, NI, body, mem_v[...].astype(f32))

    def layer(li, carry):
        layer_a(li)
        layer_b(li)
        return carry

    lax.fori_loop(0, 2, layer, 0)
    copy(xin, out_hbm, SEM_OUT).wait()


@jax.jit
def pallas_interleave_layers__linear_kernel_hedgehog__memory_aug_recurrent_mem_tr__prompt_kernel(
    A_x: jax.Array,
    A_wqkv: jax.Array,
    A_w_phi: jax.Array,
    A_wo: jax.Array,
    B_x: jax.Array,
    B_mem0: jax.Array,
    B_Wq: jax.Array,
    B_Wk: jax.Array,
    B_Wv: jax.Array,
    B_Wo: jax.Array,
    B_seg_len=SEG,
):
    del B_x, B_seg_len
    x = A_x.reshape(S, D)
    wphi = A_w_phi.transpose(1, 2, 0)
    mem0 = B_mem0.reshape(M, D)
    bq = B_Wq.transpose(1, 2, 0).reshape(NP, 3, 2, 64, D)
    bk = B_Wk.transpose(1, 2, 0).reshape(NP, 3, 2, 64, D)
    bv = B_Wv.transpose(1, 2, 0).reshape(NP, 2, 3, 64, D)
    bo = B_Wo.reshape(HE, D)

    anyspec = pl.BlockSpec(memory_space=pl.ANY)
    out = pl.pallas_call(
        _kernel,
        out_shape=jax.ShapeDtypeStruct((S, D), bf16),
        in_specs=[anyspec] * 9,
        out_specs=anyspec,
        scratch_shapes=[
            pltpu.VMEM((S, D), bf16),
            pltpu.VMEM((3, D, D), bf16),
            pltpu.VMEM((AD, AD, AH), bf16),
            pltpu.VMEM((D, D), bf16),
            pltpu.VMEM((M, D), bf16),
            pltpu.VMEM((S, D), f32),
            pltpu.VMEM((S // 2, D), u32),
            pltpu.VMEM((64, D), f32),
            pltpu.VMEM((NC, CR // 2, D), u32),
            pltpu.VMEM((NC, CR, D), u32),
            pltpu.VMEM((2 * CR, TS1), f32),
            pltpu.VMEM((NG, GR + 8, 2 * GR), f32),
            pltpu.VMEM((NG, GR + 8, 2 * GR), bf16),
            pltpu.VMEM((NW, 3, 2, 64, D), bf16),
            pltpu.VMEM((NW, D // 2, PW), u32),
            pltpu.VMEM((HE, D), bf16),
            pltpu.VMEM((NP, PW // 2, D), u32),
            pltpu.VMEM((NP, 16, 2 * PW), f32),
            pltpu.VMEM((NP, 16, 2 * PW), f32),
            pltpu.VMEM((NP, 16, 512), f32),
            pltpu.SemaphoreType.DMA((NSEM,)),
        ],
        compiler_params=pltpu.CompilerParams(vmem_limit_bytes=110 * 1024 * 1024,
                                             disable_bounds_checks=True,
                                             disable_semaphore_checks=True),
    )(x, A_wqkv, wphi, A_wo, mem0, bq, bk, bv, bo)
    return out.reshape(1, S, D)
```

```python
import jax
import jax.numpy as jnp
from jax import lax
import jax.experimental.pallas as pl
import jax.experimental.pallas.tpu as pltpu

bf16 = jnp.bfloat16
f32 = jnp.float32
u32 = jnp.uint32
i32 = jnp.int32

CFG = dict(
    pe="k0 q0 v0 S1 P2", po="q0 k0 q0 S1 v0 q0 P3",
    te=(3, 4, 2, 3), to=(1, 2, 2, 1, 2), tl=(2, 2, 2, 2, 0),
    de=1, do=0, ge="b", go="b", po1="k0 q0 S1 v0 q0 v0 q0 v0 P3",
    pe0="k0 q0 v0 S1 O0 P2", te0=(3, 3, 2, 3), de0=2, po0="k0 q0 S1 q0 v0 q0 P2", to0=(2, 3, 1, 3), go0="k",
)

S = 2048
D = 640
LOG2E = 1.4426950408889634
AH = 32
AD = 20
GR = 2 * AD
NG = AH // 2
CG = 4
CR = CG * GR
NC = NG // CG
TA = 512
TS1 = 128
TS2 = 256
NB = S // TA
BH = 32
BE = 192
HE = BH * BE
M = 8
SEG = 32
L = M + SEG
NP = BH // 2
PW = 2 * BE
QSCALE = BE ** -0.5 * LOG2E
MASKED = -1e9 * LOG2E
UB = 2
TB = 64 * UB
NI = S // TB
NW = 3 * NP
WI = NW // NB
NWO = 16

NT = (((1,), (1,)), ((), ()))

SEM_PHI, SEM_K, SEM_QV, SEM_OUT = 0, 1, 2, 3
SEM_X = 4
SEM_W = SEM_X + NB
SEM_WO = SEM_W + NB
NSEM = SEM_WO + NWO


def _dot(a, b):
    return jnp.dot(a, b, preferred_element_type=f32)


def _dot_nt(a, b):
    return lax.dot_general(a, b, NT, preferred_element_type=f32)


def _pack(x):
    return pltpu.bitcast(x, u32)


def _unpack(x):
    return pltpu.bitcast(x, bf16)


def _recip(x):
    r = pl.reciprocal(x, approx=True)
    return r * (2.0 - x * r)


def _layernorm(x):
    m = jnp.mean(x, axis=-1, keepdims=True)
    xc = x - m
    v = jnp.mean(xc * xc, axis=-1, keepdims=True)
    return xc * lax.rsqrt(v + 1e-5)


def _freduce(x3, red, op):
    r = red(x3, axis=0, keepdims=True)
    r = op(r, pltpu.roll(r, 2, 1))
    return op(r, pltpu.roll(r, 4, 1))


def _hedgehog(p):
    t = p.shape[1]
    p3 = p.reshape(GR // 8, 8, t)
    ep = jnp.exp2(p3 - _freduce(p3, jnp.max, jnp.maximum))
    en = jnp.exp2(_freduce(p3, jnp.min, jnp.minimum) - p3)
    ep = ep * _recip(_freduce(ep, jnp.sum, jnp.add))
    en = en * _recip(_freduce(en, jnp.sum, jnp.add))
    return jnp.concatenate([ep, en], axis=0).reshape(2 * GR, t).astype(bf16)


def _stage_q(y):
    lo = lax.broadcasted_iota(i32, (y.shape[0], 128), 1) < 64
    y = y * QSCALE
    qm = y[:, 128:256]
    return jnp.concatenate([y[:, :128], jnp.where(lo, qm, 0.0), jnp.where(lo, 0.0, qm), y[:, 256:]], axis=1)


def _after(x, dep, zero):
    d = pltpu.bitcast(dep, i32) & zero
    d = jnp.concatenate([d] * (x.shape[1] // 128), axis=1)
    return pltpu.bitcast(pltpu.bitcast(x, i32) | d, f32)


def _b_schedule(period, tail):
    if "O" not in period:
        period += " O0"
    ops = [(t[0], int(t[1:])) for t in period.split()]
    maxlag = max(lag for _, lag in ops)
    merged, tail = tail[-1], tail[:-1]
    assert len(tail) == maxlag + 1
    nin = NP - sum(tail) - merged
    out, o = [], 0
    for t in range(NP + maxlag + 1):
        if t >= NP:
            out += [("O", o + i) for i in range(tail[t - NP])]
            o += tail[t - NP]
        for op, lag in ops:
            if op != "O":
                if 0 <= t - lag < NP:
                    out.append((op, t - lag))
            elif NP - nin <= t < NP:
                out.append(("O", o))
                o += 1
    if merged:
        out.append(("M", o))
    return out


def _kernel(x_hbm, wqkv_hbm, wphi_hbm, wo_hbm, mem_hbm, bq_hbm, bk_hbm, bv_hbm, bo_hbm,
            out_hbm,
            xin, wqkv_v, wphi_v, wo_v, mem_v, xa, xna, xnb, wq_s, wkv_s, ylast, kv_acc, kv_s,
            stage, wb_s, bo_v, bo_s, sv_o, sv_e, sv_q, sems):
    def copy(src, dst, slot):
        return pltpu.make_async_copy(src, dst, sems.at[slot])

    def a_copy(t, slot):
        return copy(wqkv_hbm.at[:, pl.ds(t * D, D)], wqkv_v.at[t], slot)

    def x_copy(r0, n, slot):
        return copy(x_hbm.at[pl.ds(r0, n)], xin.at[pl.ds(r0, n)], slot)

    def w_start(q0, q1, slot):
        while q0 < q1:
            t, j = divmod(q0, NP)
            n = min(q1 - q0, NP - j)
            if t < 2:
                copy((bq_hbm, bk_hbm)[t].at[pl.ds(j, n)], stage.at[pl.ds(q0, n)], slot).start()
            else:
                for hh in range(2):
                    copy(bv_hbm.at[pl.ds(j, n), hh], stage.at[pl.ds(q0, n), :, hh], slot).start()
            q0 += n

    def bo_copy(b):
        rows = pl.ds(pl.multiple_of(b * (HE // NWO), HE // NWO), HE // NWO)
        return copy(bo_hbm.at[rows], bo_v.at[rows], SEM_WO + b)

    def out_copy(b):
        rows = pl.ds(pl.multiple_of(b * TB, TB), TB)
        return copy(xin.at[rows], out_hbm.at[rows], SEM_OUT)

    first_copies = [a_copy(2, SEM_QV), a_copy(0, SEM_QV), x_copy(0, TS1, SEM_QV), copy(mem_hbm, mem_v, SEM_QV)]
    copy(wphi_hbm, wphi_v, SEM_PHI).start()
    a_copy(1, SEM_K).start()
    for cp in first_copies:
        cp.start()
    for b in range(NB):
        x_copy(b * TA + TS1, TA if b + 1 < NB else TA - TS1, SEM_X + b).start()
    copy(wo_hbm, wo_v, SEM_X + NB - 1).start()
    for b in range(NB):
        w_start(b * WI, (b + 1) * WI, SEM_W + b)
    for b in range(NWO):
        bo_copy(b).start()

    kv_acc[...] = jnp.zeros_like(kv_acc)
    ylast[...] = jnp.zeros_like(ylast)
    copy(wphi_hbm, wphi_v, SEM_PHI).wait()
    row = lax.broadcasted_iota(i32, (AH, D), 0)
    col = lax.broadcasted_iota(i32, (AH, D), 1)
    dsel = col - AD * row
    wf = None
    for d in range(AD):
        y = _dot(wphi_v[d], (dsel == d).astype(bf16))
        wf = y if wf is None else y + wf
    wf = wf.astype(bf16)
    row = lax.broadcasted_iota(i32, (CR, AD), 0)
    col = lax.broadcasted_iota(i32, (CR, AD), 1)
    sel = (((row % GR) // 2) == col).astype(bf16)
    row = lax.broadcasted_iota(i32, (CR, 256), 0)
    col = lax.broadcasted_iota(i32, (CR, 256), 1)
    head = (row // GR) * 2 + row % 2
    phit = []
    for c in range(NC):
        rep = _dot(sel, wf[:, c * 128:c * 128 + 256])
        keep = (head + c * 2 * CG) == (col + c * 128) // AD
        phit.append(jnp.where(keep, rep, 0.0).astype(bf16))

    def fold(t, c):
        return _pack((_dot_nt(phit[c], wqkv_v[t, :, c * 128:c * 128 + 256]) * LOG2E).astype(bf16))

    a_copy(1, SEM_K).wait()
    for c in range(NC):
        wkv_s[c, :CR // 2] = fold(1, c)
    for cp in first_copies:
        cp.wait()
    wvt = wqkv_v[2].T
    for c in range(NC):
        wkv_s[c, CR // 2:] = _pack(wvt[c * CR:(c + 1) * CR])
        wq_s[c] = fold(0, c)

    def layer_a(li):
        first = li == 0

        def ln_rows(r0, n):
            rows = pl.ds(pl.multiple_of(r0, n), n)
            xn = _layernorm(xin[rows, :].astype(f32)).astype(bf16)
            xna[pl.ds(pl.multiple_of(r0 // 2, n // 2), n // 2), :] = _pack(xn)
            return xn

        def xn_rows(r0, n):
            return _unpack(xna[pl.ds(pl.multiple_of(r0 // 2, n // 2), n // 2), :])

        def kv_update(c, y, ones):
            for u in range(CG):
                phi = _hedgehog(y[u * GR:(u + 1) * GR])
                vt = jnp.concatenate([y[CR + u * GR:CR + (u + 1) * GR], ones], axis=0).astype(bf16)
                kv_acc[c * CG + u] += _dot_nt(vt, phi)

        def pass1(i, carry):
            @pl.when(first)
            def _():
                @pl.when(i + 1 < NB)
                def _():
                    x_copy(pl.multiple_of(i * TA + TS1, TS1), TA, SEM_X + i).wait()

                @pl.when(i + 1 == NB)
                def _():
                    x_copy(S - TA + TS1, TA - TS1, SEM_X + NB - 1).wait()
                    copy(wo_hbm, wo_v, SEM_X + NB - 1).wait()

            ones = jnp.ones((8, TS1), f32)
            pend = (NC - 1, ylast[...], jnp.where(i > 0, ones, 0.0))
            for s in range(TA // TS1):
                r0 = i * TA + s * TS1
                xn = xn_rows(r0, TS1) if s == 0 else ln_rows(r0, TS1)
                for c in range(NC):
                    y = _dot_nt(_unpack(wkv_s[c]), xn)
                    kv_update(*pend)
                    pend = (c, y, ones)
            ylast[...] = pend[1]
            ln_rows(jnp.minimum(i + 1, NB - 1) * TA, TS1)
            return carry

        def pass2(i, carry):
            @pl.when(first)
            def _():
                chunk = stage.at[pl.ds(i * WI, WI)]
                copy(chunk, chunk, SEM_W + i).wait()

            sub = lax.broadcasted_iota(i32, (8, TS2), 0) < 4
            ot = {}

            def feat(s, c, p):
                for u in range(CG):
                    g = c * CG + u
                    y = _dot(kv_s[g], _hedgehog(p[u * GR:(u + 1) * GR]))
                    r = _recip(y[GR:] + 1e-6)
                    rr = pltpu.roll(r, 4, 0)
                    r0, r1 = jnp.where(sub, r, rr), jnp.where(sub, rr, r)
                    ot[s, g] = y[:GR] * jnp.concatenate([r0, r0, r, r1, r1], axis=0)

            def back(s, half, fill=()):
                lo = half * 128
                o = jnp.concatenate([ot[s, g][:, lo:lo + 128] for g in range(NG)], axis=0).T.astype(bf16)
                rows = pl.ds(pl.multiple_of(i * TA + s * TS2 + lo, 128), 128)
                ys = []
                for n in range(5) if fill else ():
                    ys.append(_dot(o, wo_v[:, n * 128:(n + 1) * 128]))
                    if fill[n] is not None:
                        q_piece(*fill[n])
                y = jnp.concatenate(ys, axis=1) if fill else _dot(o, wo_v[...])
                xa[rows, :] = xin[rows, :].astype(f32) + y

            for u in range(WI):
                wb_s[i * WI + u] = _pack(stage[i * WI + u].reshape(PW, D).T)
            kv_acc[...] = jnp.zeros_like(kv_acc)
            ylast[...] = jnp.zeros_like(ylast)
            pend = []
            for s in range(2):
                xn = xn_rows(i * TA + s * TS2, TS2)
                for c in range(NC):
                    pend.append((s, c, _dot_nt(_unpack(wq_s[c]), xn)))
                    if len(pend) > 2:
                        feat(*pend.pop(0))
            back(0, 0)
            while pend:
                feat(*pend.pop(0))
            xn0 = _layernorm(xa[0:64, :])
            xnb[...] = xn0
            h8 = xn0[0:16].astype(bf16)
            qparts = {}

            def q_piece(u, n):
                j = i * (NP // NB) + u
                qparts[u, n] = _dot_nt(h8, stage[j, n].reshape(128, D))[:8]
                if n == 2:
                    sv_q[j, 8:16, :] = _stage_q(jnp.concatenate([qparts[u, m] for m in range(3)], axis=1))

            fill = [None, None] + [(u, n) for u in range(NP // NB) for n in range(3)] + [None]
            back(0, 1, fill[0:5])
            back(1, 0, fill[5:10])
            back(1, 1, fill[10:15])
            return carry

        ln_rows(0, TS1)
        lax.fori_loop(0, NB, pass1, 0)
        kv_update(NC - 1, ylast[...], jnp.ones((8, TS1), f32))
        row = lax.broadcasted_iota(i32, (GR + 8, 2 * GR), 0)
        col = lax.broadcasted_iota(i32, (GR + 8, 2 * GR), 1)
        keep = jnp.where(row < GR, row // AD, (row - GR) // 4) == col % 2
        for g in range(NG):
            kv_s[g] = jnp.where(keep, kv_acc[g], 0.0).astype(bf16)
        lax.fori_loop(0, NB, pass2, 0)

        @pl.when(first)
        def _():
            def repack(b, carry):
                bo_copy(b).wait()
                for u in range(NP // NWO):
                    j = b * (NP // NWO) + u
                    rows = [bo_v[pl.ds(pl.multiple_of(j * PW + hh * BE + cb * 64, 64), 64), :]
                            for cb in range(3) for hh in range(2)]
                    bo_s[j] = _pack(jnp.concatenate(rows, axis=0))
                return carry
            lax.fori_loop(0, NWO, repack, 0)

    def layer_b(li):
        lo40 = lax.broadcasted_iota(i32, (L, 128), 1) < 64
        zero40 = jnp.zeros((L, 128), f32)
        pad = jnp.zeros((128 - 2 * L, PW), f32)

        def blockdiag_k(k):
            kmid = k[:, 128:256]
            top = jnp.concatenate([k[:, :128], jnp.where(lo40, kmid, zero40), zero40], axis=1)
            bot = jnp.concatenate([zero40, jnp.where(lo40, zero40, kmid), k[:, 256:]], axis=1)
            return jnp.concatenate([top, bot, pad], axis=0).astype(bf16)

        def blockdiag_v(v):
            t = [v[:, cb * 128:(cb + 1) * 128] for cb in range(3)]
            top = jnp.concatenate([jnp.where(lo40, x, zero40) for x in t], axis=1)
            bot = jnp.concatenate([jnp.where(lo40, zero40, x) for x in t], axis=1)
            return jnp.concatenate([top, bot, pad], axis=0).astype(bf16)

        r = lax.broadcasted_iota(i32, (32, 128), 0)
        c = lax.broadcasted_iota(i32, (32, 128), 1)
        isa = c < L
        key = jnp.where(isa, c, c - L)
        valid = ((r < M) | (r >= key) | (key >= 32)) & (key < L)
        r = lax.broadcasted_iota(i32, (128, 128), 0)
        causal8 = r % 8 >= r // 8 - 8
        lo128 = lax.broadcasted_iota(i32, (128, 128), 1) < 64

        def rows8(kv, j, c0, n):
            return jnp.concatenate([jnp.broadcast_to(kv[j, t:t + 1, c0:c0 + n], (8, n)) for t in range(16)], axis=0)

        def head8(q, kv, j):
            q = jnp.concatenate([q] * 16, axis=0)
            k = rows8(kv, j, 0, PW)
            k0, k1, k2 = k[:, 0:128], k[:, 128:256], k[:, 256:384]
            sa = jnp.sum(q[:, 0:128] * k0 + q[:, 128:256] * k1, axis=1, keepdims=True)
            sb = jnp.sum(q[:, 384:512] * k2 + q[:, 256:384] * k1, axis=1, keepdims=True)
            s = jnp.where(causal8, jnp.where(lo128, sa, sb), MASKED).reshape(16, 8, 128)
            e = jnp.exp2(s - jnp.max(s, axis=0, keepdims=True))
            rl = _recip(jnp.sum(e, axis=0))
            vs = [rows8(kv, j, PW + cb * 128, 128) for cb in range(3)]
            return jnp.concatenate([jnp.sum(e * v.reshape(16, 8, 128), axis=0) * rl for v in vs], axis=1)

        def softmax(s):
            s = jnp.where(valid, s * QSCALE, MASKED)
            ma = jnp.max(jnp.where(isa, s, -jnp.inf), axis=1, keepdims=True)
            mb = jnp.max(jnp.where(isa, -jnp.inf, s), axis=1, keepdims=True)
            e = jnp.exp2(s - jnp.where(isa, ma, mb))
            la = jnp.sum(jnp.where(isa, e, 0.0), axis=1, keepdims=True)
            lb = jnp.sum(jnp.where(isa, 0.0, e), axis=1, keepdims=True)
            return e * _recip(jnp.where(isa, la, lb))

        def step(h, even, u, zero, o1e):
            first, last = even and u == 0, (not even) and u == UB - 1
            eo = "e" if even else "o"

            def opt(name):
                return CFG.get(name + eo + str(u), CFG[name + eo])

            period = opt("p")
            sched = _b_schedule(period, CFG["tl"] if last else opt("t"))
            widx = dict(q=0, k=NP, v=2 * NP)
            kv = sv_e if even else sv_o

            def proj(op, j, k0, k1, n0=0, n1=3):
                hh = h if (op == "q") != even else h[:32]
                w = wb_s[widx[op] + j, k0 * 64:k1 * 64, n0 * 128:n1 * 128]
                return _dot(hh[:, k0 * 128:k1 * 128], _unpack(w))

            part, kdone = {}, 0
            for k1 in (() if first else (2, 3)):
                for op in dict.fromkeys(op for op, j in sched if op in widx and j == 0):
                    y = proj(op, 0, kdone, k1)
                    part[op] = y + part[op] if op in part else y
                kdone = k1

            val, acc, o1 = {}, None, {}

            def lhs_o(j):
                o = val.pop(("o", j))
                if even:
                    return o
                return jnp.concatenate([o, jnp.concatenate([o1e[j], o1[j]], axis=0).astype(bf16)], axis=0)

            for op, j in sched:
                if op in widx:
                    done = val.setdefault((op, j, "n"), [])
                    n0, n1 = (len(done), len(done) + 1) if period.count(op) == 3 else (0, 3)
                    if j == 0 and part:
                        done.append(proj(op, j, kdone, 5, n0, n1) + part[op][:, n0 * 128:n1 * 128])
                    else:
                        done.append(proj(op, j, 0, 5, n0, n1))
                    if "waiting" in val:
                        val["gate", val.pop("waiting")] = done[-1][:8, :128]
                    if n1 < 3:
                        continue
                    y = jnp.concatenate(done, axis=1)
                    if op == "q":
                        val["q", j] = y[:32]
                        if not even:
                            sv_q[j] = _stage_q(y[32:])
                        continue
                    cols = slice(0, PW) if op == "k" else slice(PW, 2 * PW)
                    kv[j, 0:8, cols] = y[0:8]
                    if even:
                        sv_e[j, 8:16, cols] = y[32:40]
                        sv_o[j, 8:16, cols] = y[40:48]
                        y = y[:40]
                    else:
                        y = jnp.concatenate([y, sv_o[j, 8:16, cols]], axis=0)
                    val[op, j] = blockdiag_k(y) if op == "k" else blockdiag_v(y)
                    if opt("g") == op or (opt("g") == "b" and ("k", j) in val and ("v", j) in val):
                        val["waiting"] = j
                elif op == "S":
                    q1 = sv_q[j, 8:16, :] if even else sv_q[j, 0:8, :]
                    if ("gate", j) in val:
                        q1 = _after(q1, val.pop(("gate", j)), zero)
                    o1[j] = head8(q1, kv, j)
                    val["p", j] = softmax(_dot_nt(val.pop(("q", j)).astype(bf16), val.pop(("k", j))))
                elif op == "P":
                    p = val.pop(("p", j))
                    if j - opt("d") in o1:
                        dep = o1[j - opt("d")]
                        dep = dep[:, :128] + dep[:, 128:256] + dep[:, 256:]
                        p = jnp.concatenate([_after(p[:8], dep, zero), p[8:]], axis=0)
                    val["o", j] = _dot(p.astype(bf16), val.pop(("v", j))).astype(bf16)
                elif op == "M":
                    o = jnp.concatenate([lhs_o(jj) for jj in range(j, NP)], axis=1)
                    acc = _dot(o, _unpack(jnp.concatenate([bo_s[jj] for jj in range(j, NP)], axis=0))) + acc
                else:
                    y = _dot(lhs_o(j), _unpack(bo_s[j]))
                    acc = y if acc is None else y + acc
                    if "waiting" in val:
                        val["gate", val.pop("waiting")] = acc[:8, :128]
            return acc, o1

        def body(i, mem):
            zero = i // NI
            rn = pl.multiple_of(jnp.minimum(i + 1, NI - 1) * TB, TB)
            xns = [xnb[...]] + [_layernorm(xa[pl.ds(pl.multiple_of((i * UB + u) * 64, 64), 64), :])
                                for u in range(1, UB)]
            xns.append(_layernorm(xa[pl.ds(rn, 64), :]))
            for u in range(UB):
                r0 = pl.multiple_of((i * UB + u) * 64, 64)

                def add_rows(off, y):
                    rows = pl.ds(r0 + off, y.shape[0])
                    xin[rows, :] = (xa[rows, :] + y).astype(bf16)

                xn = xns[u]
                h = jnp.concatenate([mem, xn[8:32], xn[0:8], xn[32:40]], axis=0).astype(bf16)
                ye, o1e = step(h, True, u, zero, None)
                mem = ye[:8]
                add_rows(16, ye[16:])
                h = jnp.concatenate([mem, xn[40:64], xn[32:40], xns[u + 1][0:8]], axis=0).astype(bf16)
                yo, _ = step(h, False, u, zero, o1e)
                mem = yo[:8]
                add_rows(48, yo[16:32])
                add_rows(0, jnp.concatenate([yo[32:40], ye[8:16]], axis=0))
                add_rows(32, jnp.concatenate([yo[40:48], yo[8:16]], axis=0))
            xnb[...] = xns[UB]

            @pl.when(li == 1)
            def _():
                out_copy(i).start()
            return mem

        lax.fori_loop(0, NI, body, mem_v[...].astype(f32))

    def layer(li, carry):
        layer_a(li)
        layer_b(li)
        return carry

    lax.fori_loop(0, 2, layer, 0)
    copy(xin, out_hbm, SEM_OUT).wait()


@jax.jit
def pallas_interleave_layers__linear_kernel_hedgehog__memory_aug_recurrent_mem_tr__prompt_kernel(
    A_x: jax.Array,
    A_wqkv: jax.Array,
    A_w_phi: jax.Array,
    A_wo: jax.Array,
    B_x: jax.Array,
    B_mem0: jax.Array,
    B_Wq: jax.Array,
    B_Wk: jax.Array,
    B_Wv: jax.Array,
    B_Wo: jax.Array,
    B_seg_len=SEG,
):
    del B_x, B_seg_len
    x = A_x.reshape(S, D)
    wphi = A_w_phi.transpose(1, 2, 0)
    mem0 = B_mem0.reshape(M, D)
    bq = B_Wq.transpose(1, 2, 0).reshape(NP, 3, 2, 64, D)
    bk = B_Wk.transpose(1, 2, 0).reshape(NP, 3, 2, 64, D)
    bv = B_Wv.transpose(1, 2, 0).reshape(NP, 2, 3, 64, D)
    bo = B_Wo.reshape(HE, D)

    anyspec = pl.BlockSpec(memory_space=pl.ANY)
    out = pl.pallas_call(
        _kernel,
        out_shape=jax.ShapeDtypeStruct((S, D), bf16),
        in_specs=[anyspec] * 9,
        out_specs=anyspec,
        scratch_shapes=[
            pltpu.VMEM((S, D), bf16),
            pltpu.VMEM((3, D, D), bf16),
            pltpu.VMEM((AD, AD, AH), bf16),
            pltpu.VMEM((D, D), bf16),
            pltpu.VMEM((M, D), bf16),
            pltpu.VMEM((S, D), f32),
            pltpu.VMEM((S // 2, D), u32),
            pltpu.VMEM((64, D), f32),
            pltpu.VMEM((NC, CR // 2, D), u32),
            pltpu.VMEM((NC, CR, D), u32),
            pltpu.VMEM((2 * CR, TS1), f32),
            pltpu.VMEM((NG, GR + 8, 2 * GR), f32),
            pltpu.VMEM((NG, GR + 8, 2 * GR), bf16),
            pltpu.VMEM((NW, 3, 2, 64, D), bf16),
            pltpu.VMEM((NW, D // 2, PW), u32),
            pltpu.VMEM((HE, D), bf16),
            pltpu.VMEM((NP, PW // 2, D), u32),
            pltpu.VMEM((NP, 16, 2 * PW), f32),
            pltpu.VMEM((NP, 16, 2 * PW), f32),
            pltpu.VMEM((NP, 16, 512), f32),
            pltpu.SemaphoreType.DMA((NSEM,)),
        ],
        compiler_params=pltpu.CompilerParams(vmem_limit_bytes=110 * 1024 * 1024,
                                             disable_bounds_checks=True,
                                             disable_semaphore_checks=True),
    )(x, A_wqkv, wphi, A_wo, mem0, bq, bk, bv, bo)
    return out.reshape(1, S, D)
```

```python
import jax
import jax.numpy as jnp
from jax import lax
import jax.experimental.pallas as pl
import jax.experimental.pallas.tpu as pltpu

bf16 = jnp.bfloat16
f32 = jnp.float32
u32 = jnp.uint32
i32 = jnp.int32

CFG = dict(
    pe="k0 q0 v0 S1 P2", po="q0 k0 q0 S1 v0 q0 P3",
    te=(3, 4, 2, 3), to=(1, 2, 2, 1, 2), tl=(2, 2, 2, 2, 0),
    de=1, do=0, ge="b", go="b", po1="k0 q0 S1 v0 q0 v0 q0 v0 P3",
    pe0="k0 q0 v0 S1 O0 P2", te0=(3, 3, 2, 3), de0=2, po0="k0 q0 S1 q0 v0 q0 P2", to0=(2, 3, 1, 3), go0="k",
)

S = 2048
D = 640
LOG2E = 1.4426950408889634
AH = 32
AD = 20
GR = 2 * AD
NG = AH // 2
CG = 4
CR = CG * GR
NC = NG // CG
TA = 512
TS1 = 128
TS2 = 256
NB = S // TA
BH = 32
BE = 192
HE = BH * BE
M = 8
SEG = 32
L = M + SEG
NP = BH // 2
PW = 2 * BE
QSCALE = BE ** -0.5 * LOG2E
MASKED = -1e9 * LOG2E
UB = 2
TB = 64 * UB
NI = S // TB
PI = NP // NB
NWO = 16

NT = (((1,), (1,)), ((), ()))

SEM_PHI, SEM_K, SEM_QV, SEM_OUT = 0, 1, 2, 3
SEM_X = 4
SEM_W = SEM_X + NB
SEM_WO = SEM_W + NB
NSEM = SEM_WO + NWO


def _dot(a, b):
    return jnp.dot(a, b, preferred_element_type=f32)


def _dot_nt(a, b):
    return lax.dot_general(a, b, NT, preferred_element_type=f32)


def _pack(x):
    return pltpu.bitcast(x, u32)


def _unpack(x):
    return pltpu.bitcast(x, bf16)


def _recip(x):
    r = pl.reciprocal(x, approx=True)
    return r * (2.0 - x * r)


def _layernorm(x):
    m = jnp.mean(x, axis=-1, keepdims=True)
    xc = x - m
    v = jnp.mean(xc * xc, axis=-1, keepdims=True)
    return xc * lax.rsqrt(v + 1e-5)


def _freduce(x3, red, op):
    r = red(x3, axis=0, keepdims=True)
    r = op(r, pltpu.roll(r, 2, 1))
    return op(r, pltpu.roll(r, 4, 1))


def _hedgehog(p):
    t = p.shape[1]
    p3 = p.reshape(GR // 8, 8, t)
    ep = jnp.exp2(p3 - _freduce(p3, jnp.max, jnp.maximum))
    en = jnp.exp2(_freduce(p3, jnp.min, jnp.minimum) - p3)
    ep = ep * _recip(_freduce(ep, jnp.sum, jnp.add))
    en = en * _recip(_freduce(en, jnp.sum, jnp.add))
    return jnp.concatenate([ep, en], axis=0).reshape(2 * GR, t).astype(bf16)


def _stage_q(y):
    lo = lax.broadcasted_iota(i32, (y.shape[0], 128), 1) < 64
    y = y * QSCALE
    qm = y[:, 128:256]
    return jnp.concatenate([y[:, :128], jnp.where(lo, qm, 0.0), jnp.where(lo, 0.0, qm), y[:, 256:]], axis=1)


def _after(x, dep, zero):
    d = pltpu.bitcast(dep, i32) & zero
    d = jnp.concatenate([d] * (x.shape[1] // 128), axis=1)
    return pltpu.bitcast(pltpu.bitcast(x, i32) | d, f32)


def _b_schedule(period, tail):
    if "O" not in period:
        period += " O0"
    ops = [(t[0], int(t[1:])) for t in period.split()]
    maxlag = max(lag for _, lag in ops)
    merged, tail = tail[-1], tail[:-1]
    assert len(tail) == maxlag + 1
    nin = NP - sum(tail) - merged
    out, o = [], 0
    for t in range(NP + maxlag + 1):
        if t >= NP:
            out += [("O", o + i) for i in range(tail[t - NP])]
            o += tail[t - NP]
        for op, lag in ops:
            if op != "O":
                if 0 <= t - lag < NP:
                    out.append((op, t - lag))
            elif NP - nin <= t < NP:
                out.append(("O", o))
                o += 1
    if merged:
        out.append(("M", o))
    return out


def _kernel(x_hbm, wqkv_hbm, wphi_hbm, wo_hbm, mem_hbm, bq_hbm, bk_hbm, bv_hbm, bo_hbm,
            out_hbm,
            xin, wqkv_v, wphi_v, wo_v, mem_v, xa, xna, xnb, wq_s, wkv_s, ylast, kv_acc, kv_s,
            stage, wb_s, bo_v, bo_s, sv_o, sv_e, sv_q, sems):
    def copy(src, dst, slot):
        return pltpu.make_async_copy(src, dst, sems.at[slot])

    def a_copy(t, slot):
        return copy(wqkv_hbm.at[:, pl.ds(t * D, D)], wqkv_v.at[t], slot)

    def x_copy(r0, n, slot):
        return copy(x_hbm.at[pl.ds(r0, n)], xin.at[pl.ds(r0, n)], slot)

    def bo_copy(b):
        rows = pl.ds(pl.multiple_of(b * (HE // NWO), HE // NWO), HE // NWO)
        return copy(bo_hbm.at[rows], bo_v.at[rows], SEM_WO + b)

    def out_copy(b):
        rows = pl.ds(pl.multiple_of(b * TB, TB), TB)
        return copy(xin.at[rows], out_hbm.at[rows], SEM_OUT)

    first_copies = [a_copy(2, SEM_QV), a_copy(0, SEM_QV), x_copy(0, TS1, SEM_QV), copy(mem_hbm, mem_v, SEM_QV)]
    copy(wphi_hbm, wphi_v, SEM_PHI).start()
    a_copy(1, SEM_K).start()
    for cp in first_copies:
        cp.start()
    for b in range(NB):
        x_copy(b * TA + TS1, TA if b + 1 < NB else TA - TS1, SEM_X + b).start()
    copy(wo_hbm, wo_v, SEM_X + NB - 1).start()
    for b in range(NB):
        for t, w_hbm in enumerate((bq_hbm, bk_hbm, bv_hbm)):
            copy(w_hbm.at[pl.ds(b * PI * PW, PI * PW)], stage.at[b, t], SEM_W + b).start()
    for b in range(NWO):
        bo_copy(b).start()

    kv_acc[...] = jnp.zeros_like(kv_acc)
    ylast[...] = jnp.zeros_like(ylast)
    copy(wphi_hbm, wphi_v, SEM_PHI).wait()
    row = lax.broadcasted_iota(i32, (AH, D), 0)
    col = lax.broadcasted_iota(i32, (AH, D), 1)
    dsel = col - AD * row
    wf = None
    for d in range(AD):
        y = _dot(wphi_v[d], (dsel == d).astype(bf16))
        wf = y if wf is None else y + wf
    wf = wf.astype(bf16)
    row = lax.broadcasted_iota(i32, (CR, AD), 0)
    col = lax.broadcasted_iota(i32, (CR, AD), 1)
    sel = (((row % GR) // 2) == col).astype(bf16)
    row = lax.broadcasted_iota(i32, (CR, 256), 0)
    col = lax.broadcasted_iota(i32, (CR, 256), 1)
    head = (row // GR) * 2 + row % 2
    phit = []
    for c in range(NC):
        rep = _dot(sel, wf[:, c * 128:c * 128 + 256])
        keep = (head + c * 2 * CG) == (col + c * 128) // AD
        phit.append(jnp.where(keep, rep, 0.0).astype(bf16))

    def fold(t, c):
        return _pack((_dot_nt(phit[c], wqkv_v[t, :, c * 128:c * 128 + 256]) * LOG2E).astype(bf16))

    a_copy(1, SEM_K).wait()
    for c in range(NC):
        wkv_s[c, :CR // 2] = fold(1, c)
    for cp in first_copies:
        cp.wait()
    wvt = wqkv_v[2].T
    for c in range(NC):
        wkv_s[c, CR // 2:] = _pack(wvt[c * CR:(c + 1) * CR])
        wq_s[c] = fold(0, c)

    def layer_a(li):
        first = li == 0

        def ln_rows(r0, n):
            rows = pl.ds(pl.multiple_of(r0, n), n)
            xn = _layernorm(xin[rows, :].astype(f32)).astype(bf16)
            xna[pl.ds(pl.multiple_of(r0 // 2, n // 2), n // 2), :] = _pack(xn)
            return xn

        def xn_rows(r0, n):
            return _unpack(xna[pl.ds(pl.multiple_of(r0 // 2, n // 2), n // 2), :])

        def kv_update(c, y, ones):
            for u in range(CG):
                phi = _hedgehog(y[u * GR:(u + 1) * GR])
                vt = jnp.concatenate([y[CR + u * GR:CR + (u + 1) * GR], ones], axis=0).astype(bf16)
                kv_acc[c * CG + u] += _dot_nt(vt, phi)

        def pass1(i, carry):
            @pl.when(first)
            def _():
                @pl.when(i + 1 < NB)
                def _():
                    x_copy(pl.multiple_of(i * TA + TS1, TS1), TA, SEM_X + i).wait()

                @pl.when(i + 1 == NB)
                def _():
                    x_copy(S - TA + TS1, TA - TS1, SEM_X + NB - 1).wait()
                    copy(wo_hbm, wo_v, SEM_X + NB - 1).wait()

            ones = jnp.ones((8, TS1), f32)
            pend = (NC - 1, ylast[...], jnp.where(i > 0, ones, 0.0))
            for s in range(TA // TS1):
                r0 = i * TA + s * TS1
                xn = xn_rows(r0, TS1) if s == 0 else ln_rows(r0, TS1)
                for c in range(NC):
                    y = _dot_nt(_unpack(wkv_s[c]), xn)
                    kv_update(*pend)
                    pend = (c, y, ones)
            ylast[...] = pend[1]
            ln_rows(jnp.minimum(i + 1, NB - 1) * TA, TS1)
            return carry

        def pass2(i, carry):
            @pl.when(first)
            def _():
                copy(stage.at[i], stage.at[i], SEM_W + i).wait()

            sub = lax.broadcasted_iota(i32, (8, TS2), 0) < 4
            ot = {}

            def feat(s, c, p):
                for u in range(CG):
                    g = c * CG + u
                    y = _dot(kv_s[g], _hedgehog(p[u * GR:(u + 1) * GR]))
                    r = _recip(y[GR:] + 1e-6)
                    rr = pltpu.roll(r, 4, 0)
                    r0, r1 = jnp.where(sub, r, rr), jnp.where(sub, rr, r)
                    ot[s, g] = y[:GR] * jnp.concatenate([r0, r0, r, r1, r1], axis=0)

            def back(s, half, fill=()):
                lo = half * 128
                o = jnp.concatenate([ot[s, g][:, lo:lo + 128] for g in range(NG)], axis=0).T.astype(bf16)
                rows = pl.ds(pl.multiple_of(i * TA + s * TS2 + lo, 128), 128)
                ys = []
                for n in range(5) if fill else ():
                    ys.append(_dot(o, wo_v[:, n * 128:(n + 1) * 128]))
                    if fill[n] is not None:
                        q_piece(*fill[n])
                y = jnp.concatenate(ys, axis=1) if fill else _dot(o, wo_v[...])
                xa[rows, :] = xin[rows, :].astype(f32) + y

            for t in range(3):
                for u in range(PI):
                    if t < 2:
                        w = stage[i, t, u * PW:(u + 1) * PW, :]
                    else:
                        w = jnp.concatenate([stage[i, t, pl.ds(u * PW + hh * BE + cb * 64, 64), :]
                                             for cb in range(3) for hh in range(2)], axis=0)
                    wb_s[t * NP + i * PI + u] = _pack(w.T)
            kv_acc[...] = jnp.zeros_like(kv_acc)
            ylast[...] = jnp.zeros_like(ylast)
            pend = []
            for s in range(2):
                xn = xn_rows(i * TA + s * TS2, TS2)
                for c in range(NC):
                    pend.append((s, c, _dot_nt(_unpack(wq_s[c]), xn)))
                    if len(pend) > 2:
                        feat(*pend.pop(0))
            back(0, 0)
            while pend:
                feat(*pend.pop(0))
            xn0 = _layernorm(xa[0:64, :])
            xnb[...] = xn0
            h8 = xn0[0:16].astype(bf16)
            qparts = {}

            def q_piece(u, n):
                qparts[u, n] = _dot_nt(h8, stage[i, 0, pl.ds(u * PW + n * 128, 128), :])[:8]
                if n == 2:
                    sv_q[i * PI + u, 8:16, :] = _stage_q(jnp.concatenate([qparts[u, m] for m in range(3)], axis=1))

            fill = [None, None] + [(u, n) for u in range(PI) for n in range(3)] + [None]
            back(0, 1, fill[0:5])
            back(1, 0, fill[5:10])
            back(1, 1, fill[10:15])
            return carry

        ln_rows(0, TS1)
        lax.fori_loop(0, NB, pass1, 0)
        kv_update(NC - 1, ylast[...], jnp.ones((8, TS1), f32))
        row = lax.broadcasted_iota(i32, (GR + 8, 2 * GR), 0)
        col = lax.broadcasted_iota(i32, (GR + 8, 2 * GR), 1)
        keep = jnp.where(row < GR, row // AD, (row - GR) // 4) == col % 2
        for g in range(NG):
            kv_s[g] = jnp.where(keep, kv_acc[g], 0.0).astype(bf16)
        lax.fori_loop(0, NB, pass2, 0)

        @pl.when(first)
        def _():
            def repack(b, carry):
                bo_copy(b).wait()
                for u in range(NP // NWO):
                    j = b * (NP // NWO) + u
                    rows = [bo_v[pl.ds(pl.multiple_of(j * PW + hh * BE + cb * 64, 64), 64), :]
                            for cb in range(3) for hh in range(2)]
                    bo_s[j] = _pack(jnp.concatenate(rows, axis=0))
                return carry
            lax.fori_loop(0, NWO, repack, 0)

    def layer_b(li):
        lo40 = lax.broadcasted_iota(i32, (L, 128), 1) < 64
        zero40 = jnp.zeros((L, 128), f32)
        pad = jnp.zeros((128 - 2 * L, PW), f32)

        def blockdiag_k(k):
            kmid = k[:, 128:256]
            top = jnp.concatenate([k[:, :128], jnp.where(lo40, kmid, zero40), zero40], axis=1)
            bot = jnp.concatenate([zero40, jnp.where(lo40, zero40, kmid), k[:, 256:]], axis=1)
            return jnp.concatenate([top, bot, pad], axis=0).astype(bf16)

        def blockdiag_v(v):
            t = [v[:, cb * 128:(cb + 1) * 128] for cb in range(3)]
            top = jnp.concatenate([jnp.where(lo40, x, zero40) for x in t], axis=1)
            bot = jnp.concatenate([jnp.where(lo40, zero40, x) for x in t], axis=1)
            return jnp.concatenate([top, bot, pad], axis=0).astype(bf16)

        r = lax.broadcasted_iota(i32, (32, 128), 0)
        c = lax.broadcasted_iota(i32, (32, 128), 1)
        isa = c < L
        key = jnp.where(isa, c, c - L)
        valid = ((r < M) | (r >= key) | (key >= 32)) & (key < L)
        r = lax.broadcasted_iota(i32, (128, 128), 0)
        causal8 = r % 8 >= r // 8 - 8
        lo128 = lax.broadcasted_iota(i32, (128, 128), 1) < 64

        def rows8(kv, j, c0, n):
            return jnp.concatenate([jnp.broadcast_to(kv[j, t:t + 1, c0:c0 + n], (8, n)) for t in range(16)], axis=0)

        def head8(q, kv, j):
            q = jnp.concatenate([q] * 16, axis=0)
            k = rows8(kv, j, 0, PW)
            k0, k1, k2 = k[:, 0:128], k[:, 128:256], k[:, 256:384]
            sa = jnp.sum(q[:, 0:128] * k0 + q[:, 128:256] * k1, axis=1, keepdims=True)
            sb = jnp.sum(q[:, 384:512] * k2 + q[:, 256:384] * k1, axis=1, keepdims=True)
            s = jnp.where(causal8, jnp.where(lo128, sa, sb), MASKED).reshape(16, 8, 128)
            e = jnp.exp2(s - jnp.max(s, axis=0, keepdims=True))
            rl = _recip(jnp.sum(e, axis=0))
            vs = [rows8(kv, j, PW + cb * 128, 128) for cb in range(3)]
            return jnp.concatenate([jnp.sum(e * v.reshape(16, 8, 128), axis=0) * rl for v in vs], axis=1)

        def softmax(s):
            s = jnp.where(valid, s * QSCALE, MASKED)
            ma = jnp.max(jnp.where(isa, s, -jnp.inf), axis=1, keepdims=True)
            mb = jnp.max(jnp.where(isa, -jnp.inf, s), axis=1, keepdims=True)
            e = jnp.exp2(s - jnp.where(isa, ma, mb))
            la = jnp.sum(jnp.where(isa, e, 0.0), axis=1, keepdims=True)
            lb = jnp.sum(jnp.where(isa, 0.0, e), axis=1, keepdims=True)
            return e * _recip(jnp.where(isa, la, lb))

        def step(h, even, u, zero, o1e):
            first, last = even and u == 0, (not even) and u == UB - 1
            eo = "e" if even else "o"

            def opt(name):
                return CFG.get(name + eo + str(u), CFG[name + eo])

            period = opt("p")
            sched = _b_schedule(period, CFG["tl"] if last else opt("t"))
            widx = dict(q=0, k=NP, v=2 * NP)
            kv = sv_e if even else sv_o

            def proj(op, j, k0, k1, n0=0, n1=3):
                hh = h if (op == "q") != even else h[:32]
                w = wb_s[widx[op] + j, k0 * 64:k1 * 64, n0 * 128:n1 * 128]
                return _dot(hh[:, k0 * 128:k1 * 128], _unpack(w))

            part, kdone = {}, 0
            for k1 in (() if first else (2, 3)):
                for op in dict.fromkeys(op for op, j in sched if op in widx and j == 0):
                    y = proj(op, 0, kdone, k1)
                    part[op] = y + part[op] if op in part else y
                kdone = k1

            val, acc, o1 = {}, None, {}

            def lhs_o(j):
                o = val.pop(("o", j))
                if even:
                    return o
                return jnp.concatenate([o, jnp.concatenate([o1e[j], o1[j]], axis=0).astype(bf16)], axis=0)

            for op, j in sched:
                if op in widx:
                    done = val.setdefault((op, j, "n"), [])
                    n0, n1 = (len(done), len(done) + 1) if period.count(op) == 3 else (0, 3)
                    if j == 0 and part:
                        done.append(proj(op, j, kdone, 5, n0, n1) + part[op][:, n0 * 128:n1 * 128])
                    else:
                        done.append(proj(op, j, 0, 5, n0, n1))
                    if "waiting" in val:
                        val["gate", val.pop("waiting")] = done[-1][:8, :128]
                    if n1 < 3:
                        continue
                    y = jnp.concatenate(done, axis=1)
                    if op == "q":
                        val["q", j] = y[:32]
                        if not even:
                            sv_q[j] = _stage_q(y[32:])
                        continue
                    cols = slice(0, PW) if op == "k" else slice(PW, 2 * PW)
                    kv[j, 0:8, cols] = y[0:8]
                    if even:
                        sv_e[j, 8:16, cols] = y[32:40]
                        sv_o[j, 8:16, cols] = y[40:48]
                        y = y[:40]
                    else:
                        y = jnp.concatenate([y, sv_o[j, 8:16, cols]], axis=0)
                    val[op, j] = blockdiag_k(y) if op == "k" else blockdiag_v(y)
                    if opt("g") == op or (opt("g") == "b" and ("k", j) in val and ("v", j) in val):
                        val["waiting"] = j
                elif op == "S":
                    q1 = sv_q[j, 8:16, :] if even else sv_q[j, 0:8, :]
                    if ("gate", j) in val:
                        q1 = _after(q1, val.pop(("gate", j)), zero)
                    o1[j] = head8(q1, kv, j)
                    val["p", j] = softmax(_dot_nt(val.pop(("q", j)).astype(bf16), val.pop(("k", j))))
                elif op == "P":
                    p = val.pop(("p", j))
                    if j - opt("d") in o1:
                        dep = o1[j - opt("d")]
                        dep = dep[:, :128] + dep[:, 128:256] + dep[:, 256:]
                        p = jnp.concatenate([_after(p[:8], dep, zero), p[8:]], axis=0)
                    val["o", j] = _dot(p.astype(bf16), val.pop(("v", j))).astype(bf16)
                elif op == "M":
                    o = jnp.concatenate([lhs_o(jj) for jj in range(j, NP)], axis=1)
                    acc = _dot(o, _unpack(jnp.concatenate([bo_s[jj] for jj in range(j, NP)], axis=0))) + acc
                else:
                    y = _dot(lhs_o(j), _unpack(bo_s[j]))
                    acc = y if acc is None else y + acc
                    if "waiting" in val:
                        val["gate", val.pop("waiting")] = acc[:8, :128]
            return acc, o1

        def body(i, mem):
            zero = i // NI
            rn = pl.multiple_of(jnp.minimum(i + 1, NI - 1) * TB, TB)
            xns = [xnb[...]] + [_layernorm(xa[pl.ds(pl.multiple_of((i * UB + u) * 64, 64), 64), :])
                                for u in range(1, UB)]
            xns.append(_layernorm(xa[pl.ds(rn, 64), :]))
            for u in range(UB):
                r0 = pl.multiple_of((i * UB + u) * 64, 64)

                def add_rows(off, y):
                    rows = pl.ds(r0 + off, y.shape[0])
                    xin[rows, :] = (xa[rows, :] + y).astype(bf16)

                xn = xns[u]
                h = jnp.concatenate([mem, xn[8:32], xn[0:8], xn[32:40]], axis=0).astype(bf16)
                ye, o1e = step(h, True, u, zero, None)
                mem = ye[:8]
                add_rows(16, ye[16:])
                h = jnp.concatenate([mem, xn[40:64], xn[32:40], xns[u + 1][0:8]], axis=0).astype(bf16)
                yo, _ = step(h, False, u, zero, o1e)
                mem = yo[:8]
                add_rows(48, yo[16:32])
                add_rows(0, jnp.concatenate([yo[32:40], ye[8:16]], axis=0))
                add_rows(32, jnp.concatenate([yo[40:48], yo[8:16]], axis=0))
            xnb[...] = xns[UB]

            @pl.when(li == 1)
            def _():
                out_copy(i).start()
            return mem

        lax.fori_loop(0, NI, body, mem_v[...].astype(f32))

    def layer(li, carry):
        layer_a(li)
        layer_b(li)
        return carry

    lax.fori_loop(0, 2, layer, 0)
    copy(xin, out_hbm, SEM_OUT).wait()


@jax.jit
def pallas_interleave_layers__linear_kernel_hedgehog__memory_aug_recurrent_mem_tr__prompt_kernel(
    A_x: jax.Array,
    A_wqkv: jax.Array,
    A_w_phi: jax.Array,
    A_wo: jax.Array,
    B_x: jax.Array,
    B_mem0: jax.Array,
    B_Wq: jax.Array,
    B_Wk: jax.Array,
    B_Wv: jax.Array,
    B_Wo: jax.Array,
    B_seg_len=SEG,
):
    del B_x, B_seg_len
    x = A_x.reshape(S, D)
    wphi = A_w_phi.transpose(1, 2, 0)
    mem0 = B_mem0.reshape(M, D)
    bq = B_Wq.transpose(1, 2, 0).reshape(HE, D)
    bk = B_Wk.transpose(1, 2, 0).reshape(HE, D)
    bv = B_Wv.transpose(1, 2, 0).reshape(HE, D)
    bo = B_Wo.reshape(HE, D)

    anyspec = pl.BlockSpec(memory_space=pl.ANY)
    out = pl.pallas_call(
        _kernel,
        out_shape=jax.ShapeDtypeStruct((S, D), bf16),
        in_specs=[anyspec] * 9,
        out_specs=anyspec,
        scratch_shapes=[
            pltpu.VMEM((S, D), bf16),
            pltpu.VMEM((3, D, D), bf16),
            pltpu.VMEM((AD, AD, AH), bf16),
            pltpu.VMEM((D, D), bf16),
            pltpu.VMEM((M, D), bf16),
            pltpu.VMEM((S, D), f32),
            pltpu.VMEM((S // 2, D), u32),
            pltpu.VMEM((64, D), f32),
            pltpu.VMEM((NC, CR // 2, D), u32),
            pltpu.VMEM((NC, CR, D), u32),
            pltpu.VMEM((2 * CR, TS1), f32),
            pltpu.VMEM((NG, GR + 8, 2 * GR), f32),
            pltpu.VMEM((NG, GR + 8, 2 * GR), bf16),
            pltpu.VMEM((NB, 3, PI * PW, D), bf16),
            pltpu.VMEM((3 * NP, D // 2, PW), u32),
            pltpu.VMEM((HE, D), bf16),
            pltpu.VMEM((NP, PW // 2, D), u32),
            pltpu.VMEM((NP, 16, 2 * PW), f32),
            pltpu.VMEM((NP, 16, 2 * PW), f32),
            pltpu.VMEM((NP, 16, 512), f32),
            pltpu.SemaphoreType.DMA((NSEM,)),
        ],
        compiler_params=pltpu.CompilerParams(vmem_limit_bytes=110 * 1024 * 1024,
                                             disable_bounds_checks=True,
                                             disable_semaphore_checks=True),
    )(x, A_wqkv, wphi, A_wo, mem0, bq, bk, bv, bo)
    return out.reshape(1, S, D)
```
